```python
import jax
import jax.numpy as jnp

def _softmax(x, axis=-1):
    return jax.nn.softmax(x, axis=axis)

def _gelu(x):
    return jax.nn.gelu(x, approximate=True)

def _silu(x):
    return jax.nn.silu(x)

def _sigmoid(x):
    return jax.nn.sigmoid(x)

def _layernorm(x, axis=-1, eps=1e-05):
    m = jnp.mean(x, axis=axis, keepdims=True)
    v = jnp.var(x, axis=axis, keepdims=True)
    return (x - m) / jnp.sqrt(v + eps)

def _scatter_add(tgt, idx, src, axis=0):
    return tgt.at[idx].add(src)

def _segment_sum(src, seg, n):
    return jax.ops.segment_sum(src, seg, n)

class _Rng:

    def __init__(self, key):
        self._k = key

    def _next(self):
        self._k, sub = jax.random.split(self._k)
        return sub

    def normal(self, shape):
        return jax.random.normal(self._next(), shape, dtype=jnp.bfloat16)

    def randint(self, lo, hi, shape):
        return jax.random.randint(self._next(), shape, lo, hi, dtype=jnp.int32)

    def uniform(self, shape, lo=0.0, hi=1.0):
        return jax.random.uniform(self._next(), shape, jnp.bfloat16, lo, hi)

    def permutation(self, n):
        return jax.random.permutation(self._next(), n)
kernel_name = 'adaLN_cond__memory_aug_recurrent_mem_tr__glu_gated_swiglu__prompt'

def setup_inputs():
    _rng = _Rng(jax.random.key(int.from_bytes(__import__("os").urandom(4), "little")))
    _w = lambda a: (lambda t: t.astype(jnp.bfloat16) if jnp.issubdtype(t.dtype, jnp.floating) else t)(jnp.asarray(a))

    def _A_setup():
        B, S, Dm = (1, 2048, 1024)
        H, Dh = (32, 128)
        M, seg = (8, 32)
        seg = min(seg, S)
        S = S // seg * seg
        return {'x': _w((lambda *s: _rng.normal(s) * 0.05)(B, S, Dm)), 'mem0': _w((lambda *s: _rng.normal(s) * 0.05)(B, M, Dm)), 'Wq': _w((lambda *s: _rng.normal(s) * 0.05)(Dm, H, Dh) * Dm ** (-0.5)), 'Wk': _w((lambda *s: _rng.normal(s) * 0.05)(Dm, H, Dh) * Dm ** (-0.5)), 'Wv': _w((lambda *s: _rng.normal(s) * 0.05)(Dm, H, Dh) * Dm ** (-0.5)), 'Wo': _w((lambda *s: _rng.normal(s) * 0.05)(H, Dh, Dm) * (H * Dh) ** (-0.5)), 'seg_len': seg}
    _A_in = _A_setup()

    def _B_setup():
        B, S, D, F = (1, 2048, 1024, 3584)
        return {'x': _w((lambda *s: _rng.normal(s) * 0.05)(B, S, D)), 'w1': _w((lambda *s: _rng.normal(s) * 0.05)(D, F) * (2.0 / D) ** 0.5), 'w3': _w((lambda *s: _rng.normal(s) * 0.05)(D, F) * (2.0 / D) ** 0.5), 'w2': _w((lambda *s: _rng.normal(s) * 0.05)(F, D) * (2.0 / F) ** 0.5)}
    _B_in = _B_setup()
    return {'A_x': _A_in['x'], 'A_mem0': _A_in['mem0'], 'A_Wq': _A_in['Wq'], 'A_Wk': _A_in['Wk'], 'A_Wv': _A_in['Wv'], 'A_Wo': _A_in['Wo'], 'A_seg_len': _A_in['seg_len'], 'B_x': _B_in['x'], 'B_w1': _B_in['w1'], 'B_w3': _B_in['w3'], 'B_w2': _B_in['w2'], 'c': _w((lambda *s: _rng.normal(s) * 0.05)(1, 1024)), 'w_mod': _w((lambda *s: _rng.normal(s) * 0.05)(1024, 6 * 1024) * 1024 ** (-0.5))}

def reference(A_x, A_mem0, A_Wq, A_Wk, A_Wv, A_Wo, A_seg_len, B_x, B_w1, B_w3, B_w2, c, w_mod):

    def _A_ref(x, mem0, Wq, Wk, Wv, Wo, seg_len):
        B, S, Dm = x.shape
        H, Dh = (Wq.shape[1], Wq.shape[2])
        M = mem0.shape[1]
        scale = Dh ** (-0.5)
        n_seg = S // seg_len
        L = M + seg_len
        idx = jnp.arange(L)
        mask = (idx[:, None] < M) | (idx[:, None] >= idx[None, :])
        mem = mem0
        outs = []
        for s in range(n_seg):
            xs = x[:, s * seg_len:(s + 1) * seg_len, :].copy()
            h = jnp.concatenate([mem, xs], axis=1)
            q = jnp.einsum('btd,dhe->bhte', h, Wq)
            k = jnp.einsum('btd,dhe->bhte', h, Wk)
            v = jnp.einsum('btd,dhe->bhte', h, Wv)
            scores = jnp.einsum('bhqe,bhke->bhqk', q, k) * scale
            scores = jnp.where(mask[None, None], scores, -1000000000.0)
            p = _softmax(scores, axis=-1)
            o = jnp.einsum('bhqk,bhke->bhqe', p, v)
            o = jnp.einsum('bhte,hed->btd', o, Wo)
            mem = o[:, :M, :].copy()
            outs.append(o[:, M:, :])
        return jnp.concatenate(outs, axis=1)

    def _B_ref(x, w1, w3, w2):
        gate = jnp.einsum('bsd,df->bsf', x, w1)
        up = jnp.einsum('bsd,df->bsf', x, w3)
        h = _silu(gate) * up
        out = jnp.einsum('bsf,fd->bsd', h, w2)
        return out
    x = A_x
    mod = (_silu(c) @ w_mod).reshape(c.shape[0], 6, 1, -1)
    sa, ca, ga, sb, cb, gb = (mod[:, 0].copy(), mod[:, 1].copy(), mod[:, 2].copy(), mod[:, 3].copy(), mod[:, 4].copy(), mod[:, 5].copy())
    h = _layernorm(x, axis=-1) * (1 + ca) + sa
    x = x + ga * _A_ref(h, A_mem0, A_Wq, A_Wk, A_Wv, A_Wo, A_seg_len)
    h = _layernorm(x, axis=-1) * (1 + cb) + sb
    x = x + gb * _B_ref(h, B_w1, B_w3, B_w2)
    return x
```

```python
import functools

import jax
import jax.numpy as jnp
import jax.experimental.pallas as pl
import jax.experimental.pallas.tpu as pltpu

U32 = jnp.uint32
BF16 = jnp.bfloat16
F32 = jnp.float32
LN_EPS = 1e-5
FFN_SEGS = 4
N_STAGE = 24


def _bf(w):
    return pltpu.bitcast(w, BF16)


def _words(a):
    return pltpu.bitcast(a.astype(BF16), U32)


def _dot(a, b):
    return jax.lax.dot_general(a, b, (((1,), (0,)), ((), ())), preferred_element_type=F32)


def _dot_nt(a, b):
    return jax.lax.dot_general(a, b, (((1,), (1,)), ((), ())), preferred_element_type=F32)


def _round(a):
    return a.astype(BF16).astype(F32)


def _mod_ln(x, scale1, shift):
    m = jnp.mean(x, axis=-1, keepdims=True)
    d = x - m
    v = jnp.mean(d * d, axis=-1, keepdims=True)
    return d * jax.lax.rsqrt(v + LN_EPS) * scale1 + shift


def _kernel(c_ref, mem0_ref, x_hbm, wq_hbm, wk_hbm, wv_hbm, wo_hbm, w1_hbm, w3_hbm, w2_hbm,
            wmod_hbm, out_hbm,
            wqkv, wo, w1, w3, w2, wmod, stage, xs, outs, mod, lhs, obuf, x1, h2,
            sem_stage, sem_misc, sem_ffn, sem_out, *, seg, n_mem, dh):
    n_pairs = wqkv.shape[0]
    dm = lhs.shape[1]
    rows = n_mem + seg
    hseg = seg // 2
    n_seg = xs.shape[0] // hseg
    n_blk = n_seg // FFN_SEGS
    blk = FFN_SEGS * seg
    fc = w1.shape[2]
    scale = dh ** -0.5

    wmod32 = wmod_hbm.bitcast(U32)
    x32 = x_hbm.bitcast(U32)
    out32 = out_hbm.bitcast(U32)
    qkv32 = [w.bitcast(U32) for w in (wq_hbm, wk_hbm, wv_hbm)]
    cp_mod_a = pltpu.make_async_copy(wmod32.at[:, pl.ds(0, 2 * dm)], wmod.at[:, pl.ds(0, 2 * dm)],
                                     sem_misc.at[0])
    cp_mod_b = pltpu.make_async_copy(wmod32.at[:, pl.ds(2 * dm, 4 * dm)],
                                     wmod.at[:, pl.ds(2 * dm, 4 * dm)], sem_misc.at[1])
    cp_x = pltpu.make_async_copy(x32, xs, sem_misc.at[2])
    cp_wo = pltpu.make_async_copy(wo_hbm.bitcast(U32), wo, sem_misc.at[3])

    def cp_stage(i):
        return pltpu.make_async_copy(qkv32[i % 3].at[:, i // 3, :], stage.at[i % N_STAGE],
                                     sem_stage.at[i % N_STAGE])

    def cp_ffn(c):
        return [
            pltpu.make_async_copy(w1_hbm.bitcast(U32).at[:, pl.ds(c * fc, fc)], w1.at[c], sem_ffn.at[3 * c]),
            pltpu.make_async_copy(w3_hbm.bitcast(U32).at[:, pl.ds(c * fc, fc)], w3.at[c], sem_ffn.at[3 * c + 1]),
            pltpu.make_async_copy(w2_hbm.bitcast(U32).at[pl.ds(c * fc // 2, fc // 2), :], w2.at[c],
                                  sem_ffn.at[3 * c + 2]),
        ]

    def cp_out(b):
        r = pl.ds(pl.multiple_of(b * (blk // 2), blk // 2), blk // 2)
        return pltpu.make_async_copy(outs.at[r, :], out32.at[r, :], sem_out.at[b])

    cp_mod_a.start()
    cp_x.start()
    for i in range(N_STAGE):
        cp_stage(i).start()

    cf = c_ref[...].astype(F32)
    sc = jnp.broadcast_to(_round(cf * jax.nn.sigmoid(cf)), (8, dm))

    def set_mod(k, plus_one):
        m = _dot(sc, _bf(wmod[:, k * dm:(k + 1) * dm]))
        mod[k] = m + 1.0 if plus_one else m

    def get_mod(k, n):
        return jnp.concatenate([mod[k]] * (n // 8), axis=0)

    def seg_x(s):
        return _bf(xs[pl.ds(pl.multiple_of(s * hseg, hseg), hseg), :]).astype(F32)

    def seg_h(s):
        return _round(_mod_ln(seg_x(s), get_mod(1, seg), get_mod(0, seg)))

    cp_mod_a.wait()
    set_mod(0, False)
    set_mod(1, True)
    cp_x.wait()
    lhs[0:n_mem, :] = mem0_ref[...].astype(F32)
    lhs[n_mem:rows, :] = seg_h(0)

    for i in range(3 * n_pairs):
        cp_stage(i).wait()
        w = stage[i % N_STAGE]
        col = (i % 3) * 2 * dh
        wqkv[i // 3, :, col:col + dh] = _words(pltpu.bitcast(w << 16, F32))
        wqkv[i // 3, :, col + dh:col + 2 * dh] = _words(pltpu.bitcast(w & jnp.uint32(0xFFFF0000), F32))
        if i + N_STAGE < 3 * n_pairs:
            cp_stage(i + N_STAGE).start()
        if i + N_STAGE == 3 * n_pairs - 1:
            cp_wo.start()
            cp_mod_b.start()
    for c in range(FFN_SEGS):
        for cp in cp_ffn(c):
            cp.start()
    cp_wo.wait()
    cp_mod_b.wait()
    for k in range(2, 6):
        set_mod(k, k == 4)

    def step(s, do_attn, do_ffn):
        if do_ffn:
            fs = s - FFN_SEGS
            fb = fs // FFN_SEGS
            fch = fs % FFN_SEGS
            fslot = fb % 2
            hb = _bf(h2[fslot])
            acts = []

        def ffn_up(lo, hi):
            if do_ffn:
                g = _dot(hb, _bf(w1[fch, :, lo:hi]))
                u = _dot(hb, _bf(w3[fch, :, lo:hi]))
                acts.append((g * jax.nn.sigmoid(g) * u).astype(BF16))

        def ffn_down():
            if do_ffn:
                y = _dot(jnp.concatenate(acts, axis=1), _bf(w2[fch]))
                acc = x1[fslot] + get_mod(5, blk) * y
                x1[fslot] = acc
                outs[pl.ds(pl.multiple_of(fb * (blk // 2), blk // 2), blk // 2), :] = _words(acc)

        if not do_attn:
            ffn_up(0, fc)
            ffn_down()
        else:
            r = jax.lax.broadcasted_iota(jnp.int32, (2 * rows, 2 * rows), 0)
            q = jax.lax.broadcasted_iota(jnp.int32, (2 * rows, 2 * rows), 1)
            same = (r >= rows) == (q >= rows)
            rl = jnp.where(r >= rows, r - rows, r)
            ql = jnp.where(q >= rows, q - rows, q)
            keep = same & ((rl < n_mem) | (rl >= ql))
            fill = jnp.where(same, -1e9, -jnp.inf).astype(F32)
            a = lhs[...]
            qkv, probs = {}, {}

            def proj(j):
                t = _dot(a, _bf(wqkv[j]))
                qkv[j] = [jnp.concatenate([t[:, (2 * i) * dh:(2 * i + 1) * dh],
                                           t[:, (2 * i + 1) * dh:(2 * i + 2) * dh]], axis=0).astype(BF16)
                          for i in range(3)]

            def scores(j):
                t = jnp.where(keep, _dot_nt(qkv[j][0], qkv[j][1]) * scale, fill)
                e = jnp.exp(t - jnp.max(t, axis=-1, keepdims=True))
                probs[j] = (e / jnp.sum(e, axis=-1, keepdims=True)).astype(BF16)

            def mix(j):
                o = _round(_dot(probs[j], qkv[j][2]))
                obuf[:, 2 * j * dh:(2 * j + 1) * dh] = o[:rows]
                obuf[:, (2 * j + 1) * dh:(2 * j + 2) * dh] = o[rows:]

            def oproj(lo, hi):
                return _dot(obuf[:, lo * 2 * dh:hi * 2 * dh], _bf(wo[lo * dh:hi * dh, :]))

            for j in range(n_pairs):
                proj(j)
                if j >= 1:
                    scores(j - 1)
                if j >= 2:
                    mix(j - 2)
            ffn_up(0, 384)
            scores(n_pairs - 1)
            mix(n_pairs - 2)
            o = oproj(0, n_pairs // 2)
            mix(n_pairs - 1)
            ffn_up(384, fc)
            o = o + oproj(n_pairs // 2, n_pairs)
            ffn_down()
            lhs[0:n_mem, :] = _round(o[:n_mem])
            lhs[n_mem:rows, :] = seg_h(jnp.minimum(s + 1, n_seg - 1))
            xn = seg_x(s) + get_mod(2, seg) * o[n_mem:]
            slot = (s // FFN_SEGS) % 2
            sub = s % FFN_SEGS
            x1[slot, pl.ds(pl.multiple_of(sub * seg, seg), seg), :] = xn
            h2[slot, pl.ds(pl.multiple_of(sub * hseg, hseg), hseg), :] = _words(
                _mod_ln(xn, get_mod(4, seg), get_mod(3, seg)))

        if do_ffn:
            @pl.when(fch == FFN_SEGS - 1)
            def _():
                cp_out(fb).start()

    def run(lo, hi, do_attn, do_ffn):
        jax.lax.fori_loop(lo, hi, lambda s, _: step(s, do_attn, do_ffn), None)

    run(0, FFN_SEGS, True, False)
    for c in range(FFN_SEGS):
        for cp in cp_ffn(c):
            cp.wait()
    run(FFN_SEGS, n_seg, True, True)
    run(n_seg, n_seg + FFN_SEGS, False, True)
    for b in range(n_blk):
        cp_out(b).wait()


@functools.partial(jax.jit, static_argnames=("A_seg_len",))
def pallas_adaLN_cond__memory_aug_recurrent_mem_tr__glu_gated_swiglu__prompt_kernel(
    A_x, A_mem0, A_Wq, A_Wk, A_Wv, A_Wo, A_seg_len, B_x, B_w1, B_w3, B_w2, c, w_mod,
):
    del B_x
    bsz, s_len, dm = A_x.shape
    _, n_heads, dh = A_Wq.shape
    n_mem = A_mem0.shape[1]
    seg = int(A_seg_len)
    f = B_w1.shape[1]
    fc = f // FFN_SEGS
    blk = FFN_SEGS * seg
    assert bsz == 1 and s_len % blk == 0 and n_heads % 4 == 0 and fc % 128 == 0

    hbm = pl.BlockSpec(memory_space=pltpu.MemorySpace.HBM)
    vmem = pl.BlockSpec(memory_space=pltpu.MemorySpace.VMEM)
    out = pl.pallas_call(
        functools.partial(_kernel, seg=seg, n_mem=n_mem, dh=dh),
        out_shape=jax.ShapeDtypeStruct((s_len, dm), A_x.dtype),
        in_specs=[vmem, vmem] + [hbm] * 9,
        out_specs=hbm,
        scratch_shapes=[
            pltpu.VMEM((n_heads // 2, dm // 2, 6 * dh), U32),
            pltpu.VMEM((n_heads * dh // 2, dm), U32),
            pltpu.VMEM((FFN_SEGS, dm // 2, fc), U32),
            pltpu.VMEM((FFN_SEGS, dm // 2, fc), U32),
            pltpu.VMEM((FFN_SEGS, fc // 2, dm), U32),
            pltpu.VMEM((dm // 2, 6 * dm), U32),
            pltpu.VMEM((N_STAGE, dm, dh), U32),
            pltpu.VMEM((s_len // 2, dm), U32),
            pltpu.VMEM((s_len // 2, dm), U32),
            pltpu.VMEM((6, 8, dm), F32),
            pltpu.VMEM((n_mem + seg, dm), F32),
            pltpu.VMEM((n_mem + seg, n_heads * dh), F32),
            pltpu.VMEM((2, blk, dm), F32),
            pltpu.VMEM((2, blk // 2, dm), U32),
            pltpu.SemaphoreType.DMA((N_STAGE,)),
            pltpu.SemaphoreType.DMA((4,)),
            pltpu.SemaphoreType.DMA((3 * FFN_SEGS,)),
            pltpu.SemaphoreType.DMA((s_len // blk,)),
        ],
        compiler_params=pltpu.CompilerParams(vmem_limit_bytes=110 * 2**20),
    )(c, A_mem0.reshape(n_mem, dm), A_x.reshape(s_len, dm), A_Wq, A_Wk, A_Wv,
      A_Wo.reshape(n_heads * dh, dm), B_w1, B_w3, B_w2, w_mod)
    return out.reshape(bsz, s_len, dm)
```

```python
import functools

import jax
import jax.numpy as jnp
import jax.experimental.pallas as pl
import jax.experimental.pallas.tpu as pltpu

U32 = jnp.uint32
BF16 = jnp.bfloat16
F32 = jnp.float32
LN_EPS = 1e-5
FFN_SEGS = 4
N_STAGE = 6
N_PRE = 8
PRE_ROWS = 8


def _bf(w):
    return pltpu.bitcast(w, BF16)


def _words(a):
    return pltpu.bitcast(a.astype(BF16), U32)


def _dot(a, b):
    return jax.lax.dot_general(a, b, (((1,), (0,)), ((), ())), preferred_element_type=F32)


def _dot_nt(a, b):
    return jax.lax.dot_general(a, b, (((1,), (1,)), ((), ())), preferred_element_type=F32)


def _round(a):
    return a.astype(BF16).astype(F32)


def _mod_ln(x, scale1, shift):
    m = jnp.mean(x, axis=-1, keepdims=True)
    d = x - m
    v = jnp.mean(d * d, axis=-1, keepdims=True)
    return d * jax.lax.rsqrt(v + LN_EPS) * scale1 + shift


def _kernel(c_ref, mem0_ref, x_hbm, wq_hbm, wk_hbm, wv_hbm, wo_hbm, w1_hbm, w3_hbm, w2_hbm,
            wmod_hbm, out_hbm,
            wqkv, wo, w1, w3, w2, wmod, stage, xs, outs, mod, lhs, obuf, x1, h2, hpre, pre,
            sem_stage, sem_misc, sem_ffn, sem_out, *, seg, n_mem, dh):
    n_pairs = wqkv.shape[0]
    dm = lhs.shape[1]
    rows = n_mem + seg
    hseg = seg // 2
    n_seg = xs.shape[0] // hseg
    n_blk = n_seg // FFN_SEGS
    blk = FFN_SEGS * seg
    fc = w1.shape[2]
    scale = dh ** -0.5

    wmod32 = wmod_hbm.bitcast(U32)
    x32 = x_hbm.bitcast(U32)
    out32 = out_hbm.bitcast(U32)
    qkv32 = [w.bitcast(U32) for w in (wq_hbm, wk_hbm, wv_hbm)]
    cp_mod_a = pltpu.make_async_copy(wmod32.at[:, pl.ds(0, 2 * dm)], wmod.at[:, pl.ds(0, 2 * dm)],
                                     sem_misc.at[0])
    cp_mod_b = pltpu.make_async_copy(wmod32.at[:, pl.ds(2 * dm, 4 * dm)],
                                     wmod.at[:, pl.ds(2 * dm, 4 * dm)], sem_misc.at[1])
    cp_x = pltpu.make_async_copy(x32, xs, sem_misc.at[2])
    cp_wo = pltpu.make_async_copy(wo_hbm.bitcast(U32), wo, sem_misc.at[3])

    def cp_stage(j):
        slot = j % N_STAGE
        return [pltpu.make_async_copy(qkv32[i].at[:, j, :], stage.at[slot, i], sem_stage.at[3 * slot + i])
                for i in range(3)]

    def cp_ffn(c):
        return [
            pltpu.make_async_copy(w1_hbm.bitcast(U32).at[:, pl.ds(pl.multiple_of(c * fc, fc), fc)], w1.at[c], sem_ffn.at[3 * c]),
            pltpu.make_async_copy(w3_hbm.bitcast(U32).at[:, pl.ds(pl.multiple_of(c * fc, fc), fc)], w3.at[c], sem_ffn.at[3 * c + 1]),
            pltpu.make_async_copy(w2_hbm.bitcast(U32).at[pl.ds(pl.multiple_of(c * (fc // 2), fc // 2), fc // 2), :], w2.at[c],
                                  sem_ffn.at[3 * c + 2]),
        ]

    def cp_out(b):
        r = pl.ds(pl.multiple_of(b * (blk // 2), blk // 2), blk // 2)
        return pltpu.make_async_copy(outs.at[r, :], out32.at[r, :], sem_out.at[b])

    cp_mod_a.start()
    cp_x.start()
    for j in range(N_STAGE):
        for cp in cp_stage(j):
            cp.start()

    cf = c_ref[...].astype(F32)
    sc = jnp.broadcast_to(_round(cf * jax.nn.sigmoid(cf)), (8, dm))

    def set_mod(k, plus_one):
        m = _dot(sc, _bf(wmod[:, k * dm:(k + 1) * dm]))
        mod[k] = m + 1.0 if plus_one else m

    def get_mod(k, n):
        return jnp.concatenate([mod[k]] * (n // 8), axis=0)

    def seg_x(s):
        return _bf(xs[pl.ds(pl.multiple_of(s * hseg, hseg), hseg), :]).astype(F32)

    def seg_h(s):
        return _round(_mod_ln(seg_x(s), get_mod(1, seg), get_mod(0, seg)))

    cp_mod_a.wait()
    set_mod(0, False)
    set_mod(1, True)
    cp_x.wait()
    lhs[0:n_mem, :] = mem0_ref[...].astype(F32)
    lhs[n_mem:rows, :] = seg_h(0)

    def pre_rows(i, _):
        t = jnp.concatenate([seg_x(2 * i)[seg - PRE_ROWS:], seg_x(2 * i + 1)[seg - PRE_ROWS:]], axis=0)
        hpre[pl.ds(pl.multiple_of(i * PRE_ROWS, PRE_ROWS), PRE_ROWS), :] = _words(
            _mod_ln(t, get_mod(1, 2 * PRE_ROWS), get_mod(0, 2 * PRE_ROWS)))

    jax.lax.fori_loop(0, n_seg // 2, pre_rows, None, unroll=8)

    def relayout(j):
        for i, cp in enumerate(cp_stage(j)):
            cp.wait()
            w = stage[j % N_STAGE, i]
            wqkv[j, :, 2 * i * dh:(2 * i + 1) * dh] = _words(pltpu.bitcast(w << 16, F32))
            wqkv[j, :, (2 * i + 1) * dh:(2 * i + 2) * dh] = _words(
                pltpu.bitcast(w & jnp.uint32(0xFFFF0000), F32))

        @pl.when(j + N_STAGE < n_pairs)
        def _():
            for cp in cp_stage(j + N_STAGE):
                cp.start()

        @pl.when(j + N_STAGE == n_pairs)
        def _():
            cp_wo.start()

        @pl.when(j == n_pairs - 2)
        def _():
            cp_mod_b.start()

    def pre_proj(j, _):
        jax.lax.fori_loop(jnp.maximum(2 * j - 1, 0), jnp.minimum(2 * j + 1, n_pairs),
                          lambda i, _: relayout(i), None)
        pre[j] = _dot(_bf(hpre[...]), _bf(wqkv[j]))

    jax.lax.fori_loop(0, N_PRE, pre_proj, None)
    jax.lax.fori_loop(min(2 * N_PRE - 1, n_pairs), n_pairs, lambda i, _: relayout(i), None)
    for c in range(FFN_SEGS):
        for cp in cp_ffn(c):
            cp.start()

    def finish(s, attn):
        xn = seg_x(s) + get_mod(2, seg) * attn
        slot = (s // FFN_SEGS) % 2
        sub = s % FFN_SEGS
        x1[slot, pl.ds(pl.multiple_of(sub * seg, seg), seg), :] = xn
        h2[slot, pl.ds(pl.multiple_of(sub * hseg, hseg), hseg), :] = _words(
            _mod_ln(xn, get_mod(4, seg), get_mod(3, seg)))

    def step(s, do_attn, do_ffn):
        if do_ffn:
            fs = s - FFN_SEGS
            fb = fs // FFN_SEGS
            fch = fs % FFN_SEGS
            fslot = fb % 2

            @pl.when(fs < FFN_SEGS)
            def _():
                for cp in cp_ffn(fch):
                    cp.wait()

            hb = _bf(h2[fslot])
            acts = []

        def ffn_up(lo, hi):
            if do_ffn:
                g = _dot(hb, _bf(w1[fch, :, lo:hi]))
                u = _dot(hb, _bf(w3[fch, :, lo:hi]))
                acts.append((g * jax.nn.sigmoid(g) * u).astype(BF16))

        def ffn_down():
            if do_ffn:
                y = _dot(jnp.concatenate(acts, axis=1), _bf(w2[fch]))
                acc = x1[fslot] + get_mod(5, blk) * y
                x1[fslot] = acc
                outs[pl.ds(pl.multiple_of(fb * (blk // 2), blk // 2), blk // 2), :] = _words(acc)

        if not do_attn:
            ffn_up(0, fc)
            ffn_down()
        else:
            r = jax.lax.broadcasted_iota(jnp.int32, (2 * rows, 2 * rows), 0)
            q = jax.lax.broadcasted_iota(jnp.int32, (2 * rows, 2 * rows), 1)
            same = (r >= rows) == (q >= rows)
            rl = jnp.where(r >= rows, r - rows, r)
            ql = jnp.where(q >= rows, q - rows, q)
            keep = same & ((rl < n_mem) | (rl >= ql))
            fill = jnp.where(same, -1e9, -jnp.inf).astype(F32)
            a = lhs[...]
            a_short = a[:rows - PRE_ROWS].astype(BF16)
            qkv, probs = {}, {}

            def proj(j):
                if j < N_PRE:
                    t = jnp.concatenate(
                        [_dot(a_short, _bf(wqkv[j])),
                         pre[j, pl.ds(pl.multiple_of(s * PRE_ROWS, PRE_ROWS), PRE_ROWS), :]], axis=0)
                else:
                    t = _dot(a, _bf(wqkv[j]))
                qkv[j] = [jnp.concatenate([t[:, (2 * i) * dh:(2 * i + 1) * dh],
                                           t[:, (2 * i + 1) * dh:(2 * i + 2) * dh]], axis=0).astype(BF16)
                          for i in range(3)]

            def scores(j):
                t = jnp.where(keep, _dot_nt(qkv[j][0], qkv[j][1]) * scale, fill)
                e = jnp.exp(t - jnp.max(t, axis=-1, keepdims=True))
                probs[j] = (e / jnp.sum(e, axis=-1, keepdims=True)).astype(BF16)

            def mix(j):
                o = _round(_dot(probs[j], qkv[j][2]))
                obuf[:, 2 * j * dh:(2 * j + 1) * dh] = o[:rows]
                obuf[:, (2 * j + 1) * dh:(2 * j + 2) * dh] = o[rows:]

            def oproj(lo, hi):
                return _dot(obuf[:, lo * 2 * dh:hi * 2 * dh], _bf(wo[lo * dh:hi * dh, :]))

            order = list(range(n_pairs))
            for i, j in enumerate(order):
                proj(j)
                if i >= 1:
                    scores(order[i - 1])
                if i >= 2:
                    mix(order[i - 2])
            ffn_up(0, 384)
            scores(order[-1])
            mix(order[-2])
            ffn_up(384, fc)
            mix(order[-1])
            if not do_ffn:
                @pl.when(s == 0)
                def _():
                    cp_wo.wait()
            o = oproj(0, n_pairs)
            lhs[0:n_mem, :] = _round(o[:n_mem])
            lhs[n_mem:rows, :] = seg_h(jnp.minimum(s + 1, n_seg - 1))
            if do_ffn:
                finish(s, o[n_mem:])
            else:
                x1[0, pl.ds(pl.multiple_of(s * seg, seg), seg), :] = o[n_mem:]
            ffn_down()

        if do_ffn:
            @pl.when(fch == FFN_SEGS - 1)
            def _():
                cp_out(fb).start()

    def run(lo, hi, do_attn, do_ffn):
        jax.lax.fori_loop(lo, hi, lambda s, _: step(s, do_attn, do_ffn), None)

    run(0, FFN_SEGS, True, False)
    cp_mod_b.wait()
    for k in range(2, 6):
        set_mod(k, k == 4)
    for s in range(FFN_SEGS):
        finish(s, x1[0, s * seg:(s + 1) * seg, :])
    run(FFN_SEGS, n_seg, True, True)
    run(n_seg, n_seg + FFN_SEGS, False, True)
    for b in range(n_blk):
        cp_out(b).wait()


@functools.partial(jax.jit, static_argnames=("A_seg_len",))
def pallas_adaLN_cond__memory_aug_recurrent_mem_tr__glu_gated_swiglu__prompt_kernel(
    A_x, A_mem0, A_Wq, A_Wk, A_Wv, A_Wo, A_seg_len, B_x, B_w1, B_w3, B_w2, c, w_mod,
):
    del B_x
    bsz, s_len, dm = A_x.shape
    _, n_heads, dh = A_Wq.shape
    n_mem = A_mem0.shape[1]
    seg = int(A_seg_len)
    f = B_w1.shape[1]
    fc = f // FFN_SEGS
    blk = FFN_SEGS * seg
    assert bsz == 1 and s_len % blk == 0 and n_heads % 4 == 0 and fc % 128 == 0

    hbm = pl.BlockSpec(memory_space=pltpu.MemorySpace.HBM)
    vmem = pl.BlockSpec(memory_space=pltpu.MemorySpace.VMEM)
    out = pl.pallas_call(
        functools.partial(_kernel, seg=seg, n_mem=n_mem, dh=dh),
        out_shape=jax.ShapeDtypeStruct((s_len, dm), A_x.dtype),
        in_specs=[vmem, vmem] + [hbm] * 9,
        out_specs=hbm,
        scratch_shapes=[
            pltpu.VMEM((n_heads // 2, dm // 2, 6 * dh), U32),
            pltpu.VMEM((n_heads * dh // 2, dm), U32),
            pltpu.VMEM((FFN_SEGS, dm // 2, fc), U32),
            pltpu.VMEM((FFN_SEGS, dm // 2, fc), U32),
            pltpu.VMEM((FFN_SEGS, fc // 2, dm), U32),
            pltpu.VMEM((dm // 2, 6 * dm), U32),
            pltpu.VMEM((N_STAGE, 3, dm, dh), U32),
            pltpu.VMEM((s_len // 2, dm), U32),
            pltpu.VMEM((s_len // 2, dm), U32),
            pltpu.VMEM((6, 8, dm), F32),
            pltpu.VMEM((n_mem + seg, dm), F32),
            pltpu.VMEM((n_mem + seg, n_heads * dh), F32),
            pltpu.VMEM((2, blk, dm), F32),
            pltpu.VMEM((2, blk // 2, dm), U32),
            pltpu.VMEM((s_len // seg * PRE_ROWS // 2, dm), U32),
            pltpu.VMEM((N_PRE, s_len // seg * PRE_ROWS, 6 * dh), F32),
            pltpu.SemaphoreType.DMA((3 * N_STAGE,)),
            pltpu.SemaphoreType.DMA((4,)),
            pltpu.SemaphoreType.DMA((3 * FFN_SEGS,)),
            pltpu.SemaphoreType.DMA((s_len // blk,)),
        ],
        compiler_params=pltpu.CompilerParams(vmem_limit_bytes=120 * 2**20),
    )(c, A_mem0.reshape(n_mem, dm), A_x.reshape(s_len, dm), A_Wq, A_Wk, A_Wv,
      A_Wo.reshape(n_heads * dh, dm), B_w1, B_w3, B_w2, w_mod)
    return out.reshape(bsz, s_len, dm)
```

```python
import functools

import jax
import jax.numpy as jnp
import jax.experimental.pallas as pl
import jax.experimental.pallas.tpu as pltpu

U32 = jnp.uint32
BF16 = jnp.bfloat16
F32 = jnp.float32
LN_EPS = 1e-5
FFN_SEGS = 4
N_STAGE = 4
N_PRE = 8
PRE_ROWS = 8
DOWN_COLS = 128


def _bf(w):
    return pltpu.bitcast(w, BF16)


def _words(a):
    return pltpu.bitcast(a.astype(BF16), U32)


def _dot(a, b):
    return jax.lax.dot_general(a, b, (((1,), (0,)), ((), ())), preferred_element_type=F32)


def _dot_nt(a, b):
    return jax.lax.dot_general(a, b, (((1,), (1,)), ((), ())), preferred_element_type=F32)


def _round(a):
    return a.astype(BF16).astype(F32)


def _mod_ln(x, scale1, shift):
    m = jnp.mean(x, axis=-1, keepdims=True)
    d = x - m
    v = jnp.mean(d * d, axis=-1, keepdims=True)
    return d * jax.lax.rsqrt(v + LN_EPS) * scale1 + shift


def _strassen_lhs(a11, a12, a21, a22):
    return [a11 + a22, a21 + a22, a11, a22, a11 + a12, a21 - a11, a12 - a22]


def _strassen_out(m):
    return m[0] + m[3] - m[4] + m[6], m[2] + m[4], m[1] + m[3], m[0] - m[1] + m[2] + m[5]


RAW_SLOTS = (1, 2, 3, 4)


def _strassen_rhs(w, c, r, n):
    b11, b12, b21, b22 = [_bf(w[c, i, pl.ds(r, n), :]).astype(F32) for i in RAW_SLOTS]
    for i, t in ((0, b11 + b22), (2, b12 - b22), (3, b21 - b11), (5, b11 + b12), (6, b21 + b22)):
        w[c, i, pl.ds(r, n), :] = _words(t)


def _kernel(c_ref, mem0_ref, x_hbm, wq_hbm, wk_hbm, wv_hbm, wo_hbm, w1_hbm, w3_hbm, w2_hbm,
            wmod_hbm, out_hbm,
            wqkv, wo, wup, wdn, wrest, wmod, stage, xs, outs, mod, lhs, obuf, x1, h2, hpre, pre,
            sem_stage, sem_misc, sem_ffn, sem_out, *, seg, n_mem, dh):
    n_pairs = wqkv.shape[0]
    dm = lhs.shape[1]
    rows = n_mem + seg
    hseg = seg // 2
    n_seg = xs.shape[0] // hseg
    n_blk = n_seg // FFN_SEGS
    blk = FFN_SEGS * seg
    fc = wup.shape[3]
    kd = 2 * wdn.shape[2]
    hd = dm // 2
    scale = dh ** -0.5

    wmod32 = wmod_hbm.bitcast(U32)
    x32 = x_hbm.bitcast(U32)
    out32 = out_hbm.bitcast(U32)
    qkv32 = [w.bitcast(U32) for w in (wq_hbm, wk_hbm, wv_hbm)]
    cp_mod_a = pltpu.make_async_copy(wmod32.at[:, pl.ds(0, 2 * dm)], wmod.at[:, pl.ds(0, 2 * dm)],
                                     sem_misc.at[0])
    cp_mod_b = pltpu.make_async_copy(wmod32.at[:, pl.ds(2 * dm, 4 * dm)],
                                     wmod.at[:, pl.ds(2 * dm, 4 * dm)], sem_misc.at[1])
    cp_x = pltpu.make_async_copy(x32, xs, sem_misc.at[2])
    cp_wo = pltpu.make_async_copy(wo_hbm.bitcast(U32), wo, sem_misc.at[3])

    def cp_stage(j):
        slot = j % N_STAGE
        return [pltpu.make_async_copy(qkv32[i].at[:, j, :], stage.at[slot, i], sem_stage.at[3 * slot + i])
                for i in range(3)]

    def cp_ffn(c):
        cols = pl.ds(pl.multiple_of(c * fc, fc), fc)
        w1_32, w3_32, w2_32 = w1_hbm.bitcast(U32), w3_hbm.bitcast(U32), w2_hbm.bitcast(U32)

        def w2_rows(off, n):
            return pl.ds(pl.multiple_of(c * (fc // 2) + off, 64), n)

        pairs = []
        for i, slot in enumerate(RAW_SLOTS):
            pairs.append(((w1_32, w3_32)[i % 2].at[pl.ds(i // 2 * (hd // 2), hd // 2), cols], wup.at[c, slot]))
            pairs.append((w2_32.at[w2_rows(i // 2 * (kd // 2), kd // 2), pl.ds(i % 2 * hd, hd)], wdn.at[c, slot]))
        pairs.append((w2_32.at[w2_rows(kd, fc // 2 - kd), :], wrest.at[c]))
        return [pltpu.make_async_copy(src, dst, sem_ffn.at[9 * c + i]) for i, (src, dst) in enumerate(pairs)]

    def cp_out(b):
        r = pl.ds(pl.multiple_of(b * (blk // 2), blk // 2), blk // 2)
        return pltpu.make_async_copy(outs.at[r, :], out32.at[r, :], sem_out.at[b])

    cp_mod_a.start()
    cp_x.start()
    for j in range(N_STAGE):
        for cp in cp_stage(j):
            cp.start()

    cf = c_ref[...].astype(F32)
    sc = jnp.broadcast_to(_round(cf * jax.nn.sigmoid(cf)), (8, dm))

    def set_mod(k, plus_one):
        m = _dot(sc, _bf(wmod[:, k * dm:(k + 1) * dm]))
        mod[k] = m + 1.0 if plus_one else m

    def get_mod(k, n):
        return jnp.concatenate([mod[k]] * (n // 8), axis=0)

    def seg_x(s):
        return _bf(xs[pl.ds(pl.multiple_of(s * hseg, hseg), hseg), :]).astype(F32)

    def seg_h(s):
        return _round(_mod_ln(seg_x(s), get_mod(1, seg), get_mod(0, seg)))

    cp_mod_a.wait()
    set_mod(0, False)
    set_mod(1, True)
    cp_x.wait()
    lhs[0:n_mem, :] = mem0_ref[...].astype(F32)
    lhs[n_mem:rows, :] = seg_h(0)

    def pre_rows(i, _):
        t = jnp.concatenate([seg_x(2 * i)[seg - PRE_ROWS:], seg_x(2 * i + 1)[seg - PRE_ROWS:]], axis=0)
        hpre[pl.ds(pl.multiple_of(i * PRE_ROWS, PRE_ROWS), PRE_ROWS), :] = _words(
            _mod_ln(t, get_mod(1, 2 * PRE_ROWS), get_mod(0, 2 * PRE_ROWS)))

    jax.lax.fori_loop(0, n_seg // 2, pre_rows, None, unroll=8)

    def relayout(j):
        for i, cp in enumerate(cp_stage(j)):
            cp.wait()
            w = stage[j % N_STAGE, i]
            wqkv[j, :, 2 * i * dh:(2 * i + 1) * dh] = _words(pltpu.bitcast(w << 16, F32))
            wqkv[j, :, (2 * i + 1) * dh:(2 * i + 2) * dh] = _words(
                pltpu.bitcast(w & jnp.uint32(0xFFFF0000), F32))

        @pl.when(j + N_STAGE < n_pairs)
        def _():
            for cp in cp_stage(j + N_STAGE):
                cp.start()

        @pl.when(j + N_STAGE == n_pairs)
        def _():
            cp_wo.start()

        @pl.when(j == n_pairs - 2)
        def _():
            cp_mod_b.start()

    def pre_proj(j, _):
        jax.lax.fori_loop(jnp.maximum(2 * j - 1, 0), jnp.minimum(2 * j + 1, n_pairs),
                          lambda i, _: relayout(i), None)
        pre[j] = _dot(_bf(hpre[...]), _bf(wqkv[j]))

    jax.lax.fori_loop(0, N_PRE, pre_proj, None)
    jax.lax.fori_loop(min(2 * N_PRE - 1, n_pairs), n_pairs, lambda i, _: relayout(i), None)
    for c in range(FFN_SEGS):
        for cp in cp_ffn(c):
            cp.start()

    def finish(s, attn):
        xn = seg_x(s) + get_mod(2, seg) * attn
        slot = (s // FFN_SEGS) % 2
        sub = s % FFN_SEGS
        x1[slot, pl.ds(pl.multiple_of(sub * seg, seg), seg), :] = xn
        h = _mod_ln(xn, get_mod(4, seg), get_mod(3, seg))
        for i, t in enumerate(_strassen_lhs(h[:hseg, :hd], h[:hseg, hd:], h[hseg:, :hd], h[hseg:, hd:])):
            h2[slot, i, pl.ds(pl.multiple_of(sub * (hseg // 2), hseg // 2), hseg // 2), :] = _words(t)

    def step(s, do_attn, do_ffn):
        if do_ffn:
            fs = s - FFN_SEGS
            fb = fs // FFN_SEGS
            fch = fs % FFN_SEGS
            fslot = fb % 2

            @pl.when(fs < FFN_SEGS)
            def _():
                for cp in cp_ffn(fch):
                    cp.wait()
                jax.lax.fori_loop(0, hd // 32, lambda i, _: _strassen_rhs(
                    wup, fch, pl.multiple_of(i * 16, 16), 16), None)
                jax.lax.fori_loop(0, kd // 64, lambda i, _: _strassen_rhs(
                    wdn, fch, pl.multiple_of(i * 32, 32), 32), None)

            act_a, act_b = [], []

        def ffn_up(lo, hi):
            if do_ffn:
                for t in range(lo, hi, 128):
                    ga, ua, gb, ub = _strassen_out(
                        [_dot(_bf(h2[fslot, i]), _bf(wup[fch, i, :, t:t + 128])) for i in range(7)])
                    act_a.append(ga * jax.nn.sigmoid(ga) * ua)
                    act_b.append(gb * jax.nn.sigmoid(gb) * ub)

        def ffn_down():
            if do_ffn:
                aa, ab = jnp.concatenate(act_a, axis=1), jnp.concatenate(act_b, axis=1)
                ops = [t.astype(BF16) for t in _strassen_lhs(
                    aa[:, :kd], aa[:, kd:2 * kd], ab[:, :kd], ab[:, kd:2 * kd])]
                rest = _dot(jnp.concatenate([aa[:, 2 * kd:], ab[:, 2 * kd:]], axis=0).astype(BF16),
                            _bf(wrest[fch]))
                for t in range(0, hd, DOWN_COLS):
                    y = _strassen_out([_dot(ops[i], _bf(wdn[fch, i, :, t:t + DOWN_COLS])) for i in range(7)])
                    for side in range(2):
                        cols = slice(side * hd + t, side * hd + t + DOWN_COLS)
                        ya = y[side] + rest[:blk // 2, cols]
                        yb = y[2 + side] + rest[blk // 2:, cols]
                        yy = jnp.concatenate([v[k * hseg:(k + 1) * hseg] for k in range(FFN_SEGS)
                                              for v in (ya, yb)], axis=0)
                        acc = x1[fslot, :, cols] + get_mod(5, blk)[:, cols] * yy
                        x1[fslot, :, cols] = acc
                        outs[pl.ds(pl.multiple_of(fb * (blk // 2), blk // 2), blk // 2), cols] = _words(acc)

        if not do_attn:
            ffn_up(0, fc)
            ffn_down()
        else:
            r = jax.lax.broadcasted_iota(jnp.int32, (2 * rows, 2 * rows), 0)
            q = jax.lax.broadcasted_iota(jnp.int32, (2 * rows, 2 * rows), 1)
            same = (r >= rows) == (q >= rows)
            rl = jnp.where(r >= rows, r - rows, r)
            ql = jnp.where(q >= rows, q - rows, q)
            keep = same & ((rl < n_mem) | (rl >= ql))
            fill = jnp.where(same, -1e9, -jnp.inf).astype(F32)
            a = lhs[...]
            a_short = a[:rows - PRE_ROWS].astype(BF16)
            qkv, probs = {}, {}

            def proj(j):
                if j < N_PRE:
                    t = jnp.concatenate(
                        [_dot(a_short, _bf(wqkv[j])),
                         pre[j, pl.ds(pl.multiple_of(s * PRE_ROWS, PRE_ROWS), PRE_ROWS), :]], axis=0)
                else:
                    t = _dot(a, _bf(wqkv[j]))
                qkv[j] = [jnp.concatenate([t[:, (2 * i) * dh:(2 * i + 1) * dh],
                                           t[:, (2 * i + 1) * dh:(2 * i + 2) * dh]], axis=0).astype(BF16)
                          for i in range(3)]

            def scores(j):
                t = jnp.where(keep, _dot_nt(qkv[j][0], qkv[j][1]) * scale, fill)
                e = jnp.exp(t - jnp.max(t, axis=-1, keepdims=True))
                probs[j] = (e / jnp.sum(e, axis=-1, keepdims=True)).astype(BF16)

            def mix(j):
                o = _round(_dot(probs[j], qkv[j][2]))
                obuf[:, 2 * j * dh:(2 * j + 1) * dh] = o[:rows]
                obuf[:, (2 * j + 1) * dh:(2 * j + 2) * dh] = o[rows:]

            def oproj(lo, hi):
                return _dot(obuf[:, lo * 2 * dh:hi * 2 * dh], _bf(wo[lo * dh:hi * dh, :]))

            order = list(range(n_pairs))
            for i, j in enumerate(order):
                proj(j)
                if i >= 1:
                    scores(order[i - 1])
                if i >= 2:
                    mix(order[i - 2])
            ffn_up(0, 384)
            scores(order[-1])
            mix(order[-2])
            ffn_up(384, fc)
            mix(order[-1])
            if not do_ffn:
                @pl.when(s == 0)
                def _():
                    cp_wo.wait()
            o = oproj(0, n_pairs)
            lhs[0:n_mem, :] = _round(o[:n_mem])
            lhs[n_mem:rows, :] = seg_h(jnp.minimum(s + 1, n_seg - 1))
            if do_ffn:
                finish(s, o[n_mem:])
            else:
                x1[0, pl.ds(pl.multiple_of(s * seg, seg), seg), :] = o[n_mem:]
            ffn_down()

        if do_ffn:
            @pl.when(fch == FFN_SEGS - 1)
            def _():
                cp_out(fb).start()

    def run(lo, hi, do_attn, do_ffn):
        jax.lax.fori_loop(lo, hi, lambda s, _: step(s, do_attn, do_ffn), None)

    run(0, FFN_SEGS, True, False)
    cp_mod_b.wait()
    for k in range(2, 6):
        set_mod(k, k == 4)
    for s in range(FFN_SEGS):
        finish(s, x1[0, s * seg:(s + 1) * seg, :])
    run(FFN_SEGS, n_seg, True, True)
    run(n_seg, n_seg + FFN_SEGS, False, True)
    for b in range(n_blk):
        cp_out(b).wait()


@functools.partial(jax.jit, static_argnames=("A_seg_len",))
def pallas_adaLN_cond__memory_aug_recurrent_mem_tr__glu_gated_swiglu__prompt_kernel(
    A_x, A_mem0, A_Wq, A_Wk, A_Wv, A_Wo, A_seg_len, B_x, B_w1, B_w3, B_w2, c, w_mod,
):
    del B_x
    bsz, s_len, dm = A_x.shape
    _, n_heads, dh = A_Wq.shape
    n_mem = A_mem0.shape[1]
    seg = int(A_seg_len)
    f = B_w1.shape[1]
    fc = f // FFN_SEGS
    kd = (fc - 1) // 256 * 128
    blk = FFN_SEGS * seg
    assert bsz == 1 and s_len % blk == 0 and n_heads % 4 == 0 and fc % 128 == 0

    hbm = pl.BlockSpec(memory_space=pltpu.MemorySpace.HBM)
    vmem = pl.BlockSpec(memory_space=pltpu.MemorySpace.VMEM)
    out = pl.pallas_call(
        functools.partial(_kernel, seg=seg, n_mem=n_mem, dh=dh),
        out_shape=jax.ShapeDtypeStruct((s_len, dm), A_x.dtype),
        in_specs=[vmem, vmem] + [hbm] * 9,
        out_specs=hbm,
        scratch_shapes=[
            pltpu.VMEM((n_heads // 2, dm // 2, 6 * dh), U32),
            pltpu.VMEM((n_heads * dh // 2, dm), U32),
            pltpu.VMEM((FFN_SEGS, 7, dm // 4, fc), U32),
            pltpu.VMEM((FFN_SEGS, 7, kd // 2, dm // 2), U32),
            pltpu.VMEM((FFN_SEGS, fc // 2 - kd, dm), U32),
            pltpu.VMEM((dm // 2, 6 * dm), U32),
            pltpu.VMEM((N_STAGE, 3, dm, dh), U32),
            pltpu.VMEM((s_len // 2, dm), U32),
            pltpu.VMEM((s_len // 2, dm), U32),
            pltpu.VMEM((6, 8, dm), F32),
            pltpu.VMEM((n_mem + seg, dm), F32),
            pltpu.VMEM((n_mem + seg, n_heads * dh), F32),
            pltpu.VMEM((2, blk, dm), F32),
            pltpu.VMEM((2, 7, blk // 4, dm // 2), U32),
            pltpu.VMEM((s_len // seg * PRE_ROWS // 2, dm), U32),
            pltpu.VMEM((N_PRE, s_len // seg * PRE_ROWS, 6 * dh), F32),
            pltpu.SemaphoreType.DMA((3 * N_STAGE,)),
            pltpu.SemaphoreType.DMA((4,)),
            pltpu.SemaphoreType.DMA((9 * FFN_SEGS,)),
            pltpu.SemaphoreType.DMA((s_len // blk,)),
        ],
        compiler_params=pltpu.CompilerParams(vmem_limit_bytes=124 * 2**20),
    )(c, A_mem0.reshape(n_mem, dm), A_x.reshape(s_len, dm), A_Wq, A_Wk, A_Wv,
      A_Wo.reshape(n_heads * dh, dm), B_w1, B_w3, B_w2, w_mod)
    return out.reshape(bsz, s_len, dm)
```

```python
import functools

import jax
import jax.numpy as jnp
import jax.experimental.pallas as pl
import jax.experimental.pallas.tpu as pltpu

U32 = jnp.uint32
BF16 = jnp.bfloat16
F32 = jnp.float32
LN_EPS = 1e-5
FFN_SEGS = 4
N_STAGE = 4
N_PRE = 8
PRE_ROWS = 8
DOWN_COLS = 128
CMB = 32


def _bf(w):
    return pltpu.bitcast(w, BF16)


def _words(a):
    return pltpu.bitcast(a.astype(BF16), U32)


def _dot(a, b):
    return jax.lax.dot_general(a, b, (((1,), (0,)), ((), ())), preferred_element_type=F32)


def _dot_nt(a, b):
    return jax.lax.dot_general(a, b, (((1,), (1,)), ((), ())), preferred_element_type=F32)


def _round(a):
    return a.astype(BF16).astype(F32)


def _mod_ln(x, scale1, shift):
    m = jnp.mean(x, axis=-1, keepdims=True)
    d = x - m
    v = jnp.mean(d * d, axis=-1, keepdims=True)
    return d * jax.lax.rsqrt(v + LN_EPS) * scale1 + shift


def _strassen_lhs(a11, a12, a21, a22):
    return [a11 + a22, a21 + a22, a11, a22, a11 + a12, a21 - a11, a12 - a22]


def _strassen_out(m):
    return m[0] + m[3] - m[4] + m[6], m[2] + m[4], m[1] + m[3], m[0] - m[1] + m[2] + m[5]


RAW_SLOTS = (1, 2, 3, 4)


def _strassen_rhs(w, c, r, n):
    for k in range(0, w.shape[3], 128):
        at = (pl.ds(r, n), slice(k, k + 128))
        b11, b12, b21, b22 = [_bf(w[(c, i) + at]).astype(F32) for i in RAW_SLOTS]
        for i, t in ((0, b11 + b22), (2, b12 - b22), (3, b21 - b11), (5, b11 + b12), (6, b21 + b22)):
            w[(c, i) + at] = _words(t)


def _kernel(c_ref, mem0_ref, x_hbm, wq_hbm, wk_hbm, wv_hbm, wo_hbm, w1_hbm, w3_hbm, w2_hbm,
            wmod_hbm, out_hbm,
            wqkv, wo, wup, wdn, wrest, wmod, stage, xs, outs, mod, lhs, obuf, x1, h2, hpre, pre,
            sem_stage, sem_misc, sem_ffn, sem_out, *, seg, n_mem, dh):
    n_pairs = wqkv.shape[0]
    dm = lhs.shape[1]
    rows = n_mem + seg
    hseg = seg // 2
    n_seg = xs.shape[0] // hseg
    n_blk = n_seg // FFN_SEGS
    blk = FFN_SEGS * seg
    fc = wup.shape[3]
    kd = 2 * wdn.shape[2]
    hd = dm // 2
    scale = dh ** -0.5

    wmod32 = wmod_hbm.bitcast(U32)
    x32 = x_hbm.bitcast(U32)
    out32 = out_hbm.bitcast(U32)
    qkv32 = [w.bitcast(U32) for w in (wq_hbm, wk_hbm, wv_hbm)]
    cp_mod_a = pltpu.make_async_copy(wmod32.at[:, pl.ds(0, 2 * dm)], wmod.at[:, pl.ds(0, 2 * dm)],
                                     sem_misc.at[0])
    cp_mod_b = pltpu.make_async_copy(wmod32.at[:, pl.ds(2 * dm, 4 * dm)],
                                     wmod.at[:, pl.ds(2 * dm, 4 * dm)], sem_misc.at[1])
    cp_x = pltpu.make_async_copy(x32, xs, sem_misc.at[2])
    cp_wo = pltpu.make_async_copy(wo_hbm.bitcast(U32), wo, sem_misc.at[3])

    def cp_stage(j):
        slot = j % N_STAGE
        return [pltpu.make_async_copy(qkv32[i].at[:, j, :], stage.at[slot, i], sem_stage.at[3 * slot + i])
                for i in range(3)]

    def cp_ffn(c):
        cols = pl.ds(pl.multiple_of(c * fc, fc), fc)
        w1_32, w3_32, w2_32 = w1_hbm.bitcast(U32), w3_hbm.bitcast(U32), w2_hbm.bitcast(U32)

        def w2_rows(off, n):
            return pl.ds(pl.multiple_of(c * (fc // 2) + off, 64), n)

        pairs = []
        for i, slot in enumerate(RAW_SLOTS):
            pairs.append(((w1_32, w3_32)[i % 2].at[pl.ds(i // 2 * (hd // 2), hd // 2), cols], wup.at[c, slot]))
            pairs.append((w2_32.at[w2_rows(i // 2 * (kd // 2), kd // 2), pl.ds(i % 2 * hd, hd)], wdn.at[c, slot]))
        pairs.append((w2_32.at[w2_rows(kd, fc // 2 - kd), :], wrest.at[c]))
        return [pltpu.make_async_copy(src, dst, sem_ffn.at[9 * c + i]) for i, (src, dst) in enumerate(pairs)]

    def cp_out(b):
        r = pl.ds(pl.multiple_of(b * (blk // 2), blk // 2), blk // 2)
        return pltpu.make_async_copy(outs.at[r, :], out32.at[r, :], sem_out.at[b])

    cp_mod_a.start()
    cp_x.start()
    for j in range(N_STAGE):
        for cp in cp_stage(j):
            cp.start()

    cf = c_ref[...].astype(F32)
    sc = jnp.broadcast_to(_round(cf * jax.nn.sigmoid(cf)), (8, dm))

    def set_mod(k, plus_one):
        m = _dot(sc, _bf(wmod[:, k * dm:(k + 1) * dm]))
        mod[k] = m + 1.0 if plus_one else m

    def get_mod(k, n):
        return jnp.concatenate([mod[k]] * (n // 8), axis=0)

    def seg_x(s):
        return _bf(xs[pl.ds(pl.multiple_of(s * hseg, hseg), hseg), :]).astype(F32)

    def seg_h(s):
        return _round(_mod_ln(seg_x(s), get_mod(1, seg), get_mod(0, seg)))

    cp_mod_a.wait()
    set_mod(0, False)
    set_mod(1, True)
    cp_x.wait()
    lhs[0:n_mem, :] = mem0_ref[...].astype(F32)
    lhs[n_mem:rows, :] = seg_h(0)

    def pre_rows(i, _):
        t = jnp.concatenate([seg_x(2 * i)[seg - PRE_ROWS:], seg_x(2 * i + 1)[seg - PRE_ROWS:]], axis=0)
        hpre[pl.ds(pl.multiple_of(i * PRE_ROWS, PRE_ROWS), PRE_ROWS), :] = _words(
            _mod_ln(t, get_mod(1, 2 * PRE_ROWS), get_mod(0, 2 * PRE_ROWS)))

    jax.lax.fori_loop(0, n_seg // 2, pre_rows, None, unroll=8)

    def relayout(j):
        for cp in cp_stage(j):
            cp.wait()

        def rows64(t, _):
            r = pl.multiple_of(t * 64, 64)
            for i in range(3):
                even, odd = [stage[j % N_STAGE, i, pl.ds(2 * r + k, 64, stride=2), :] for k in range(2)]
                wqkv[j, pl.ds(r, 64), 2 * i * dh:(2 * i + 1) * dh] = (even & jnp.uint32(0xFFFF)) | (odd << 16)
                wqkv[j, pl.ds(r, 64), (2 * i + 1) * dh:(2 * i + 2) * dh] = (
                    (even >> 16) | (odd & jnp.uint32(0xFFFF0000)))

        jax.lax.fori_loop(0, dm // 128, rows64, None)

        @pl.when(j + N_STAGE < n_pairs)
        def _():
            for cp in cp_stage(j + N_STAGE):
                cp.start()

        @pl.when(j + N_STAGE == n_pairs)
        def _():
            cp_wo.start()

        @pl.when(j == n_pairs - 2)
        def _():
            cp_mod_b.start()

    def pre_proj(j, _):
        jax.lax.fori_loop(jnp.maximum(2 * j - 1, 0), jnp.minimum(2 * j + 1, n_pairs),
                          lambda i, _: relayout(i), None)
        pre[j] = _dot(_bf(hpre[...]), _bf(wqkv[j]))

    jax.lax.fori_loop(0, N_PRE, pre_proj, None)
    jax.lax.fori_loop(min(2 * N_PRE - 1, n_pairs), n_pairs, lambda i, _: relayout(i), None)
    for c in range(FFN_SEGS):
        for cp in cp_ffn(c):
            cp.start()

    def finish(s, attn):
        xn = seg_x(s) + get_mod(2, seg) * attn
        slot = (s // FFN_SEGS) % 2
        sub = s % FFN_SEGS
        x1[slot, pl.ds(pl.multiple_of(sub * seg, seg), seg), :] = xn
        h = _mod_ln(xn, get_mod(4, seg), get_mod(3, seg))
        for i, t in enumerate(_strassen_lhs(h[:hseg, :hd], h[:hseg, hd:], h[hseg:, :hd], h[hseg:, hd:])):
            h2[slot, i, pl.ds(pl.multiple_of(sub * (hseg // 2), hseg // 2), hseg // 2), :] = _words(t)

    def step(s, phase):
        do_attn = phase != "ffn"
        do_ffn = phase in ("both", "ffn")
        if do_ffn:
            fb = s // FFN_SEGS - 1
            fch = s % FFN_SEGS
            fslot = fb % 2
            act_a, act_b = [], []
        if phase == "both":
            @pl.when(fb == 0)
            def _():
                for cp in cp_ffn(fch):
                    cp.wait()
                jax.lax.fori_loop(0, hd // 2 // CMB, lambda i, _: _strassen_rhs(
                    wup, fch, pl.multiple_of(i * CMB, CMB), CMB), None)
                jax.lax.fori_loop(0, kd // 2 // CMB, lambda i, _: _strassen_rhs(
                    wdn, fch, pl.multiple_of(i * CMB, CMB), CMB), None)

        def ffn_up(lo, hi):
            if do_ffn:
                for t in range(lo, hi, 128):
                    ga, ua, gb, ub = _strassen_out(
                        [_dot(_bf(h2[fslot, i]), _bf(wup[fch, i, :, t:t + 128])) for i in range(7)])
                    act_a.append(ga * jax.nn.sigmoid(ga) * ua)
                    act_b.append(gb * jax.nn.sigmoid(gb) * ub)

        def ffn_down():
            if do_ffn:
                aa, ab = jnp.concatenate(act_a, axis=1), jnp.concatenate(act_b, axis=1)
                ops = [t.astype(BF16) for t in _strassen_lhs(
                    aa[:, :kd], aa[:, kd:2 * kd], ab[:, :kd], ab[:, kd:2 * kd])]
                rest = _dot(jnp.concatenate([aa[:, 2 * kd:], ab[:, 2 * kd:]], axis=0).astype(BF16),
                            _bf(wrest[fch]))
                for t in range(0, hd, DOWN_COLS):
                    y = _strassen_out([_dot(ops[i], _bf(wdn[fch, i, :, t:t + DOWN_COLS])) for i in range(7)])
                    for side in range(2):
                        cols = slice(side * hd + t, side * hd + t + DOWN_COLS)
                        ya = y[side] + rest[:blk // 2, cols]
                        yb = y[2 + side] + rest[blk // 2:, cols]
                        yy = jnp.concatenate([v[k * hseg:(k + 1) * hseg] for k in range(FFN_SEGS)
                                              for v in (ya, yb)], axis=0)
                        acc = x1[fslot, :, cols] + get_mod(5, blk)[:, cols] * yy
                        x1[fslot, :, cols] = acc
                        outs[pl.ds(pl.multiple_of(fb * (blk // 2), blk // 2), blk // 2), cols] = _words(acc)

        if not do_attn:
            ffn_up(0, fc)
            ffn_down()
        else:
            r = jax.lax.broadcasted_iota(jnp.int32, (2 * rows, 2 * rows), 0)
            q = jax.lax.broadcasted_iota(jnp.int32, (2 * rows, 2 * rows), 1)
            same = (r >= rows) == (q >= rows)
            rl = jnp.where(r >= rows, r - rows, r)
            ql = jnp.where(q >= rows, q - rows, q)
            keep = same & ((rl < n_mem) | (rl >= ql))
            fill = jnp.where(same, -1e9, -jnp.inf).astype(F32)
            a = lhs[...]
            a_short = a[:rows - PRE_ROWS].astype(BF16)
            qkv, probs = {}, {}

            def proj(j):
                if j < N_PRE:
                    t = jnp.concatenate(
                        [_dot(a_short, _bf(wqkv[j])),
                         pre[j, pl.ds(pl.multiple_of(s * PRE_ROWS, PRE_ROWS), PRE_ROWS), :]], axis=0)
                else:
                    t = _dot(a, _bf(wqkv[j]))
                qkv[j] = [jnp.concatenate([t[:, (2 * i) * dh:(2 * i + 1) * dh],
                                           t[:, (2 * i + 1) * dh:(2 * i + 2) * dh]], axis=0).astype(BF16)
                          for i in range(3)]

            def scores(j):
                t = jnp.where(keep, _dot_nt(qkv[j][0], qkv[j][1]) * scale, fill)
                e = jnp.exp(t - jnp.max(t, axis=-1, keepdims=True))
                probs[j] = (e / jnp.sum(e, axis=-1, keepdims=True)).astype(BF16)

            def mix(j):
                o = _round(_dot(probs[j], qkv[j][2]))
                obuf[:, 2 * j * dh:(2 * j + 1) * dh] = o[:rows]
                obuf[:, (2 * j + 1) * dh:(2 * j + 2) * dh] = o[rows:]

            def oproj(lo, hi):
                return _dot(obuf[:, lo * 2 * dh:hi * 2 * dh], _bf(wo[lo * dh:hi * dh, :]))

            order = list(range(n_pairs))
            for i, j in enumerate(order):
                proj(j)
                if i >= 1:
                    scores(order[i - 1])
                if i >= 2:
                    mix(order[i - 2])
            ffn_up(0, 384)
            scores(order[-1])
            mix(order[-2])
            ffn_up(384, fc)
            mix(order[-1])
            if phase == "first":
                @pl.when(s == 0)
                def _():
                    cp_wo.wait()
            o = oproj(0, n_pairs)
            lhs[0:n_mem, :] = _round(o[:n_mem])
            lhs[n_mem:rows, :] = seg_h(jnp.minimum(s + 1, n_seg - 1))
            if phase != "first":
                finish(s, o[n_mem:])
            else:
                x1[0, pl.ds(pl.multiple_of(s * seg, seg), seg), :] = o[n_mem:]
            ffn_down()

        if do_ffn:
            @pl.when(fch == FFN_SEGS - 1)
            def _():
                cp_out(fb).start()

    def run(lo, hi, phase):
        jax.lax.fori_loop(lo, hi, lambda s, _: step(s, phase), None)

    run(0, FFN_SEGS, "first")
    cp_mod_b.wait()
    for k in range(2, 6):
        set_mod(k, k == 4)
    for s in range(FFN_SEGS):
        finish(s, x1[0, s * seg:(s + 1) * seg, :])
    run(FFN_SEGS, n_seg, "both")
    run(n_seg, n_seg + FFN_SEGS, "ffn")
    for b in range(n_blk):
        cp_out(b).wait()


@functools.partial(jax.jit, static_argnames=("A_seg_len",))
def pallas_adaLN_cond__memory_aug_recurrent_mem_tr__glu_gated_swiglu__prompt_kernel(
    A_x, A_mem0, A_Wq, A_Wk, A_Wv, A_Wo, A_seg_len, B_x, B_w1, B_w3, B_w2, c, w_mod,
):
    del B_x
    bsz, s_len, dm = A_x.shape
    _, n_heads, dh = A_Wq.shape
    n_mem = A_mem0.shape[1]
    seg = int(A_seg_len)
    f = B_w1.shape[1]
    fc = f // FFN_SEGS
    kd = (fc - 1) // 256 * 128
    blk = FFN_SEGS * seg
    assert bsz == 1 and s_len % blk == 0 and n_heads % 4 == 0 and fc % 128 == 0

    hbm = pl.BlockSpec(memory_space=pltpu.MemorySpace.HBM)
    vmem = pl.BlockSpec(memory_space=pltpu.MemorySpace.VMEM)
    out = pl.pallas_call(
        functools.partial(_kernel, seg=seg, n_mem=n_mem, dh=dh),
        out_shape=jax.ShapeDtypeStruct((s_len, dm), A_x.dtype),
        in_specs=[vmem, vmem] + [hbm] * 9,
        out_specs=hbm,
        scratch_shapes=[
            pltpu.VMEM((n_heads // 2, dm // 2, 6 * dh), U32),
            pltpu.VMEM((n_heads * dh // 2, dm), U32),
            pltpu.VMEM((FFN_SEGS, 7, dm // 4, fc), U32),
            pltpu.VMEM((FFN_SEGS, 7, kd // 2, dm // 2), U32),
            pltpu.VMEM((FFN_SEGS, fc // 2 - kd, dm), U32),
            pltpu.VMEM((dm // 2, 6 * dm), U32),
            pltpu.VMEM((N_STAGE, 3, dm, dh), U32),
            pltpu.VMEM((s_len // 2, dm), U32),
            pltpu.VMEM((s_len // 2, dm), U32),
            pltpu.VMEM((6, 8, dm), F32),
            pltpu.VMEM((n_mem + seg, dm), F32),
            pltpu.VMEM((n_mem + seg, n_heads * dh), F32),
            pltpu.VMEM((2, blk, dm), F32),
            pltpu.VMEM((2, 7, blk // 4, dm // 2), U32),
            pltpu.VMEM((s_len // seg * PRE_ROWS // 2, dm), U32),
            pltpu.VMEM((N_PRE, s_len // seg * PRE_ROWS, 6 * dh), F32),
            pltpu.SemaphoreType.DMA((3 * N_STAGE,)),
            pltpu.SemaphoreType.DMA((4,)),
            pltpu.SemaphoreType.DMA((9 * FFN_SEGS,)),
            pltpu.SemaphoreType.DMA((s_len // blk,)),
        ],
        compiler_params=pltpu.CompilerParams(vmem_limit_bytes=124 * 2**20),
    )(c, A_mem0.reshape(n_mem, dm), A_x.reshape(s_len, dm), A_Wq, A_Wk, A_Wv,
      A_Wo.reshape(n_heads * dh, dm), B_w1, B_w3, B_w2, w_mod)
    return out.reshape(bsz, s_len, dm)
```

```python
import functools

import jax
import jax.numpy as jnp
import jax.experimental.pallas as pl
import jax.experimental.pallas.tpu as pltpu

U32 = jnp.uint32
BF16 = jnp.bfloat16
F32 = jnp.float32
LN_EPS = 1e-5
FFN_SEGS = 4
N_STAGE = 5
N_PRE = 8
PRE_ROWS = 8
DOWN_COLS = 128
CMB = 32
X_HEAD = 8


def _bf(w):
    return pltpu.bitcast(w, BF16)


def _words(a):
    return pltpu.bitcast(a.astype(BF16), U32)


def _dot(a, b):
    return jax.lax.dot_general(a, b, (((1,), (0,)), ((), ())), preferred_element_type=F32)


def _dot_nt(a, b):
    return jax.lax.dot_general(a, b, (((1,), (1,)), ((), ())), preferred_element_type=F32)


def _round(a):
    return a.astype(BF16).astype(F32)


def _ln(x):
    m = jnp.mean(x, axis=-1, keepdims=True)
    d = x - m
    v = jnp.mean(d * d, axis=-1, keepdims=True)
    return d * jax.lax.rsqrt(v + LN_EPS)


def _mod_ln(x, scale1, shift):
    return _ln(x) * scale1 + shift


def _strassen_lhs(a11, a12, a21, a22):
    return [a11 + a22, a21 + a22, a11, a22, a11 + a12, a21 - a11, a12 - a22]


def _strassen_out(m):
    return m[0] + m[3] - m[4] + m[6], m[2] + m[4], m[1] + m[3], m[0] - m[1] + m[2] + m[5]


RAW_SLOTS = (1, 2, 3, 4)


def _strassen_rhs(w, c, r, n):
    for k in range(0, w.shape[3], 128):
        at = (pl.ds(r, n), slice(k, k + 128))
        b11, b12, b21, b22 = [_bf(w[(c, i) + at]).astype(F32) for i in RAW_SLOTS]
        for i, t in ((0, b11 + b22), (2, b12 - b22), (3, b21 - b11), (5, b11 + b12), (6, b21 + b22)):
            w[(c, i) + at] = _words(t)


def _kernel(c_ref, mem0_ref, x_hbm, wq_hbm, wk_hbm, wv_hbm, wo_hbm, w1_hbm, w3_hbm, w2_hbm,
            wmod_hbm, out_hbm,
            wqkv, wo, wup, wdn, wrest, wmod, stage, xs, outs, mod, lhs, obuf, x1, h2, xpre, npre, hpre, pre,
            sem_stage, sem_misc, sem_mod, sem_ffn, sem_out, *, seg, n_mem, dh):
    n_pairs = wqkv.shape[0]
    dm = lhs.shape[1]
    rows = n_mem + seg
    hseg = seg // 2
    n_seg = xs.shape[0]
    n_blk = n_seg // FFN_SEGS
    blk = FFN_SEGS * seg
    fc = wup.shape[3]
    kd = 2 * wdn.shape[2]
    hd = dm // 2
    scale = dh ** -0.5

    wmod32 = wmod_hbm.bitcast(U32)
    x32 = x_hbm.bitcast(U32)
    out32 = out_hbm.bitcast(U32)
    qkv32 = [w.bitcast(U32) for w in (wq_hbm, wk_hbm, wv_hbm)]
    hpr = PRE_ROWS // 2
    cp_xpre = pltpu.make_async_copy(x32.at[:, pl.ds(hseg - hpr, hpr), :], xpre.at[:, pl.ds(0, hpr), :],
                                    sem_misc.at[0])
    cp_x0 = pltpu.make_async_copy(x32.at[pl.ds(0, X_HEAD)], xs.at[pl.ds(0, X_HEAD)], sem_misc.at[1])
    cp_x1 = pltpu.make_async_copy(x32.at[pl.ds(X_HEAD, n_seg - X_HEAD)], xs.at[pl.ds(X_HEAD, n_seg - X_HEAD)],
                                  sem_misc.at[2])
    cp_wo = pltpu.make_async_copy(wo_hbm.bitcast(U32), wo, sem_misc.at[3])

    def cp_mod(k):
        return pltpu.make_async_copy(wmod32.at[:, pl.ds(pl.multiple_of(k * dm, dm), dm)], wmod.at[k],
                                     sem_mod.at[k])

    def cp_stage(j):
        slot = j % N_STAGE
        return [pltpu.make_async_copy(qkv32[i].at[:, j, :], stage.at[slot, i], sem_stage.at[3 * slot + i])
                for i in range(3)]

    def cp_ffn(c):
        cols = pl.ds(pl.multiple_of(c * fc, fc), fc)
        w1_32, w3_32, w2_32 = w1_hbm.bitcast(U32), w3_hbm.bitcast(U32), w2_hbm.bitcast(U32)

        def w2_rows(off, n):
            return pl.ds(pl.multiple_of(c * (fc // 2) + off, 64), n)

        pairs = []
        for i, slot in enumerate(RAW_SLOTS):
            pairs.append(((w1_32, w3_32)[i % 2].at[pl.ds(i // 2 * (hd // 2), hd // 2), cols], wup.at[c, slot]))
            pairs.append((w2_32.at[w2_rows(i // 2 * (kd // 2), kd // 2), pl.ds(i % 2 * hd, hd)], wdn.at[c, slot]))
        pairs.append((w2_32.at[w2_rows(kd, fc // 2 - kd), :], wrest.at[c]))
        return [pltpu.make_async_copy(src, dst, sem_ffn.at[9 * c + i]) for i, (src, dst) in enumerate(pairs)]

    def cp_out(b):
        r = pl.ds(pl.multiple_of(b * (blk // 2), blk // 2), blk // 2)
        return pltpu.make_async_copy(outs.at[r, :], out32.at[r, :], sem_out.at[b])

    cp_xpre.start()
    cp_mod(1).start()
    cp_mod(0).start()
    for j in range(N_STAGE):
        for cp in cp_stage(j):
            cp.start()

    cf = c_ref[...].astype(F32)
    sc = jnp.broadcast_to(_round(cf * jax.nn.sigmoid(cf)), (8, dm))

    def set_mod(k):
        mod[k] = _dot(sc, _bf(wmod[k])) + jnp.where(k % 3 == 1, 1.0, 0.0)

    def get_mod(k, n):
        return jnp.concatenate([mod[k]] * (n // 8), axis=0)

    def seg_x(s):
        return _bf(xs[s]).astype(F32)

    def seg_h(s):
        return _round(_mod_ln(seg_x(s), get_mod(1, seg), get_mod(0, seg)))

    def pre_norm(i, _):
        t = _bf(jnp.concatenate([xpre[2 * i, 0:hpr], xpre[2 * i + 1, 0:hpr]], axis=0)).astype(F32)
        npre[pl.ds(pl.multiple_of(i * 2 * PRE_ROWS, 2 * PRE_ROWS), 2 * PRE_ROWS), :] = _ln(t)

    def pre_mod(i, _):
        t = npre[pl.ds(pl.multiple_of(i * 64, 64), 64), :]
        hpre[pl.ds(pl.multiple_of(i * 32, 32), 32), :] = _words(t * get_mod(1, 64) + get_mod(0, 64))

    cp_xpre.wait()
    jax.lax.fori_loop(0, n_seg // 2, pre_norm, None, unroll=8)
    for k in (1, 0):
        cp_mod(k).wait()
        set_mod(k)
    jax.lax.fori_loop(0, n_seg * PRE_ROWS // 64, pre_mod, None)

    def relayout(j):
        for cp in cp_stage(j):
            cp.wait()

        def rows64(t, _):
            r = pl.multiple_of(t * 64, 64)
            for i in range(3):
                even, odd = [stage[j % N_STAGE, i, pl.ds(2 * r + k, 64, stride=2), :] for k in range(2)]
                wqkv[j, pl.ds(r, 64), 2 * i * dh:(2 * i + 1) * dh] = (even & jnp.uint32(0xFFFF)) | (odd << 16)
                wqkv[j, pl.ds(r, 64), (2 * i + 1) * dh:(2 * i + 2) * dh] = (
                    (even >> 16) | (odd & jnp.uint32(0xFFFF0000)))

        jax.lax.fori_loop(0, dm // 128, rows64, None)

        @pl.when(j + N_STAGE < n_pairs)
        def _():
            for cp in cp_stage(j + N_STAGE):
                cp.start()

        @pl.when(j + N_STAGE == n_pairs)
        def _():
            cp_x0.start()
            cp_wo.start()
            for k in range(2, 6):
                cp_mod(k).start()
            cp_x1.start()

    def pre_proj(j, _):
        jax.lax.fori_loop(jnp.maximum(2 * j - 1, 0), jnp.minimum(2 * j + 1, n_pairs),
                          lambda i, _: relayout(i), None)
        pre[j] = _dot(_bf(hpre[...]), _bf(wqkv[j]))

    jax.lax.fori_loop(0, N_PRE, pre_proj, None)
    jax.lax.fori_loop(min(2 * N_PRE - 1, n_pairs), n_pairs, lambda i, _: relayout(i), None)
    for c in range(FFN_SEGS):
        for cp in cp_ffn(c):
            cp.start()
    cp_x0.wait()
    lhs[0:n_mem, :] = mem0_ref[...].astype(F32)
    lhs[n_mem:rows, :] = seg_h(0)

    def finish(s, attn):
        xn = seg_x(s) + get_mod(2, seg) * attn
        slot = (s // FFN_SEGS) % 2
        sub = s % FFN_SEGS
        x1[slot, pl.ds(pl.multiple_of(sub * seg, seg), seg), :] = xn
        h = _mod_ln(xn, get_mod(4, seg), get_mod(3, seg))
        for i, t in enumerate(_strassen_lhs(h[:hseg, :hd], h[:hseg, hd:], h[hseg:, :hd], h[hseg:, hd:])):
            h2[slot, i, pl.ds(pl.multiple_of(sub * (hseg // 2), hseg // 2), hseg // 2), :] = _words(t)

    def step(s, phase):
        do_attn = phase != "ffn"
        do_ffn = phase in ("both", "ffn")
        if do_ffn:
            fb = s // FFN_SEGS - 1
            fch = s % FFN_SEGS
            fslot = fb % 2
            act_a, act_b = [], []
        if phase == "both":
            @pl.when(fb == 0)
            def _():
                for cp in cp_ffn(fch):
                    cp.wait()
                jax.lax.fori_loop(0, hd // 2 // CMB, lambda i, _: _strassen_rhs(
                    wup, fch, pl.multiple_of(i * CMB, CMB), CMB), None)
                jax.lax.fori_loop(0, kd // 2 // CMB, lambda i, _: _strassen_rhs(
                    wdn, fch, pl.multiple_of(i * CMB, CMB), CMB), None)

        def ffn_up(lo, hi):
            if do_ffn:
                for t in range(lo, hi, 128):
                    ga, ua, gb, ub = _strassen_out(
                        [_dot(_bf(h2[fslot, i]), _bf(wup[fch, i, :, t:t + 128])) for i in range(7)])
                    act_a.append(ga * jax.nn.sigmoid(ga) * ua)
                    act_b.append(gb * jax.nn.sigmoid(gb) * ub)

        def ffn_down():
            if do_ffn:
                aa, ab = jnp.concatenate(act_a, axis=1), jnp.concatenate(act_b, axis=1)
                ops = [t.astype(BF16) for t in _strassen_lhs(
                    aa[:, :kd], aa[:, kd:2 * kd], ab[:, :kd], ab[:, kd:2 * kd])]
                rest = _dot(jnp.concatenate([aa[:, 2 * kd:], ab[:, 2 * kd:]], axis=0).astype(BF16),
                            _bf(wrest[fch]))
                for t in range(0, hd, DOWN_COLS):
                    y = _strassen_out([_dot(ops[i], _bf(wdn[fch, i, :, t:t + DOWN_COLS])) for i in range(7)])
                    for side in range(2):
                        cols = slice(side * hd + t, side * hd + t + DOWN_COLS)
                        ya = y[side] + rest[:blk // 2, cols]
                        yb = y[2 + side] + rest[blk // 2:, cols]
                        yy = jnp.concatenate([v[k * hseg:(k + 1) * hseg] for k in range(FFN_SEGS)
                                              for v in (ya, yb)], axis=0)
                        acc = x1[fslot, :, cols] + get_mod(5, blk)[:, cols] * yy
                        x1[fslot, :, cols] = acc
                        outs[pl.ds(pl.multiple_of(fb * (blk // 2), blk // 2), blk // 2), cols] = _words(acc)

        if not do_attn:
            ffn_up(0, fc)
            ffn_down()
        else:
            r = jax.lax.broadcasted_iota(jnp.int32, (2 * rows, 2 * rows), 0)
            q = jax.lax.broadcasted_iota(jnp.int32, (2 * rows, 2 * rows), 1)
            same = (r >= rows) == (q >= rows)
            rl = jnp.where(r >= rows, r - rows, r)
            ql = jnp.where(q >= rows, q - rows, q)
            keep = same & ((rl < n_mem) | (rl >= ql))
            fill = jnp.where(same, -1e9, -jnp.inf).astype(F32)
            a = lhs[...]
            a_short = a[:rows - PRE_ROWS].astype(BF16)
            qkv, probs = {}, {}

            def proj(j):
                if j < N_PRE:
                    t = jnp.concatenate(
                        [_dot(a_short, _bf(wqkv[j])),
                         pre[j, pl.ds(pl.multiple_of(s * PRE_ROWS, PRE_ROWS), PRE_ROWS), :]], axis=0)
                else:
                    t = _dot(a, _bf(wqkv[j]))
                qkv[j] = [jnp.concatenate([t[:, (2 * i) * dh:(2 * i + 1) * dh],
                                           t[:, (2 * i + 1) * dh:(2 * i + 2) * dh]], axis=0).astype(BF16)
                          for i in range(3)]

            def scores(j):
                t = jnp.where(keep, _dot_nt(qkv[j][0], qkv[j][1]) * scale, fill)
                e = jnp.exp(t - jnp.max(t, axis=-1, keepdims=True))
                probs[j] = (e / jnp.sum(e, axis=-1, keepdims=True)).astype(BF16)

            def mix(j):
                o = _round(_dot(probs[j], qkv[j][2]))
                obuf[:, 2 * j * dh:(2 * j + 1) * dh] = o[:rows]
                obuf[:, (2 * j + 1) * dh:(2 * j + 2) * dh] = o[rows:]

            def oproj(lo, hi):
                return _dot(obuf[:, lo * 2 * dh:hi * 2 * dh], _bf(wo[lo * dh:hi * dh, :]))

            order = list(range(n_pairs))
            for i, j in enumerate(order):
                proj(j)
                if i >= 1:
                    scores(order[i - 1])
                if i >= 2:
                    mix(order[i - 2])
            ffn_up(0, 384)
            scores(order[-1])
            mix(order[-2])
            ffn_up(384, fc)
            mix(order[-1])
            if phase == "first":
                @pl.when(s == 0)
                def _():
                    cp_wo.wait()
                cp_mod(s + 2).wait()
            o = oproj(0, n_pairs)
            lhs[0:n_mem, :] = _round(o[:n_mem])
            lhs[n_mem:rows, :] = seg_h(jnp.minimum(s + 1, n_seg - 1))
            if phase != "first":
                finish(s, o[n_mem:])
            else:
                x1[0, pl.ds(pl.multiple_of(s * seg, seg), seg), :] = o[n_mem:]
                set_mod(s + 2)
            ffn_down()

        if do_ffn:
            @pl.when(fch == FFN_SEGS - 1)
            def _():
                cp_out(fb).start()

    def run(lo, hi, phase):
        jax.lax.fori_loop(lo, hi, lambda s, _: step(s, phase), None)

    run(0, FFN_SEGS, "first")
    cp_x1.wait()
    for s in range(FFN_SEGS):
        finish(s, x1[0, s * seg:(s + 1) * seg, :])
    run(FFN_SEGS, n_seg, "both")
    run(n_seg, n_seg + FFN_SEGS, "ffn")
    for b in range(n_blk):
        cp_out(b).wait()


@functools.partial(jax.jit, static_argnames=("A_seg_len",))
def pallas_adaLN_cond__memory_aug_recurrent_mem_tr__glu_gated_swiglu__prompt_kernel(
    A_x, A_mem0, A_Wq, A_Wk, A_Wv, A_Wo, A_seg_len, B_x, B_w1, B_w3, B_w2, c, w_mod,
):
    del B_x
    bsz, s_len, dm = A_x.shape
    _, n_heads, dh = A_Wq.shape
    n_mem = A_mem0.shape[1]
    seg = int(A_seg_len)
    f = B_w1.shape[1]
    fc = f // FFN_SEGS
    kd = (fc - 1) // 256 * 128
    blk = FFN_SEGS * seg
    assert bsz == 1 and s_len % blk == 0 and n_heads % 4 == 0 and fc % 128 == 0 and FFN_SEGS == 4

    hbm = pl.BlockSpec(memory_space=pltpu.MemorySpace.HBM)
    vmem = pl.BlockSpec(memory_space=pltpu.MemorySpace.VMEM)
    scratch = dict(
        wqkv=pltpu.VMEM((n_heads // 2, dm // 2, 6 * dh), U32),
        wo=pltpu.VMEM((n_heads * dh // 2, dm), U32),
        wup=pltpu.VMEM((FFN_SEGS, 7, dm // 4, fc), U32),
        wdn=pltpu.VMEM((FFN_SEGS, 7, kd // 2, dm // 2), U32),
        wrest=pltpu.VMEM((FFN_SEGS, fc // 2 - kd, dm), U32),
        wmod=pltpu.VMEM((6, dm // 2, dm), U32),
        stage=pltpu.VMEM((N_STAGE, 3, dm, dh), U32),
        xs=pltpu.VMEM((s_len // seg, seg // 2, dm), U32),
        outs=pltpu.VMEM((s_len // 2, dm), U32),
        mod=pltpu.VMEM((6, 8, dm), F32),
        lhs=pltpu.VMEM((n_mem + seg, dm), F32),
        obuf=pltpu.VMEM((n_mem + seg, n_heads * dh), F32),
        x1=pltpu.VMEM((2, blk, dm), F32),
        h2=pltpu.VMEM((2, 7, blk // 4, dm // 2), U32),
        xpre=pltpu.VMEM((s_len // seg, 8, dm), U32),
        npre=pltpu.VMEM((s_len // seg * PRE_ROWS, dm), F32),
        hpre=pltpu.VMEM((s_len // seg * PRE_ROWS // 2, dm), U32),
        pre=pltpu.VMEM((N_PRE, s_len // seg * PRE_ROWS, 6 * dh), F32),
        sem_stage=pltpu.SemaphoreType.DMA((3 * N_STAGE,)),
        sem_misc=pltpu.SemaphoreType.DMA((4,)),
        sem_mod=pltpu.SemaphoreType.DMA((6,)),
        sem_ffn=pltpu.SemaphoreType.DMA((9 * FFN_SEGS,)),
        sem_out=pltpu.SemaphoreType.DMA((s_len // blk,)),
    )

    def body(*refs):
        n_io = len(refs) - len(scratch)
        _kernel(*refs[:n_io], **dict(zip(scratch, refs[n_io:])), seg=seg, n_mem=n_mem, dh=dh)

    out = pl.pallas_call(
        body,
        out_shape=jax.ShapeDtypeStruct((s_len, dm), A_x.dtype),
        in_specs=[vmem, vmem] + [hbm] * 9,
        out_specs=hbm,
        scratch_shapes=list(scratch.values()),
        compiler_params=pltpu.CompilerParams(vmem_limit_bytes=124 * 2**20),
    )(c, A_mem0.reshape(n_mem, dm), A_x.reshape(s_len // seg, seg, dm), A_Wq, A_Wk, A_Wv,
      A_Wo.reshape(n_heads * dh, dm), B_w1, B_w3, B_w2, w_mod)
    return out.reshape(bsz, s_len, dm)
```

```python
import functools

import jax
import jax.numpy as jnp
import jax.experimental.pallas as pl
import jax.experimental.pallas.tpu as pltpu

U32 = jnp.uint32
BF16 = jnp.bfloat16
F32 = jnp.float32
LN_EPS = 1e-5
FFN_SEGS = 4
N_STAGE = 5
N_PRE = 8
PRE_ROWS = 8
DOWN_COLS = 128
CMB = 8
X_HEAD = 8


def _bf(w):
    return pltpu.bitcast(w, BF16)


def _words(a):
    return pltpu.bitcast(a.astype(BF16), U32)


def _dot(a, b):
    return jax.lax.dot_general(a, b, (((1,), (0,)), ((), ())), preferred_element_type=F32)


def _dot_nt(a, b):
    return jax.lax.dot_general(a, b, (((1,), (1,)), ((), ())), preferred_element_type=F32)


def _round(a):
    return a.astype(BF16).astype(F32)


def _ln(x):
    m = jnp.mean(x, axis=-1, keepdims=True)
    d = x - m
    v = jnp.mean(d * d, axis=-1, keepdims=True)
    return d * jax.lax.rsqrt(v + LN_EPS)


def _mod_ln(x, scale1, shift):
    return _ln(x) * scale1 + shift


def _strassen_lhs(a11, a12, a21, a22):
    return [a11 + a22, a21 + a22, a11, a22, a11 + a12, a21 - a11, a12 - a22]


def _strassen_out(m):
    return m[0] + m[3] - m[4] + m[6], m[2] + m[4], m[1] + m[3], m[0] - m[1] + m[2] + m[5]


RAW_SLOTS = (1, 2, 3, 4)


def _strassen_rhs(w, c, r, n):
    for k in range(0, w.shape[3], 128):
        at = (pl.ds(r, n), slice(k, k + 128))
        b11, b12, b21, b22 = [_bf(w[(c, i) + at]).astype(F32) for i in RAW_SLOTS]
        for i, t in ((0, b11 + b22), (2, b12 - b22), (3, b21 - b11), (5, b11 + b12), (6, b21 + b22)):
            w[(c, i) + at] = _words(t)


def _kernel(c_ref, mem0_ref, x_hbm, wq_hbm, wk_hbm, wv_hbm, wo_hbm, w1_hbm, w3_hbm, w2_hbm,
            wmod_hbm, out_hbm,
            wqkv, wo, wup, wdn, wrest, wmod, stage, xs, outs, mod, lhs, obuf, x1, h2, xpre, npre, hpre, pre,
            sem_stage, sem_misc, sem_mod, sem_ffn, sem_out, *, seg, n_mem, dh):
    n_pairs = wqkv.shape[0]
    dm = lhs.shape[1]
    rows = n_mem + seg
    hseg = seg // 2
    n_seg = xs.shape[0]
    n_blk = n_seg // FFN_SEGS
    blk = FFN_SEGS * seg
    fc = wup.shape[3]
    kd = 2 * wdn.shape[2]
    hd = dm // 2
    scale = dh ** -0.5

    wmod32 = wmod_hbm.bitcast(U32)
    x32 = x_hbm.bitcast(U32)
    out32 = out_hbm.bitcast(U32)
    qkv32 = [w.bitcast(U32) for w in (wq_hbm, wk_hbm, wv_hbm)]
    hpr = PRE_ROWS // 2
    cp_xpre = pltpu.make_async_copy(x32.at[:, pl.ds(hseg - hpr, hpr), :], xpre.at[:, pl.ds(0, hpr), :],
                                    sem_misc.at[0])
    cp_x0 = pltpu.make_async_copy(x32.at[pl.ds(0, X_HEAD)], xs.at[pl.ds(0, X_HEAD)], sem_misc.at[1])
    cp_x1 = pltpu.make_async_copy(x32.at[pl.ds(X_HEAD, n_seg - X_HEAD)], xs.at[pl.ds(X_HEAD, n_seg - X_HEAD)],
                                  sem_misc.at[2])
    cp_wo = pltpu.make_async_copy(wo_hbm.bitcast(U32), wo, sem_misc.at[3])

    def cp_mod(k):
        return pltpu.make_async_copy(wmod32.at[:, pl.ds(pl.multiple_of(k * dm, dm), dm)], wmod.at[k],
                                     sem_mod.at[k])

    def cp_stage(j):
        slot = j % N_STAGE
        return [pltpu.make_async_copy(qkv32[i].at[:, j, :], stage.at[slot, i], sem_stage.at[3 * slot + i])
                for i in range(3)]

    def cp_ffn(c):
        cols = pl.ds(pl.multiple_of(c * fc, fc), fc)
        w1_32, w3_32, w2_32 = w1_hbm.bitcast(U32), w3_hbm.bitcast(U32), w2_hbm.bitcast(U32)

        def w2_rows(off, n):
            return pl.ds(pl.multiple_of(c * (fc // 2) + off, 64), n)

        pairs = []
        for i, slot in enumerate(RAW_SLOTS):
            pairs.append(((w1_32, w3_32)[i % 2].at[pl.ds(i // 2 * (hd // 2), hd // 2), cols], wup.at[c, slot]))
            pairs.append((w2_32.at[w2_rows(i // 2 * (kd // 2), kd // 2), pl.ds(i % 2 * hd, hd)], wdn.at[c, slot]))
        pairs.append((w2_32.at[w2_rows(kd, fc // 2 - kd), :], wrest.at[c]))
        return [pltpu.make_async_copy(src, dst, sem_ffn.at[9 * c + i]) for i, (src, dst) in enumerate(pairs)]

    def cp_out(b):
        r = pl.ds(pl.multiple_of(b * (blk // 2), blk // 2), blk // 2)
        return pltpu.make_async_copy(outs.at[r, :], out32.at[r, :], sem_out.at[b])

    cp_xpre.start()
    cp_mod(1).start()
    cp_mod(0).start()
    for j in range(N_STAGE):
        for cp in cp_stage(j):
            cp.start()

    cf = c_ref[...].astype(F32)
    sc = jnp.broadcast_to(_round(cf * jax.nn.sigmoid(cf)), (8, dm))

    def set_mod(k):
        mod[k] = _dot(sc, _bf(wmod[k])) + jnp.where(k % 3 == 1, 1.0, 0.0)

    def get_mod(k, n):
        return jnp.concatenate([mod[k]] * (n // 8), axis=0)

    def seg_x(s):
        return _bf(xs[s]).astype(F32)

    def seg_h(s):
        return _round(_mod_ln(seg_x(s), get_mod(1, seg), get_mod(0, seg)))

    def pre_norm(i, _):
        t = _bf(jnp.concatenate([xpre[2 * i, 0:hpr], xpre[2 * i + 1, 0:hpr]], axis=0)).astype(F32)
        npre[pl.ds(pl.multiple_of(i * 2 * PRE_ROWS, 2 * PRE_ROWS), 2 * PRE_ROWS), :] = _ln(t)

    def pre_mod(i, _):
        t = npre[pl.ds(pl.multiple_of(i * 64, 64), 64), :]
        hpre[pl.ds(pl.multiple_of(i * 32, 32), 32), :] = _words(t * get_mod(1, 64) + get_mod(0, 64))

    cp_xpre.wait()
    jax.lax.fori_loop(0, n_seg // 2, pre_norm, None, unroll=8)
    for k in (1, 0):
        cp_mod(k).wait()
        set_mod(k)
    jax.lax.fori_loop(0, n_seg * PRE_ROWS // 64, pre_mod, None)

    def relayout(j):
        for cp in cp_stage(j):
            cp.wait()

        def rows64(t, _):
            r = pl.multiple_of(t * 64, 64)
            for i in range(3):
                even, odd = [stage[j % N_STAGE, i, pl.ds(2 * r + k, 64, stride=2), :] for k in range(2)]
                wqkv[j, pl.ds(r, 64), 2 * i * dh:(2 * i + 1) * dh] = (even & jnp.uint32(0xFFFF)) | (odd << 16)
                wqkv[j, pl.ds(r, 64), (2 * i + 1) * dh:(2 * i + 2) * dh] = (
                    (even >> 16) | (odd & jnp.uint32(0xFFFF0000)))

        jax.lax.fori_loop(0, dm // 128, rows64, None)

        @pl.when(j + N_STAGE < n_pairs)
        def _():
            for cp in cp_stage(j + N_STAGE):
                cp.start()

        @pl.when(j + N_STAGE == n_pairs)
        def _():
            cp_x0.start()
            cp_wo.start()
            for k in range(2, 6):
                cp_mod(k).start()
            cp_x1.start()

    def pre_proj(j, _):
        jax.lax.fori_loop(jnp.maximum(2 * j - 1, 0), jnp.minimum(2 * j + 1, n_pairs),
                          lambda i, _: relayout(i), None)
        pre[j] = _dot(_bf(hpre[...]), _bf(wqkv[j]))

    jax.lax.fori_loop(0, N_PRE, pre_proj, None)
    jax.lax.fori_loop(min(2 * N_PRE - 1, n_pairs), n_pairs, lambda i, _: relayout(i), None)
    for c in range(FFN_SEGS):
        for cp in cp_ffn(c):
            cp.start()
    cp_x0.wait()
    lhs[0:n_mem, :] = mem0_ref[...].astype(F32)
    lhs[n_mem:rows, :] = seg_h(0)

    def finish(s, attn):
        xn = seg_x(s) + get_mod(2, seg) * attn
        slot = (s // FFN_SEGS) % 2
        sub = s % FFN_SEGS
        x1[slot, pl.ds(pl.multiple_of(sub * seg, seg), seg), :] = xn
        h = _mod_ln(xn, get_mod(4, seg), get_mod(3, seg))
        for i, t in enumerate(_strassen_lhs(h[:hseg, :hd], h[:hseg, hd:], h[hseg:, :hd], h[hseg:, hd:])):
            h2[slot, i, pl.ds(pl.multiple_of(sub * (hseg // 2), hseg // 2), hseg // 2), :] = _words(t)

    def step(s, phase):
        do_attn = phase != "ffn"
        do_ffn = phase != "first"
        if do_ffn:
            fb = s // FFN_SEGS - 1
            fch = s % FFN_SEGS
            fslot = fb % 2
            act_a, act_b = [], []
        side_work = []
        if phase == "prep":
            for cp in cp_ffn(fch):
                cp.wait()
            side_work = [(wup, r, CMB) for r in range(0, hd // 2, CMB)]
            side_work += [(wdn, r, 2 * CMB) for r in range(0, kd // 2, 2 * CMB)]

        def prepare_weights(i, n, anchor):
            for w, r, size in side_work[len(side_work) * i // n:len(side_work) * (i + 1) // n]:
                w[fch, fb, r:r + 8, 0:128] = pltpu.bitcast(anchor, U32)
                _strassen_rhs(w, fch, r, size)

        def ffn_up(lo, hi):
            if do_ffn:
                for t in range(lo, hi, 128):
                    ga, ua, gb, ub = _strassen_out(
                        [_dot(_bf(h2[fslot, i]), _bf(wup[fch, i, :, t:t + 128])) for i in range(7)])
                    act_a.append(ga * jax.nn.sigmoid(ga) * ua)
                    act_b.append(gb * jax.nn.sigmoid(gb) * ub)

        def ffn_down():
            if do_ffn:
                aa, ab = jnp.concatenate(act_a, axis=1), jnp.concatenate(act_b, axis=1)
                ops = [t.astype(BF16) for t in _strassen_lhs(
                    aa[:, :kd], aa[:, kd:2 * kd], ab[:, :kd], ab[:, kd:2 * kd])]
                rest = _dot(jnp.concatenate([aa[:, 2 * kd:], ab[:, 2 * kd:]], axis=0).astype(BF16),
                            _bf(wrest[fch]))
                for t in range(0, hd, DOWN_COLS):
                    y = _strassen_out([_dot(ops[i], _bf(wdn[fch, i, :, t:t + DOWN_COLS])) for i in range(7)])
                    for side in range(2):
                        cols = slice(side * hd + t, side * hd + t + DOWN_COLS)
                        ya = y[side] + rest[:blk // 2, cols]
                        yb = y[2 + side] + rest[blk // 2:, cols]
                        yy = jnp.concatenate([v[k * hseg:(k + 1) * hseg] for k in range(FFN_SEGS)
                                              for v in (ya, yb)], axis=0)
                        acc = x1[fslot, :, cols] + get_mod(5, blk)[:, cols] * yy
                        x1[fslot, :, cols] = acc
                        outs[pl.ds(pl.multiple_of(fb * (blk // 2), blk // 2), blk // 2), cols] = _words(acc)

        if not do_attn:
            ffn_up(0, fc)
            ffn_down()
        else:
            r = jax.lax.broadcasted_iota(jnp.int32, (2 * rows, 2 * rows), 0)
            q = jax.lax.broadcasted_iota(jnp.int32, (2 * rows, 2 * rows), 1)
            same = (r >= rows) == (q >= rows)
            rl = jnp.where(r >= rows, r - rows, r)
            ql = jnp.where(q >= rows, q - rows, q)
            keep = same & ((rl < n_mem) | (rl >= ql))
            fill = jnp.where(same, -1e9, -jnp.inf).astype(F32)
            a = lhs[...]
            a_short = a[:rows - PRE_ROWS].astype(BF16)
            qkv, probs = {}, {}

            def proj(j):
                if j < N_PRE:
                    t = jnp.concatenate(
                        [_dot(a_short, _bf(wqkv[j])),
                         pre[j, pl.ds(pl.multiple_of(s * PRE_ROWS, PRE_ROWS), PRE_ROWS), :]], axis=0)
                else:
                    t = _dot(a, _bf(wqkv[j]))
                prepare_weights(j, n_pairs, t[0:8, 0:128])
                qkv[j] = [jnp.concatenate([t[:, (2 * i) * dh:(2 * i + 1) * dh],
                                           t[:, (2 * i + 1) * dh:(2 * i + 2) * dh]], axis=0).astype(BF16)
                          for i in range(3)]

            def scores(j):
                t = jnp.where(keep, _dot_nt(qkv[j][0], qkv[j][1]) * scale, fill)
                e = jnp.exp(t - jnp.max(t, axis=-1, keepdims=True))
                probs[j] = (e / jnp.sum(e, axis=-1, keepdims=True)).astype(BF16)

            def mix(j):
                o = _round(_dot(probs[j], qkv[j][2]))
                obuf[:, 2 * j * dh:(2 * j + 1) * dh] = o[:rows]
                obuf[:, (2 * j + 1) * dh:(2 * j + 2) * dh] = o[rows:]

            def oproj(lo, hi):
                return _dot(obuf[:, lo * 2 * dh:hi * 2 * dh], _bf(wo[lo * dh:hi * dh, :]))

            order = list(range(n_pairs))
            for i, j in enumerate(order):
                proj(j)
                if i >= 1:
                    scores(order[i - 1])
                if i >= 2:
                    mix(order[i - 2])
            ffn_up(0, 384)
            scores(order[-1])
            mix(order[-2])
            ffn_up(384, fc)
            mix(order[-1])
            if phase == "first":
                @pl.when(s == 0)
                def _():
                    cp_wo.wait()
                cp_mod(s + 2).wait()
            o = oproj(0, n_pairs)
            lhs[0:n_mem, :] = _round(o[:n_mem])
            lhs[n_mem:rows, :] = seg_h(jnp.minimum(s + 1, n_seg - 1))
            if phase != "first":
                finish(s, o[n_mem:])
            else:
                x1[0, pl.ds(pl.multiple_of(s * seg, seg), seg), :] = o[n_mem:]
                set_mod(s + 2)
            ffn_down()

        if do_ffn:
            @pl.when(fch == FFN_SEGS - 1)
            def _():
                cp_out(fb).start()

    def run(lo, hi, phase):
        jax.lax.fori_loop(lo, hi, lambda s, _: step(s, phase), None)

    run(0, FFN_SEGS, "first")
    cp_x1.wait()
    for s in range(FFN_SEGS):
        finish(s, x1[0, s * seg:(s + 1) * seg, :])
    run(FFN_SEGS, 2 * FFN_SEGS, "prep")
    run(2 * FFN_SEGS, n_seg, "both")
    run(n_seg, n_seg + FFN_SEGS, "ffn")
    for b in range(n_blk):
        cp_out(b).wait()


@functools.partial(jax.jit, static_argnames=("A_seg_len",))
def pallas_adaLN_cond__memory_aug_recurrent_mem_tr__glu_gated_swiglu__prompt_kernel(
    A_x, A_mem0, A_Wq, A_Wk, A_Wv, A_Wo, A_seg_len, B_x, B_w1, B_w3, B_w2, c, w_mod,
):
    del B_x
    bsz, s_len, dm = A_x.shape
    _, n_heads, dh = A_Wq.shape
    n_mem = A_mem0.shape[1]
    seg = int(A_seg_len)
    f = B_w1.shape[1]
    fc = f // FFN_SEGS
    kd = (fc - 1) // 256 * 128
    blk = FFN_SEGS * seg
    assert bsz == 1 and s_len % blk == 0 and n_heads % 4 == 0 and fc % 128 == 0 and FFN_SEGS == 4

    hbm = pl.BlockSpec(memory_space=pltpu.MemorySpace.HBM)
    vmem = pl.BlockSpec(memory_space=pltpu.MemorySpace.VMEM)
    scratch = dict(
        wqkv=pltpu.VMEM((n_heads // 2, dm // 2, 6 * dh), U32),
        wo=pltpu.VMEM((n_heads * dh // 2, dm), U32),
        wup=pltpu.VMEM((FFN_SEGS, 7, dm // 4, fc), U32),
        wdn=pltpu.VMEM((FFN_SEGS, 7, kd // 2, dm // 2), U32),
        wrest=pltpu.VMEM((FFN_SEGS, fc // 2 - kd, dm), U32),
        wmod=pltpu.VMEM((6, dm // 2, dm), U32),
        stage=pltpu.VMEM((N_STAGE, 3, dm, dh), U32),
        xs=pltpu.VMEM((s_len // seg, seg // 2, dm), U32),
        outs=pltpu.VMEM((s_len // 2, dm), U32),
        mod=pltpu.VMEM((6, 8, dm), F32),
        lhs=pltpu.VMEM((n_mem + seg, dm), F32),
        obuf=pltpu.VMEM((n_mem + seg, n_heads * dh), F32),
        x1=pltpu.VMEM((2, blk, dm), F32),
        h2=pltpu.VMEM((2, 7, blk // 4, dm // 2), U32),
        xpre=pltpu.VMEM((s_len // seg, 8, dm), U32),
        npre=pltpu.VMEM((s_len // seg * PRE_ROWS, dm), F32),
        hpre=pltpu.VMEM((s_len // seg * PRE_ROWS // 2, dm), U32),
        pre=pltpu.VMEM((N_PRE, s_len // seg * PRE_ROWS, 6 * dh), F32),
        sem_stage=pltpu.SemaphoreType.DMA((3 * N_STAGE,)),
        sem_misc=pltpu.SemaphoreType.DMA((4,)),
        sem_mod=pltpu.SemaphoreType.DMA((6,)),
        sem_ffn=pltpu.SemaphoreType.DMA((9 * FFN_SEGS,)),
        sem_out=pltpu.SemaphoreType.DMA((s_len // blk,)),
    )

    def body(*refs):
        n_io = len(refs) - len(scratch)
        _kernel(*refs[:n_io], **dict(zip(scratch, refs[n_io:])), seg=seg, n_mem=n_mem, dh=dh)

    out = pl.pallas_call(
        body,
        out_shape=jax.ShapeDtypeStruct((s_len, dm), A_x.dtype),
        in_specs=[vmem, vmem] + [hbm] * 9,
        out_specs=hbm,
        scratch_shapes=list(scratch.values()),
        compiler_params=pltpu.CompilerParams(vmem_limit_bytes=124 * 2**20),
    )(c, A_mem0.reshape(n_mem, dm), A_x.reshape(s_len // seg, seg, dm), A_Wq, A_Wk, A_Wv,
      A_Wo.reshape(n_heads * dh, dm), B_w1, B_w3, B_w2, w_mod)
    return out.reshape(bsz, s_len, dm)
```

```python
import functools

import jax
import jax.numpy as jnp
import jax.experimental.pallas as pl
import jax.experimental.pallas.tpu as pltpu

U32 = jnp.uint32
BF16 = jnp.bfloat16
F32 = jnp.float32
LN_EPS = 1e-5
FFN_SEGS = 4
N_STAGE = 5
N_PRE = 8
PRE_ROWS = 8
DOWN_COLS = 128
CMB = 8
X_HEAD = 8


def _bf(w):
    return pltpu.bitcast(w, BF16)


def _words(a):
    return pltpu.bitcast(a.astype(BF16), U32)


def _dot(a, b):
    return jax.lax.dot_general(a, b, (((1,), (0,)), ((), ())), preferred_element_type=F32)


def _dot_nt(a, b):
    return jax.lax.dot_general(a, b, (((1,), (1,)), ((), ())), preferred_element_type=F32)


def _round(a):
    return a.astype(BF16).astype(F32)


def _ln(x):
    m = jnp.mean(x, axis=-1, keepdims=True)
    d = x - m
    v = jnp.mean(d * d, axis=-1, keepdims=True)
    return d * jax.lax.rsqrt(v + LN_EPS)


def _mod_ln(x, scale1, shift):
    return _ln(x) * scale1 + shift


def _strassen_lhs(a11, a12, a21, a22):
    return [a11 + a22, a21 + a22, a11, a22, a11 + a12, a21 - a11, a12 - a22]


def _strassen_out(m):
    return m[0] + m[3] - m[4] + m[6], m[2] + m[4], m[1] + m[3], m[0] - m[1] + m[2] + m[5]


RAW_SLOTS = (1, 2, 3, 4)


def _strassen_rhs(w, c, r, n):
    for k in range(0, w.shape[3], 128):
        at = (pl.ds(r, n), slice(k, k + 128))
        b11, b12, b21, b22 = [_bf(w[(c, i) + at]).astype(F32) for i in RAW_SLOTS]
        for i, t in ((0, b11 + b22), (2, b12 - b22), (3, b21 - b11), (5, b11 + b12), (6, b21 + b22)):
            w[(c, i) + at] = _words(t)


def _kernel(c_ref, mem0_ref, x_hbm, wq_hbm, wk_hbm, wv_hbm, wo_hbm, w1_hbm, w3_hbm, w2_hbm,
            wmod_hbm, out_hbm,
            wqkv, wo, wup, wdn, wrest, wmod, stage, xs, outs, mod, lhs, obuf, x1, h2, xpre, npre, hpre, pre,
            sem_stage, sem_misc, sem_mod, sem_ffn, sem_out, *, seg, n_mem, dh):
    n_pairs = wqkv.shape[0]
    dm = lhs.shape[1]
    rows = n_mem + seg
    hseg = seg // 2
    n_seg = xs.shape[0]
    n_blk = n_seg // FFN_SEGS
    blk = FFN_SEGS * seg
    fc = wup.shape[3]
    kd = 2 * wdn.shape[2]
    hd = dm // 2
    scale = dh ** -0.5

    wmod32 = wmod_hbm.bitcast(U32)
    x32 = x_hbm.bitcast(U32)
    out32 = out_hbm.bitcast(U32)
    qkv32 = [w.bitcast(U32) for w in (wq_hbm, wk_hbm, wv_hbm)]
    hpr = PRE_ROWS // 2
    cp_xpre = pltpu.make_async_copy(x32.at[:, pl.ds(hseg - hpr, hpr), :], xpre.at[:, pl.ds(0, hpr), :],
                                    sem_misc.at[0])
    cp_x0 = pltpu.make_async_copy(x32.at[pl.ds(0, X_HEAD)], xs.at[pl.ds(0, X_HEAD)], sem_misc.at[1])
    cp_x1 = pltpu.make_async_copy(x32.at[pl.ds(X_HEAD, n_seg - X_HEAD)], xs.at[pl.ds(X_HEAD, n_seg - X_HEAD)],
                                  sem_misc.at[2])
    cp_wo = pltpu.make_async_copy(wo_hbm.bitcast(U32), wo, sem_misc.at[3])

    def cp_mod(k):
        return pltpu.make_async_copy(wmod32.at[:, pl.ds(pl.multiple_of(k * dm, dm), dm)], wmod.at[k],
                                     sem_mod.at[k])

    def cp_stage(j):
        slot = j % N_STAGE
        return [pltpu.make_async_copy(qkv32[i].at[:, j, :], stage.at[slot, i, pl.ds(0, dm)],
                                      sem_stage.at[3 * slot + i])
                for i in range(3)]

    def cp_ffn(c):
        cols = pl.ds(pl.multiple_of(c * fc, fc), fc)
        w1_32, w3_32, w2_32 = w1_hbm.bitcast(U32), w3_hbm.bitcast(U32), w2_hbm.bitcast(U32)

        def w2_rows(off, n):
            return pl.ds(pl.multiple_of(c * (fc // 2) + off, 64), n)

        pairs = []
        for i, slot in enumerate(RAW_SLOTS):
            pairs.append(((w1_32, w3_32)[i % 2].at[pl.ds(i // 2 * (hd // 2), hd // 2), cols], wup.at[c, slot]))
            pairs.append((w2_32.at[w2_rows(i // 2 * (kd // 2), kd // 2), pl.ds(i % 2 * hd, hd)], wdn.at[c, slot]))
        pairs.append((w2_32.at[w2_rows(kd, fc // 2 - kd), :], wrest.at[c]))
        return [pltpu.make_async_copy(src, dst, sem_ffn.at[9 * c + i]) for i, (src, dst) in enumerate(pairs)]

    def cp_out(b):
        r = pl.ds(pl.multiple_of(b * (blk // 2), blk // 2), blk // 2)
        return pltpu.make_async_copy(outs.at[r, :], out32.at[r, :], sem_out.at[b])

    cp_xpre.start()
    cp_mod(1).start()
    cp_mod(0).start()
    for j in range(N_STAGE):
        for cp in cp_stage(j):
            cp.start()

    cf = c_ref[...].astype(F32)
    sc = jnp.broadcast_to(_round(cf * jax.nn.sigmoid(cf)), (8, dm))

    def set_mod(k):
        mod[k] = _dot(sc, _bf(wmod[k])) + jnp.where(k % 3 == 1, 1.0, 0.0)

    def get_mod(k, n):
        return jnp.concatenate([mod[k]] * (n // 8), axis=0)

    def seg_x(s):
        return _bf(xs[s]).astype(F32)

    def seg_h(s):
        return _round(_mod_ln(seg_x(s), get_mod(1, seg), get_mod(0, seg)))

    def pre_norm(i, _):
        t = _bf(jnp.concatenate([xpre[2 * i, 0:hpr], xpre[2 * i + 1, 0:hpr]], axis=0)).astype(F32)
        npre[pl.ds(pl.multiple_of(i * 2 * PRE_ROWS, 2 * PRE_ROWS), 2 * PRE_ROWS), :] = _ln(t)

    def pre_mod(i, _):
        t = npre[pl.ds(pl.multiple_of(i * 64, 64), 64), :]
        hpre[pl.ds(pl.multiple_of(i * 32, 32), 32), :] = _words(t * get_mod(1, 64) + get_mod(0, 64))

    cp_xpre.wait()
    jax.lax.fori_loop(0, n_seg // 2, pre_norm, None, unroll=8)
    for k in (1, 0):
        cp_mod(k).wait()
        set_mod(k)
    jax.lax.fori_loop(0, n_seg * PRE_ROWS // 64, pre_mod, None)

    def relayout(j, r, n):
        for i in range(3):
            even, odd = [stage[j % N_STAGE, i, pl.ds(2 * r + k, n, stride=2), :] for k in range(2)]
            wqkv[j, pl.ds(r, n), 2 * i * dh:(2 * i + 1) * dh] = (even & jnp.uint32(0xFFFF)) | (odd << 16)
            wqkv[j, pl.ds(r, n), (2 * i + 1) * dh:(2 * i + 2) * dh] = (
                (even >> 16) | (odd & jnp.uint32(0xFFFF0000)))

    def refill(j):
        @pl.when(j + N_STAGE < n_pairs)
        def _():
            for cp in cp_stage(j + N_STAGE):
                cp.start()

        @pl.when(j + N_STAGE == n_pairs)
        def _():
            cp_x0.start()
            cp_wo.start()
            for k in range(2, 6):
                cp_mod(k).start()
            cp_x1.start()

    def pre_proj(i, _):
        nxt = jnp.minimum(i + 1, n_pairs - 1)

        @pl.when(i + 1 < n_pairs)
        def _():
            for cp in cp_stage(nxt):
                cp.wait()

        half = hpre.shape[0] // 2
        a = _bf(hpre[pl.ds(pl.multiple_of(i % 2 * half, half), half), :])
        res = []
        for t in range(6):
            res.append(_dot(a, _bf(wqkv[i // 2, :, t * dh:(t + 1) * dh])))
            pre[i // 2, pl.ds(pl.multiple_of(i % 2 * 2 * half, 2 * half), 2 * half), t * dh:(t + 1) * dh] = res[t]
            if 1 <= t <= 4:
                for g in range(2):
                    stage[nxt % N_STAGE, 0, pl.ds(pl.multiple_of(dm + i // n_pairs * 8, 8), 8), :] = (
                        pltpu.bitcast(res[t - 1][g * half:g * half + 8], U32))
                    relayout(nxt, (2 * t - 2 + g) * (dm // 16), dm // 16)
        refill(i + 1)

    for cp in cp_stage(0):
        cp.wait()
    jax.lax.fori_loop(0, dm // 128, lambda t, _: relayout(0, pl.multiple_of(t * 64, 64), 64), None)
    refill(0)
    jax.lax.fori_loop(0, n_pairs, pre_proj, None)
    for c in range(FFN_SEGS):
        for cp in cp_ffn(c):
            cp.start()
    cp_x0.wait()
    lhs[0:n_mem, :] = mem0_ref[...].astype(F32)
    lhs[n_mem:rows, :] = seg_h(0)

    def finish(s, attn):
        xn = seg_x(s) + get_mod(2, seg) * attn
        slot = (s >> 2) & 1
        sub = s & 3
        x1[slot, pl.ds(pl.multiple_of(sub * seg, seg), seg), :] = xn
        h = _mod_ln(xn, get_mod(4, seg), get_mod(3, seg))
        for i, t in enumerate(_strassen_lhs(h[:hseg, :hd], h[:hseg, hd:], h[hseg:, :hd], h[hseg:, hd:])):
            h2[slot, i, pl.ds(pl.multiple_of(sub * (hseg // 2), hseg // 2), hseg // 2), :] = _words(t)

    def step(s, phase):
        do_attn = phase != "ffn"
        do_ffn = phase != "first"
        if do_ffn:
            fb = (s >> 2) - 1
            fch = s & 3
            fslot = fb & 1
            act_a, act_b = [], []
        side_work = []
        if phase == "prep":
            for cp in cp_ffn(fch):
                cp.wait()
            side_work = [(wup, r, CMB) for r in range(0, hd // 2, CMB)]
            side_work += [(wdn, r, 2 * CMB) for r in range(0, kd // 2, 2 * CMB)]

        def prepare_weights(i, n, anchor):
            for w, r, size in side_work[len(side_work) * i // n:len(side_work) * (i + 1) // n]:
                w[fch, fb, r:r + 8, 0:128] = pltpu.bitcast(anchor, U32)
                _strassen_rhs(w, fch, r, size)

        def ffn_up(lo, hi):
            if do_ffn:
                for t in range(lo, hi, 128):
                    ga, ua, gb, ub = _strassen_out(
                        [_dot(_bf(h2[fslot, i]), _bf(wup[fch, i, :, t:t + 128])) for i in range(7)])
                    act_a.append(ga * jax.nn.sigmoid(ga) * ua)
                    act_b.append(gb * jax.nn.sigmoid(gb) * ub)

        def ffn_down():
            if do_ffn:
                aa, ab = jnp.concatenate(act_a, axis=1), jnp.concatenate(act_b, axis=1)
                ops = [t.astype(BF16) for t in _strassen_lhs(
                    aa[:, :kd], aa[:, kd:2 * kd], ab[:, :kd], ab[:, kd:2 * kd])]
                rest = _dot(jnp.concatenate([aa[:, 2 * kd:], ab[:, 2 * kd:]], axis=0).astype(BF16),
                            _bf(wrest[fch]))
                for t in range(0, hd, DOWN_COLS):
                    y = _strassen_out([_dot(ops[i], _bf(wdn[fch, i, :, t:t + DOWN_COLS])) for i in range(7)])
                    for side in range(2):
                        cols = slice(side * hd + t, side * hd + t + DOWN_COLS)
                        ya = y[side] + rest[:blk // 2, cols]
                        yb = y[2 + side] + rest[blk // 2:, cols]
                        yy = jnp.concatenate([v[k * hseg:(k + 1) * hseg] for k in range(FFN_SEGS)
                                              for v in (ya, yb)], axis=0)
                        acc = x1[fslot, :, cols] + get_mod(5, blk)[:, cols] * yy
                        x1[fslot, :, cols] = acc
                        outs[pl.ds(pl.multiple_of(fb * (blk // 2), blk // 2), blk // 2), cols] = _words(acc)

        if not do_attn:
            ffn_up(0, fc)
            ffn_down()
        else:
            r = jax.lax.broadcasted_iota(jnp.int32, (2 * rows, 2 * rows), 0)
            q = jax.lax.broadcasted_iota(jnp.int32, (2 * rows, 2 * rows), 1)
            same = (r >= rows) == (q >= rows)
            rl = jnp.where(r >= rows, r - rows, r)
            ql = jnp.where(q >= rows, q - rows, q)
            keep = same & ((rl < n_mem) | (rl >= ql))
            fill = jnp.where(same, -1e9, -jnp.inf).astype(F32)
            a = lhs[...]
            a_short = a[:rows - PRE_ROWS].astype(BF16)
            qkv, probs = {}, {}

            def proj(j):
                if j < N_PRE:
                    t = jnp.concatenate(
                        [_dot(a_short, _bf(wqkv[j])),
                         pre[j, pl.ds(pl.multiple_of(s * PRE_ROWS, PRE_ROWS), PRE_ROWS), :]], axis=0)
                else:
                    t = _dot(a, _bf(wqkv[j]))
                prepare_weights(j, n_pairs, t[0:8, 0:128])
                qkv[j] = [jnp.concatenate([t[:, (2 * i) * dh:(2 * i + 1) * dh],
                                           t[:, (2 * i + 1) * dh:(2 * i + 2) * dh]], axis=0).astype(BF16)
                          for i in range(3)]

            def scores(j):
                t = jnp.where(keep, _dot_nt(qkv[j][0], qkv[j][1]) * scale, fill)
                e = jnp.exp(t - jnp.max(t, axis=-1, keepdims=True))
                probs[j] = (e / jnp.sum(e, axis=-1, keepdims=True)).astype(BF16)

            def mix(j):
                o = _round(_dot(probs[j], qkv[j][2]))
                obuf[:, 2 * j * dh:(2 * j + 1) * dh] = o[:rows]
                obuf[:, (2 * j + 1) * dh:(2 * j + 2) * dh] = o[rows:]

            def oproj(lo, hi):
                return _dot(obuf[:, lo * 2 * dh:hi * 2 * dh], _bf(wo[lo * dh:hi * dh, :]))

            order = list(range(n_pairs))
            for i, j in enumerate(order):
                proj(j)
                if i >= 1:
                    scores(order[i - 1])
                if i >= 2:
                    mix(order[i - 2])
            ffn_up(0, 384)
            scores(order[-1])
            mix(order[-2])
            ffn_up(384, fc)
            mix(order[-1])
            if phase == "first":
                @pl.when(s == 0)
                def _():
                    cp_wo.wait()

                @pl.when(s > 0)
                def _():
                    cp_mod(s + 1).wait()
            o = oproj(0, n_pairs)
            lhs[0:n_mem, :] = _round(o[:n_mem])
            lhs[n_mem:rows, :] = seg_h(jnp.minimum(s + 1, n_seg - 1))
            if phase != "first":
                finish(s, o[n_mem:])
            else:
                x1[0, pl.ds(pl.multiple_of(s * seg, seg), seg), :] = o[n_mem:]
                set_mod(s + 1)
            ffn_down()

        if do_ffn:
            @pl.when(fch == FFN_SEGS - 1)
            def _():
                cp_out(fb).start()

    def run(lo, hi, phase):
        jax.lax.fori_loop(lo, hi, lambda s, _: step(s, phase), None)

    run(0, FFN_SEGS, "first")
    cp_x1.wait()
    cp_mod(5).wait()
    set_mod(5)
    for s in range(FFN_SEGS):
        finish(s, x1[0, s * seg:(s + 1) * seg, :])
    run(FFN_SEGS, 2 * FFN_SEGS, "prep")
    run(2 * FFN_SEGS, n_seg, "both")
    run(n_seg, n_seg + FFN_SEGS, "ffn")
    for b in range(n_blk):
        cp_out(b).wait()


@functools.partial(jax.jit, static_argnames=("A_seg_len",))
def pallas_adaLN_cond__memory_aug_recurrent_mem_tr__glu_gated_swiglu__prompt_kernel(
    A_x, A_mem0, A_Wq, A_Wk, A_Wv, A_Wo, A_seg_len, B_x, B_w1, B_w3, B_w2, c, w_mod,
):
    del B_x
    bsz, s_len, dm = A_x.shape
    _, n_heads, dh = A_Wq.shape
    n_mem = A_mem0.shape[1]
    seg = int(A_seg_len)
    f = B_w1.shape[1]
    fc = f // FFN_SEGS
    kd = (fc - 1) // 256 * 128
    blk = FFN_SEGS * seg
    assert bsz == 1 and s_len % blk == 0 and n_heads % 4 == 0 and fc % 128 == 0 and FFN_SEGS == 4
    assert n_heads == 4 * N_PRE

    hbm = pl.BlockSpec(memory_space=pltpu.MemorySpace.HBM)
    vmem = pl.BlockSpec(memory_space=pltpu.MemorySpace.VMEM)
    scratch = dict(
        wqkv=pltpu.VMEM((n_heads // 2, dm // 2, 6 * dh), U32),
        wo=pltpu.VMEM((n_heads * dh // 2, dm), U32),
        wup=pltpu.VMEM((FFN_SEGS, 7, dm // 4, fc), U32),
        wdn=pltpu.VMEM((FFN_SEGS, 7, kd // 2, dm // 2), U32),
        wrest=pltpu.VMEM((FFN_SEGS, fc // 2 - kd, dm), U32),
        wmod=pltpu.VMEM((6, dm // 2, dm), U32),
        stage=pltpu.VMEM((N_STAGE, 3, dm + 8, dh), U32),
        xs=pltpu.VMEM((s_len // seg, seg // 2, dm), U32),
        outs=pltpu.VMEM((s_len // 2, dm), U32),
        mod=pltpu.VMEM((6, 8, dm), F32),
        lhs=pltpu.VMEM((n_mem + seg, dm), F32),
        obuf=pltpu.VMEM((n_mem + seg, n_heads * dh), F32),
        x1=pltpu.VMEM((2, blk, dm), F32),
        h2=pltpu.VMEM((2, 7, blk // 4, dm // 2), U32),
        xpre=pltpu.VMEM((s_len // seg, 8, dm), U32),
        npre=pltpu.VMEM((s_len // seg * PRE_ROWS, dm), F32),
        hpre=pltpu.VMEM((s_len // seg * PRE_ROWS // 2, dm), U32),
        pre=pltpu.VMEM((N_PRE, s_len // seg * PRE_ROWS, 6 * dh), F32),
        sem_stage=pltpu.SemaphoreType.DMA((3 * N_STAGE,)),
        sem_misc=pltpu.SemaphoreType.DMA((4,)),
        sem_mod=pltpu.SemaphoreType.DMA((6,)),
        sem_ffn=pltpu.SemaphoreType.DMA((9 * FFN_SEGS,)),
        sem_out=pltpu.SemaphoreType.DMA((s_len // blk,)),
    )

    def body(*refs):
        n_io = len(refs) - len(scratch)
        _kernel(*refs[:n_io], **dict(zip(scratch, refs[n_io:])), seg=seg, n_mem=n_mem, dh=dh)

    out = pl.pallas_call(
        body,
        out_shape=jax.ShapeDtypeStruct((s_len, dm), A_x.dtype),
        in_specs=[vmem, vmem] + [hbm] * 9,
        out_specs=hbm,
        scratch_shapes=list(scratch.values()),
        compiler_params=pltpu.CompilerParams(vmem_limit_bytes=124 * 2**20),
    )(c, A_mem0.reshape(n_mem, dm), A_x.reshape(s_len // seg, seg, dm), A_Wq, A_Wk, A_Wv,
      A_Wo.reshape(n_heads * dh, dm), B_w1, B_w3, B_w2, w_mod)
    return out.reshape(bsz, s_len, dm)
```

```python
import functools

import jax
import jax.numpy as jnp
import jax.experimental.pallas as pl
import jax.experimental.pallas.tpu as pltpu

U32 = jnp.uint32
BF16 = jnp.bfloat16
F32 = jnp.float32
LN_EPS = 1e-5
FFN_SEGS = 4
N_STAGE = 5
PRE_TILES = 7
PRE_ROWS = 8
DOWN_COLS = 128
CMB = 8
LAG_S, LAG_M = 2, 4
X_HEAD = 8


def _bf(w):
    return pltpu.bitcast(w, BF16)


def _words(a):
    return pltpu.bitcast(a.astype(BF16), U32)


def _dot(a, b):
    return jax.lax.dot_general(a, b, (((1,), (0,)), ((), ())), preferred_element_type=F32)


def _dot_nt(a, b):
    return jax.lax.dot_general(a, b, (((1,), (1,)), ((), ())), preferred_element_type=F32)


def _round(a):
    return a.astype(BF16).astype(F32)


def _ln(x):
    m = jnp.mean(x, axis=-1, keepdims=True)
    d = x - m
    v = jnp.mean(d * d, axis=-1, keepdims=True)
    return d * jax.lax.rsqrt(v + LN_EPS)


def _mod_ln(x, scale1, shift):
    return _ln(x) * scale1 + shift


def _strassen_lhs(a11, a12, a21, a22):
    return [a11 + a22, a21 + a22, a11, a22, a11 + a12, a21 - a11, a12 - a22]


def _strassen_out(m):
    return m[0] + m[3] - m[4] + m[6], m[2] + m[4], m[1] + m[3], m[0] - m[1] + m[2] + m[5]


RAW_SLOTS = (1, 2, 3, 4)


def _strassen_rhs(w, c, r, n):
    for k in range(0, w.shape[3], 128):
        at = (pl.ds(r, n), slice(k, k + 128))
        b11, b12, b21, b22 = [_bf(w[(c, i) + at]).astype(F32) for i in RAW_SLOTS]
        for i, t in ((0, b11 + b22), (2, b12 - b22), (3, b21 - b11), (5, b11 + b12), (6, b21 + b22)):
            w[(c, i) + at] = _words(t)


def _kernel(c_ref, mem0_ref, x_hbm, wq_hbm, wk_hbm, wv_hbm, wo_hbm, w1_hbm, w3_hbm, w2_hbm,
            wmod_hbm, out_hbm,
            wqkv, wo, wup, wdn, wrest, wmod, stage, xs, outs, mod, lhs, obuf, x1, h2, xpre, npre, hpre, pre,
            sem_stage, sem_misc, sem_mod, sem_ffn, sem_out, *, seg, n_mem, dh):
    n_pairs = wqkv.shape[0] // 6
    dm = lhs.shape[1]
    rows = n_mem + seg
    hseg = seg // 2
    n_seg = xs.shape[0]
    n_blk = n_seg // FFN_SEGS
    blk = FFN_SEGS * seg
    fc = wup.shape[3]
    kd = 2 * wdn.shape[2]
    hd = dm // 2
    scale = dh ** -0.5

    wmod32 = wmod_hbm.bitcast(U32)
    x32 = x_hbm.bitcast(U32)
    out32 = out_hbm.bitcast(U32)
    qkv32 = [w.bitcast(U32) for w in (wq_hbm, wk_hbm, wv_hbm)]
    hpr = PRE_ROWS // 2
    cp_xpre = pltpu.make_async_copy(x32.at[:, pl.ds(hseg - hpr, hpr), :], xpre.at[:, pl.ds(0, hpr), :],
                                    sem_misc.at[0])
    cp_x0 = pltpu.make_async_copy(x32.at[pl.ds(0, X_HEAD)], xs.at[pl.ds(0, X_HEAD)], sem_misc.at[1])
    cp_x1 = pltpu.make_async_copy(x32.at[pl.ds(X_HEAD, n_seg - X_HEAD)], xs.at[pl.ds(X_HEAD, n_seg - X_HEAD)],
                                  sem_misc.at[2])
    cp_wo = pltpu.make_async_copy(wo_hbm.bitcast(U32), wo, sem_misc.at[3])

    def cp_mod(k):
        return pltpu.make_async_copy(wmod32.at[:, pl.ds(pl.multiple_of(k * dm, dm), dm)], wmod.at[k],
                                     sem_mod.at[k])

    def cp_stage(j):
        slot = j % N_STAGE
        return [pltpu.make_async_copy(qkv32[i].at[:, j, :], stage.at[slot, i, pl.ds(0, dm)],
                                      sem_stage.at[3 * slot + i])
                for i in range(3)]

    def cp_ffn(c):
        cols = pl.ds(pl.multiple_of(c * fc, fc), fc)
        w1_32, w3_32, w2_32 = w1_hbm.bitcast(U32), w3_hbm.bitcast(U32), w2_hbm.bitcast(U32)

        def w2_rows(off, n):
            return pl.ds(pl.multiple_of(c * (fc // 2) + off, 64), n)

        pairs = []
        for i, slot in enumerate(RAW_SLOTS):
            pairs.append(((w1_32, w3_32)[i % 2].at[pl.ds(i // 2 * (hd // 2), hd // 2), cols], wup.at[c, slot]))
            pairs.append((w2_32.at[w2_rows(i // 2 * (kd // 2), kd // 2), pl.ds(i % 2 * hd, hd)], wdn.at[c, slot]))
        pairs.append((w2_32.at[w2_rows(kd, fc // 2 - kd), :], wrest.at[c]))
        return [pltpu.make_async_copy(src, dst, sem_ffn.at[9 * c + i]) for i, (src, dst) in enumerate(pairs)]

    def cp_out(b):
        r = pl.ds(pl.multiple_of(b * (blk // 2), blk // 2), blk // 2)
        return pltpu.make_async_copy(outs.at[r, :], out32.at[r, :], sem_out.at[b])

    cp_xpre.start()
    cp_mod(1).start()
    cp_mod(0).start()
    for j in range(N_STAGE):
        for cp in cp_stage(j):
            cp.start()

    cf = c_ref[...].astype(F32)
    sc = jnp.broadcast_to(_round(cf * jax.nn.sigmoid(cf)), (8, dm))

    def set_mod(k):
        mod[k] = _dot(sc, _bf(wmod[k])) + jnp.where(k % 3 == 1, 1.0, 0.0)

    def get_mod(k, n):
        return jnp.concatenate([mod[k]] * (n // 8), axis=0)

    def seg_x(s):
        return _bf(xs[s]).astype(F32)

    def seg_h(s):
        return _round(_mod_ln(seg_x(s), get_mod(1, seg), get_mod(0, seg)))

    def pre_norm(i, _):
        t = _bf(jnp.concatenate([xpre[2 * i, 0:hpr], xpre[2 * i + 1, 0:hpr]], axis=0)).astype(F32)
        npre[pl.ds(pl.multiple_of(i * 2 * PRE_ROWS, 2 * PRE_ROWS), 2 * PRE_ROWS), :] = _ln(t)

    def pre_mod(i, _):
        t = npre[pl.ds(pl.multiple_of(i * 64, 64), 64), :]
        hpre[pl.ds(pl.multiple_of(i * 32, 32), 32), :] = _words(t * get_mod(1, 64) + get_mod(0, 64))

    cp_xpre.wait()
    jax.lax.fori_loop(0, n_seg // 2, pre_norm, None, unroll=8)
    for k in (1, 0):
        cp_mod(k).wait()
        set_mod(k)
    jax.lax.fori_loop(0, n_seg * PRE_ROWS // 64, pre_mod, None)

    def relayout(j, r, n):
        for i in range(3):
            even, odd = [stage[j % N_STAGE, i, pl.ds(2 * r + k, n, stride=2), :] for k in range(2)]
            wqkv[6 * j + 2 * i, pl.ds(r, n), :] = (even & jnp.uint32(0xFFFF)) | (odd << 16)
            wqkv[6 * j + 2 * i + 1, pl.ds(r, n), :] = (even >> 16) | (odd & jnp.uint32(0xFFFF0000))

    def refill(j):
        @pl.when(j + N_STAGE < n_pairs)
        def _():
            for cp in cp_stage(j + N_STAGE):
                cp.start()

        def queue_rest(*_):
            cp_x0.start()
            cp_wo.start()
            for k in range(2, 6):
                cp_mod(k).start()
            cp_x1.start()

        jax.lax.fori_loop(0, jnp.where(j + N_STAGE == n_pairs, 1, 0), queue_rest, None)

    def pre_proj(i, _):
        nxt = jnp.minimum(i + 1, n_pairs - 1)

        @pl.when(i + 1 < n_pairs)
        def _():
            for cp in cp_stage(nxt):
                cp.wait()

        half = hpre.shape[0] // 2
        a = _bf(hpre[pl.ds(pl.multiple_of(i % 2 * half, half), half), :])
        res = []
        for t in range(PRE_TILES):
            tile = i // 2 * PRE_TILES + t
            res.append(_dot(a, _bf(wqkv[tile])))
            pre[tile, pl.ds(pl.multiple_of(i % 2 * 2 * half, 2 * half), 2 * half), :] = res[t]
            if 1 <= t <= 4:
                for g in range(2):
                    stage[nxt % N_STAGE, 0, pl.ds(pl.multiple_of(dm + i // n_pairs * 8, 8), 8), :] = (
                        pltpu.bitcast(res[t - 1][g * half:g * half + 8], U32))
                    relayout(nxt, (2 * t - 2 + g) * (dm // 16), dm // 16)
        refill(i + 1)

    for cp in cp_stage(0):
        cp.wait()
    jax.lax.fori_loop(0, dm // 128, lambda t, _: relayout(0, pl.multiple_of(t * 64, 64), 64), None)
    refill(0)
    jax.lax.fori_loop(0, n_pairs, pre_proj, None)
    for c in range(FFN_SEGS):
        for cp in cp_ffn(c):
            cp.start()
    cp_x0.wait()
    lhs[0:n_mem, :] = mem0_ref[...].astype(F32)
    lhs[n_mem:rows, :] = seg_h(0)

    def finish(s, attn):
        xn = seg_x(s) + get_mod(2, seg) * attn
        slot = (s >> 2) & 1
        sub = s & 3
        x1[slot, pl.ds(pl.multiple_of(sub * seg, seg), seg), :] = xn
        h = _mod_ln(xn, get_mod(4, seg), get_mod(3, seg))
        for i, t in enumerate(_strassen_lhs(h[:hseg, :hd], h[:hseg, hd:], h[hseg:, :hd], h[hseg:, hd:])):
            h2[slot, i, pl.ds(pl.multiple_of(sub * (hseg // 2), hseg // 2), hseg // 2), :] = _words(t)

    def step(s, phase):
        do_attn = phase != "ffn"
        do_ffn = phase != "first"
        if do_ffn:
            fb = (s >> 2) - 1
            fch = s & 3
            fslot = fb & 1
            act_a, act_b = [], []
        side_work = []
        if phase == "prep":
            for cp in cp_ffn(fch):
                cp.wait()
            side_work = [(wup, r, CMB) for r in range(0, hd // 2, CMB)]
            side_work += [(wdn, r, 2 * CMB) for r in range(0, kd // 2, 2 * CMB)]

        def prepare_weights(i, n, anchor):
            for w, r, size in side_work[len(side_work) * i // n:len(side_work) * (i + 1) // n]:
                w[fch, fb, r:r + 8, 0:128] = pltpu.bitcast(anchor, U32)
                _strassen_rhs(w, fch, r, size)

        def ffn_up(lo, hi):
            if do_ffn:
                for t in range(lo, hi, 128):
                    ga, ua, gb, ub = _strassen_out(
                        [_dot(_bf(h2[fslot, i]), _bf(wup[fch, i, :, t:t + 128])) for i in range(7)])
                    act_a.append(ga * jax.nn.sigmoid(ga) * ua)
                    act_b.append(gb * jax.nn.sigmoid(gb) * ub)

        def ffn_down():
            if do_ffn:
                aa, ab = jnp.concatenate(act_a, axis=1), jnp.concatenate(act_b, axis=1)
                ops = [t.astype(BF16) for t in _strassen_lhs(
                    aa[:, :kd], aa[:, kd:2 * kd], ab[:, :kd], ab[:, kd:2 * kd])]
                rest = _dot(jnp.concatenate([aa[:, 2 * kd:], ab[:, 2 * kd:]], axis=0).astype(BF16),
                            _bf(wrest[fch]))
                for t in range(0, hd, DOWN_COLS):
                    y = _strassen_out([_dot(ops[i], _bf(wdn[fch, i, :, t:t + DOWN_COLS])) for i in range(7)])
                    for side in range(2):
                        cols = slice(side * hd + t, side * hd + t + DOWN_COLS)
                        ya = y[side] + rest[:blk // 2, cols]
                        yb = y[2 + side] + rest[blk // 2:, cols]
                        yy = jnp.concatenate([v[k * hseg:(k + 1) * hseg] for k in range(FFN_SEGS)
                                              for v in (ya, yb)], axis=0)
                        acc = x1[fslot, :, cols] + get_mod(5, blk)[:, cols] * yy
                        x1[fslot, :, cols] = acc
                        outs[pl.ds(pl.multiple_of(fb * (blk // 2), blk // 2), blk // 2), cols] = _words(acc)

        if not do_attn:
            ffn_up(0, fc)
            ffn_down()
        else:
            r = jax.lax.broadcasted_iota(jnp.int32, (2 * rows, 2 * rows), 0)
            q = jax.lax.broadcasted_iota(jnp.int32, (2 * rows, 2 * rows), 1)
            same = (r >= rows) == (q >= rows)
            rl = jnp.where(r >= rows, r - rows, r)
            ql = jnp.where(q >= rows, q - rows, q)
            keep = same & ((rl < n_mem) | (rl >= ql))
            fill = jnp.where(same, -1e9, -jnp.inf).astype(F32)
            a = lhs[...]
            a_short = a[:rows - PRE_ROWS].astype(BF16)
            qkv, probs = {}, {}

            def proj(j):
                t = []
                for tile in range(6 * j, 6 * j + 6):
                    if tile < pre.shape[0]:
                        t.append(jnp.concatenate(
                            [_dot(a_short, _bf(wqkv[tile])),
                             pre[tile, pl.ds(pl.multiple_of(s * PRE_ROWS, PRE_ROWS), PRE_ROWS), :]], axis=0))
                    else:
                        t.append(_dot(a, _bf(wqkv[tile])))
                prepare_weights(j, n_pairs, t[0][0:8])
                qkv[j] = [jnp.concatenate(t[2 * i:2 * i + 2], axis=0).astype(BF16) for i in range(3)]

            def scores(j):
                t = jnp.where(keep, _dot_nt(qkv[j][0], qkv[j][1]) * scale, fill)
                e = jnp.exp(t - jnp.max(t, axis=-1, keepdims=True))
                probs[j] = (e / jnp.sum(e, axis=-1, keepdims=True)).astype(BF16)

            def mix(j):
                o = _round(_dot(probs[j], qkv[j][2]))
                obuf[:, 2 * j * dh:(2 * j + 1) * dh] = o[:rows]
                obuf[:, (2 * j + 1) * dh:(2 * j + 2) * dh] = o[rows:]

            def oproj(lo, hi):
                return _dot(obuf[:, lo * 2 * dh:hi * 2 * dh], _bf(wo[lo * dh:hi * dh, :]))

            def first_waits():
                @pl.when(s == 0)
                def _():
                    cp_wo.wait()

                @pl.when(s > 0)
                def _():
                    cp_mod(s + 1).wait()

            fillers = [functools.partial(proj, j) for j in range(n_pairs)]
            parts = []
            if do_ffn:
                fillers += [functools.partial(ffn_up, t, t + 128) for t in range(0, fc, 128)]
                done = 0
            else:
                fillers.insert(n_pairs - 1, first_waits)
                fillers += [lambda k=k: parts.append(oproj(3 * k, 3 * k + 3)) for k in range(LAG_M)]
                done = 3 * LAG_M
            for i, filler in enumerate(fillers):
                filler()
                if 0 <= i - LAG_S < n_pairs:
                    scores(i - LAG_S)
                if 0 <= i - LAG_M < n_pairs:
                    mix(i - LAG_M)
            o = sum(parts, oproj(done, n_pairs))
            lhs[0:n_mem, :] = _round(o[:n_mem])
            lhs[n_mem:rows, :] = seg_h(jnp.minimum(s + 1, n_seg - 1))
            if phase != "first":
                finish(s, o[n_mem:])
            else:
                x1[0, pl.ds(pl.multiple_of(s * seg, seg), seg), :] = o[n_mem:]
                set_mod(s + 1)
            ffn_down()

        if do_ffn:
            @pl.when(fch == FFN_SEGS - 1)
            def _():
                cp_out(fb).start()

    def run(lo, hi, phase):
        jax.lax.fori_loop(lo, hi, lambda s, _: step(s, phase), None)

    run(0, FFN_SEGS, "first")
    cp_x1.wait()
    cp_mod(5).wait()
    set_mod(5)
    for s in range(FFN_SEGS):
        finish(s, x1[0, s * seg:(s + 1) * seg, :])
    run(FFN_SEGS, 2 * FFN_SEGS, "prep")
    run(2 * FFN_SEGS, n_seg, "both")
    run(n_seg, n_seg + FFN_SEGS, "ffn")
    for b in range(n_blk):
        cp_out(b).wait()


@functools.partial(jax.jit, static_argnames=("A_seg_len",))
def pallas_adaLN_cond__memory_aug_recurrent_mem_tr__glu_gated_swiglu__prompt_kernel(
    A_x, A_mem0, A_Wq, A_Wk, A_Wv, A_Wo, A_seg_len, B_x, B_w1, B_w3, B_w2, c, w_mod,
):
    del B_x
    bsz, s_len, dm = A_x.shape
    _, n_heads, dh = A_Wq.shape
    n_mem = A_mem0.shape[1]
    seg = int(A_seg_len)
    f = B_w1.shape[1]
    fc = f // FFN_SEGS
    kd = (fc - 1) // 256 * 128
    blk = FFN_SEGS * seg
    assert bsz == 1 and s_len % blk == 0 and n_heads % 4 == 0 and fc % 128 == 0 and FFN_SEGS == 4

    hbm = pl.BlockSpec(memory_space=pltpu.MemorySpace.HBM)
    vmem = pl.BlockSpec(memory_space=pltpu.MemorySpace.VMEM)
    scratch = dict(
        wqkv=pltpu.VMEM((3 * n_heads, dm // 2, dh), U32),
        wo=pltpu.VMEM((n_heads * dh // 2, dm), U32),
        wup=pltpu.VMEM((FFN_SEGS, 7, dm // 4, fc), U32),
        wdn=pltpu.VMEM((FFN_SEGS, 7, kd // 2, dm // 2), U32),
        wrest=pltpu.VMEM((FFN_SEGS, fc // 2 - kd, dm), U32),
        wmod=pltpu.VMEM((6, dm // 2, dm), U32),
        stage=pltpu.VMEM((N_STAGE, 3, dm + 8, dh), U32),
        xs=pltpu.VMEM((s_len // seg, seg // 2, dm), U32),
        outs=pltpu.VMEM((s_len // 2, dm), U32),
        mod=pltpu.VMEM((6, 8, dm), F32),
        lhs=pltpu.VMEM((n_mem + seg, dm), F32),
        obuf=pltpu.VMEM((n_mem + seg, n_heads * dh), F32),
        x1=pltpu.VMEM((2, blk, dm), F32),
        h2=pltpu.VMEM((2, 7, blk // 4, dm // 2), U32),
        xpre=pltpu.VMEM((s_len // seg, 8, dm), U32),
        npre=pltpu.VMEM((s_len // seg * PRE_ROWS, dm), F32),
        hpre=pltpu.VMEM((s_len // seg * PRE_ROWS // 2, dm), U32),
        pre=pltpu.VMEM((n_heads // 4 * PRE_TILES, s_len // seg * PRE_ROWS, dh), F32),
        sem_stage=pltpu.SemaphoreType.DMA((3 * N_STAGE,)),
        sem_misc=pltpu.SemaphoreType.DMA((4,)),
        sem_mod=pltpu.SemaphoreType.DMA((6,)),
        sem_ffn=pltpu.SemaphoreType.DMA((9 * FFN_SEGS,)),
        sem_out=pltpu.SemaphoreType.DMA((s_len // blk,)),
    )

    def body(*refs):
        n_io = len(refs) - len(scratch)
        _kernel(*refs[:n_io], **dict(zip(scratch, refs[n_io:])), seg=seg, n_mem=n_mem, dh=dh)

    out = pl.pallas_call(
        body,
        out_shape=jax.ShapeDtypeStruct((s_len, dm), A_x.dtype),
        in_specs=[vmem, vmem] + [hbm] * 9,
        out_specs=hbm,
        scratch_shapes=list(scratch.values()),
        compiler_params=pltpu.CompilerParams(vmem_limit_bytes=124 * 2**20),
    )(c, A_mem0.reshape(n_mem, dm), A_x.reshape(s_len // seg, seg, dm), A_Wq, A_Wk, A_Wv,
      A_Wo.reshape(n_heads * dh, dm), B_w1, B_w3, B_w2, w_mod)
    return out.reshape(bsz, s_len, dm)
```

```python
import functools

import jax
import jax.numpy as jnp
import jax.experimental.pallas as pl
import jax.experimental.pallas.tpu as pltpu

U32 = jnp.uint32
BF16 = jnp.bfloat16
F32 = jnp.float32
LN_EPS = 1e-5
FFN_SEGS = 4
N_STAGE = 5
N_PRE = 9
PRE_ROWS = 8
DOWN_COLS = 128
CMB = 8
LAG_S, LAG_M = 2, 4
X_HEAD = 8


def _bf(w):
    return pltpu.bitcast(w, BF16)


def _words(a):
    return pltpu.bitcast(a.astype(BF16), U32)


def _dot(a, b):
    return jax.lax.dot_general(a, b, (((1,), (0,)), ((), ())), preferred_element_type=F32)


def _dot_nt(a, b):
    return jax.lax.dot_general(a, b, (((1,), (1,)), ((), ())), preferred_element_type=F32)


def _round(a):
    return a.astype(BF16).astype(F32)


def _ln(x):
    m = jnp.mean(x, axis=-1, keepdims=True)
    d = x - m
    v = jnp.mean(d * d, axis=-1, keepdims=True)
    return d * jax.lax.rsqrt(v + LN_EPS)


def _mod_ln(x, scale1, shift):
    return _ln(x) * scale1 + shift


def _strassen_lhs(a11, a12, a21, a22):
    return [a11 + a22, a21 + a22, a11, a22, a11 + a12, a21 - a11, a12 - a22]


def _strassen_out(m):
    return m[0] + m[3] - m[4] + m[6], m[2] + m[4], m[1] + m[3], m[0] - m[1] + m[2] + m[5]


RAW_SLOTS = (1, 2, 3, 4)


def _strassen_rhs(w, c, r, n):
    for k in range(0, w.shape[3], 128):
        at = (pl.ds(r, n), slice(k, k + 128))
        b11, b12, b21, b22 = [_bf(w[(c, i) + at]).astype(F32) for i in RAW_SLOTS]
        for i, t in ((0, b11 + b22), (2, b12 - b22), (3, b21 - b11), (5, b11 + b12), (6, b21 + b22)):
            w[(c, i) + at] = _words(t)


def _kernel(c_ref, mem0_ref, x_hbm, wq_hbm, wk_hbm, wv_hbm, wo_hbm, w1_hbm, w3_hbm, w2_hbm,
            wmod_hbm, out_hbm,
            wqkv, wo, wup, wdn, wrest, wmod, stage, xs, outs, mod, lhs, obuf, x1, h2, xpre, npre, hpre, pre,
            sem_stage, sem_misc, sem_mod, sem_ffn, sem_out, *, seg, n_mem, dh):
    n_pairs = wqkv.shape[0] // 6
    dm = lhs.shape[1]
    rows = n_mem + seg
    hseg = seg // 2
    n_seg = xs.shape[0]
    n_blk = n_seg // FFN_SEGS
    blk = FFN_SEGS * seg
    fc = wup.shape[3]
    kd = 2 * wdn.shape[2]
    hd = dm // 2
    scale = dh ** -0.5

    wmod32 = wmod_hbm.bitcast(U32)
    x32 = x_hbm.bitcast(U32)
    out32 = out_hbm.bitcast(U32)
    qkv32 = [w.bitcast(U32) for w in (wq_hbm, wk_hbm, wv_hbm)]
    hpr = PRE_ROWS // 2
    cp_xpre = pltpu.make_async_copy(x32.at[:, pl.ds(hseg - hpr, hpr), :], xpre.at[:, pl.ds(0, hpr), :],
                                    sem_misc.at[0])
    cp_x0 = pltpu.make_async_copy(x32.at[pl.ds(0, X_HEAD)], xs.at[pl.ds(0, X_HEAD)], sem_misc.at[1])
    cp_x1 = pltpu.make_async_copy(x32.at[pl.ds(X_HEAD, n_seg - X_HEAD)], xs.at[pl.ds(X_HEAD, n_seg - X_HEAD)],
                                  sem_misc.at[2])
    cp_wo = pltpu.make_async_copy(wo_hbm.bitcast(U32), wo, sem_misc.at[3])

    def cp_mod(k):
        return pltpu.make_async_copy(wmod32.at[:, pl.ds(pl.multiple_of(k * dm, dm), dm)], wmod.at[k],
                                     sem_mod.at[k])

    def cp_stage(j):
        slot = j % N_STAGE
        return [pltpu.make_async_copy(qkv32[i].at[:, j, :], stage.at[slot, i, pl.ds(0, dm)],
                                      sem_stage.at[3 * slot + i])
                for i in range(3)]

    def cp_ffn(c):
        cols = pl.ds(pl.multiple_of(c * fc, fc), fc)
        w1_32, w3_32, w2_32 = w1_hbm.bitcast(U32), w3_hbm.bitcast(U32), w2_hbm.bitcast(U32)

        def w2_rows(off, n):
            return pl.ds(pl.multiple_of(c * (fc // 2) + off, 64), n)

        pairs = []
        for i, slot in enumerate(RAW_SLOTS):
            pairs.append(((w1_32, w3_32)[i % 2].at[pl.ds(i // 2 * (hd // 2), hd // 2), cols], wup.at[c, slot]))
            pairs.append((w2_32.at[w2_rows(i // 2 * (kd // 2), kd // 2), pl.ds(i % 2 * hd, hd)], wdn.at[c, slot]))
        pairs.append((w2_32.at[w2_rows(kd, fc // 2 - kd), :], wrest.at[c]))
        return [pltpu.make_async_copy(src, dst, sem_ffn.at[9 * c + i]) for i, (src, dst) in enumerate(pairs)]

    def cp_out(b):
        r = pl.ds(pl.multiple_of(b * (blk // 2), blk // 2), blk // 2)
        return pltpu.make_async_copy(outs.at[r, :], out32.at[r, :], sem_out.at[b])

    cp_xpre.start()
    cp_mod(1).start()
    cp_mod(0).start()
    for j in range(N_STAGE):
        for cp in cp_stage(j):
            cp.start()

    cf = c_ref[...].astype(F32)
    sc = jnp.broadcast_to(_round(cf * jax.nn.sigmoid(cf)), (8, dm))

    def set_mod(k):
        mod[k] = _dot(sc, _bf(wmod[k])) + jnp.where(k % 3 == 1, 1.0, 0.0)

    def get_mod(k, n):
        return jnp.concatenate([mod[k]] * (n // 8), axis=0)

    def seg_x(s):
        return _bf(xs[s]).astype(F32)

    def seg_h(s):
        return _round(_mod_ln(seg_x(s), get_mod(1, seg), get_mod(0, seg)))

    def pre_norm(i, _):
        t = _bf(jnp.concatenate([xpre[2 * i, 0:hpr], xpre[2 * i + 1, 0:hpr]], axis=0)).astype(F32)
        npre[pl.ds(pl.multiple_of(i * 2 * PRE_ROWS, 2 * PRE_ROWS), 2 * PRE_ROWS), :] = _ln(t)

    def pre_mod(i, _):
        t = npre[pl.ds(pl.multiple_of(i * 64, 64), 64), :]
        hpre[pl.ds(pl.multiple_of(i * 32, 32), 32), :] = _words(t * get_mod(1, 64) + get_mod(0, 64))

    cp_xpre.wait()
    jax.lax.fori_loop(0, n_seg // 2, pre_norm, None, unroll=8)
    for k in (1, 0):
        cp_mod(k).wait()
        set_mod(k)
    jax.lax.fori_loop(0, n_seg * PRE_ROWS // 64, pre_mod, None)

    def relayout(j, r, n):
        for i in range(3):
            even, odd = [stage[j % N_STAGE, i, pl.ds(2 * r + k, n, stride=2), :] for k in range(2)]
            wqkv[6 * j + 2 * i, pl.ds(r, n), :] = (even & jnp.uint32(0xFFFF)) | (odd << 16)
            wqkv[6 * j + 2 * i + 1, pl.ds(r, n), :] = (even >> 16) | (odd & jnp.uint32(0xFFFF0000))

    def refill(j):
        @pl.when(j + N_STAGE < n_pairs)
        def _():
            for cp in cp_stage(j + N_STAGE):
                cp.start()

        def queue_rest(*_):
            cp_x0.start()
            cp_wo.start()
            for k in range(2, 6):
                cp_mod(k).start()
            cp_x1.start()

        jax.lax.fori_loop(0, jnp.where(j + N_STAGE == n_pairs, 1, 0), queue_rest, None)

    def pre_proj(i, _):
        j = jnp.minimum(i, n_pairs - 1)

        @pl.when(jnp.logical_and(i > 0, i < n_pairs))
        def _():
            for cp in cp_stage(j):
                cp.wait()

        half = hpre.shape[0] // 2
        a = _bf(hpre[pl.ds(pl.multiple_of(i % 2 * half, half), half), :])
        res = []
        for t in range(6):
            tile = i // 2 * 6 + t
            res.append(_dot(a, _bf(wqkv[tile])))
            pre[tile, pl.ds(pl.multiple_of(i % 2 * 2 * half, 2 * half), 2 * half), :] = res[t]
            if 1 <= t <= 4:
                for g in range(2):
                    stage[j % N_STAGE, 0, pl.ds(pl.multiple_of(dm + i // (2 * N_PRE) * 8, 8), 8), :] = (
                        pltpu.bitcast(res[t - 1][g * half:g * half + 8], U32))
                    relayout(j, (2 * t - 2 + g) * (dm // 16), dm // 16)
        refill(i)

    for cp in cp_stage(0):
        cp.wait()
    jax.lax.fori_loop(0, dm // 128, lambda t, _: relayout(0, pl.multiple_of(t * 64, 64), 64), None)
    jax.lax.fori_loop(0, 2 * N_PRE, pre_proj, None)
    for c in range(FFN_SEGS):
        for cp in cp_ffn(c):
            cp.start()
    cp_x0.wait()
    lhs[0:n_mem, :] = mem0_ref[...].astype(F32)
    lhs[n_mem:rows, :] = seg_h(0)

    def finish(s, attn):
        xn = seg_x(s) + get_mod(2, seg) * attn
        slot = (s >> 2) & 1
        sub = s & 3
        x1[slot, pl.ds(pl.multiple_of(sub * seg, seg), seg), :] = xn
        h = _mod_ln(xn, get_mod(4, seg), get_mod(3, seg))
        for i, t in enumerate(_strassen_lhs(h[:hseg, :hd], h[:hseg, hd:], h[hseg:, :hd], h[hseg:, hd:])):
            h2[slot, i, pl.ds(pl.multiple_of(sub * (hseg // 2), hseg // 2), hseg // 2), :] = _words(t)

    def step(s, phase):
        do_attn = phase != "ffn"
        do_ffn = phase != "first"
        if do_ffn:
            fb = (s >> 2) - 1
            fch = s & 3
            fslot = fb & 1
            act_a, act_b = [], []
        side_work = []
        if phase == "prep":
            for cp in cp_ffn(fch):
                cp.wait()
            side_work = [(wup, r, CMB) for r in range(0, hd // 2, CMB)]
            side_work += [(wdn, r, 2 * CMB) for r in range(0, kd // 2, 2 * CMB)]

        def prepare_weights(i, n, anchor):
            for w, r, size in side_work[len(side_work) * i // n:len(side_work) * (i + 1) // n]:
                w[fch, fb, r:r + 8, 0:128] = pltpu.bitcast(anchor, U32)
                _strassen_rhs(w, fch, r, size)

        def ffn_up(lo, hi):
            if do_ffn:
                for t in range(lo, hi, 128):
                    ga, ua, gb, ub = _strassen_out(
                        [_dot(_bf(h2[fslot, i]), _bf(wup[fch, i, :, t:t + 128])) for i in range(7)])
                    act_a.append(ga * jax.nn.sigmoid(ga) * ua)
                    act_b.append(gb * jax.nn.sigmoid(gb) * ub)

        def ffn_down():
            if do_ffn:
                aa, ab = jnp.concatenate(act_a, axis=1), jnp.concatenate(act_b, axis=1)
                ops = [t.astype(BF16) for t in _strassen_lhs(
                    aa[:, :kd], aa[:, kd:2 * kd], ab[:, :kd], ab[:, kd:2 * kd])]
                rest = _dot(jnp.concatenate([aa[:, 2 * kd:], ab[:, 2 * kd:]], axis=0).astype(BF16),
                            _bf(wrest[fch]))
                for t in range(0, hd, DOWN_COLS):
                    y = _strassen_out([_dot(ops[i], _bf(wdn[fch, i, :, t:t + DOWN_COLS])) for i in range(7)])
                    for side in range(2):
                        cols = slice(side * hd + t, side * hd + t + DOWN_COLS)
                        ya = y[side] + rest[:blk // 2, cols]
                        yb = y[2 + side] + rest[blk // 2:, cols]
                        yy = jnp.concatenate([v[k * hseg:(k + 1) * hseg] for k in range(FFN_SEGS)
                                              for v in (ya, yb)], axis=0)
                        acc = x1[fslot, :, cols] + get_mod(5, blk)[:, cols] * yy
                        x1[fslot, :, cols] = acc
                        outs[pl.ds(pl.multiple_of(fb * (blk // 2), blk // 2), blk // 2), cols] = _words(acc)

        if not do_attn:
            ffn_up(0, fc)
            ffn_down()
        else:
            r = jax.lax.broadcasted_iota(jnp.int32, (2 * rows, 2 * rows), 0)
            q = jax.lax.broadcasted_iota(jnp.int32, (2 * rows, 2 * rows), 1)
            same = (r >= rows) == (q >= rows)
            rl = jnp.where(r >= rows, r - rows, r)
            ql = jnp.where(q >= rows, q - rows, q)
            keep = same & ((rl < n_mem) | (rl >= ql))
            fill = jnp.where(same, -1e9, -jnp.inf).astype(F32)
            a = lhs[...]
            a_short = a[:rows - PRE_ROWS].astype(BF16)
            qkv, probs = {}, {}

            def proj(j):
                t = []
                for tile in range(6 * j, 6 * j + 6):
                    if tile < pre.shape[0]:
                        t.append(jnp.concatenate(
                            [_dot(a_short, _bf(wqkv[tile])),
                             pre[tile, pl.ds(pl.multiple_of(s * PRE_ROWS, PRE_ROWS), PRE_ROWS), :]], axis=0))
                    else:
                        t.append(_dot(a, _bf(wqkv[tile])))
                prepare_weights(j, n_pairs, t[0][0:8])
                qkv[j] = [jnp.concatenate(t[2 * i:2 * i + 2], axis=0).astype(BF16) for i in range(3)]

            def scores(j):
                t = jnp.where(keep, _dot_nt(qkv[j][0], qkv[j][1]) * scale, fill)
                e = jnp.exp(t - jnp.max(t, axis=-1, keepdims=True))
                probs[j] = (e / jnp.sum(e, axis=-1, keepdims=True)).astype(BF16)

            def mix(j):
                o = _round(_dot(probs[j], qkv[j][2]))
                obuf[:, 2 * j * dh:(2 * j + 1) * dh] = o[:rows]
                obuf[:, (2 * j + 1) * dh:(2 * j + 2) * dh] = o[rows:]

            def oproj(lo, hi):
                return _dot(obuf[:, lo * 2 * dh:hi * 2 * dh], _bf(wo[lo * dh:hi * dh, :]))

            def first_waits():
                @pl.when(s == 0)
                def _():
                    cp_wo.wait()

                @pl.when(s > 0)
                def _():
                    cp_mod(s + 1).wait()

            fillers = [functools.partial(proj, j) for j in range(n_pairs)]
            parts = []
            if do_ffn:
                fillers += [functools.partial(ffn_up, t, t + 128) for t in range(0, fc, 128)]
                done = 0
            else:
                fillers.insert(n_pairs - 1, first_waits)
                fillers += [lambda k=k: parts.append(oproj(3 * k, 3 * k + 3)) for k in range(LAG_M)]
                done = 3 * LAG_M
            for i, filler in enumerate(fillers):
                filler()
                if 0 <= i - LAG_S < n_pairs:
                    scores(i - LAG_S)
                if 0 <= i - LAG_M < n_pairs:
                    mix(i - LAG_M)
            o = sum(parts, oproj(done, n_pairs))
            lhs[0:n_mem, :] = _round(o[:n_mem])
            lhs[n_mem:rows, :] = seg_h(jnp.minimum(s + 1, n_seg - 1))
            if phase != "first":
                finish(s, o[n_mem:])
            else:
                x1[0, pl.ds(pl.multiple_of(s * seg, seg), seg), :] = o[n_mem:]
                set_mod(s + 1)
            ffn_down()

        if do_ffn:
            @pl.when(fch == FFN_SEGS - 1)
            def _():
                cp_out(fb).start()

    def run(lo, hi, phase):
        jax.lax.fori_loop(lo, hi, lambda s, _: step(s, phase), None)

    run(0, FFN_SEGS, "first")
    cp_x1.wait()
    cp_mod(5).wait()
    set_mod(5)
    for s in range(FFN_SEGS):
        finish(s, x1[0, s * seg:(s + 1) * seg, :])
    run(FFN_SEGS, 2 * FFN_SEGS, "prep")
    run(2 * FFN_SEGS, n_seg, "both")
    run(n_seg, n_seg + FFN_SEGS, "ffn")
    for b in range(n_blk):
        cp_out(b).wait()


@functools.partial(jax.jit, static_argnames=("A_seg_len",))
def pallas_adaLN_cond__memory_aug_recurrent_mem_tr__glu_gated_swiglu__prompt_kernel(
    A_x, A_mem0, A_Wq, A_Wk, A_Wv, A_Wo, A_seg_len, B_x, B_w1, B_w3, B_w2, c, w_mod,
):
    del B_x
    bsz, s_len, dm = A_x.shape
    _, n_heads, dh = A_Wq.shape
    n_mem = A_mem0.shape[1]
    seg = int(A_seg_len)
    f = B_w1.shape[1]
    fc = f // FFN_SEGS
    kd = (fc - 1) // 256 * 128
    blk = FFN_SEGS * seg
    assert bsz == 1 and s_len % blk == 0 and n_heads % 4 == 0 and fc % 128 == 0 and FFN_SEGS == 4
    assert n_heads // 4 <= N_PRE <= n_heads // 2

    hbm = pl.BlockSpec(memory_space=pltpu.MemorySpace.HBM)
    vmem = pl.BlockSpec(memory_space=pltpu.MemorySpace.VMEM)
    scratch = dict(
        wqkv=pltpu.VMEM((3 * n_heads, dm // 2, dh), U32),
        wo=pltpu.VMEM((n_heads * dh // 2, dm), U32),
        wup=pltpu.VMEM((FFN_SEGS, 7, dm // 4, fc), U32),
        wdn=pltpu.VMEM((FFN_SEGS, 7, kd // 2, dm // 2), U32),
        wrest=pltpu.VMEM((FFN_SEGS, fc // 2 - kd, dm), U32),
        wmod=pltpu.VMEM((6, dm // 2, dm), U32),
        stage=pltpu.VMEM((N_STAGE, 3, dm + 8, dh), U32),
        xs=pltpu.VMEM((s_len // seg, seg // 2, dm), U32),
        outs=pltpu.VMEM((s_len // 2, dm), U32),
        mod=pltpu.VMEM((6, 8, dm), F32),
        lhs=pltpu.VMEM((n_mem + seg, dm), F32),
        obuf=pltpu.VMEM((n_mem + seg, n_heads * dh), F32),
        x1=pltpu.VMEM((2, blk, dm), F32),
        h2=pltpu.VMEM((2, 7, blk // 4, dm // 2), U32),
        xpre=pltpu.VMEM((s_len // seg, 8, dm), U32),
        npre=pltpu.VMEM((s_len // seg * PRE_ROWS, dm), F32),
        hpre=pltpu.VMEM((s_len // seg * PRE_ROWS // 2, dm), U32),
        pre=pltpu.VMEM((6 * N_PRE, s_len // seg * PRE_ROWS, dh), F32),
        sem_stage=pltpu.SemaphoreType.DMA((3 * N_STAGE,)),
        sem_misc=pltpu.SemaphoreType.DMA((4,)),
        sem_mod=pltpu.SemaphoreType.DMA((6,)),
        sem_ffn=pltpu.SemaphoreType.DMA((9 * FFN_SEGS,)),
        sem_out=pltpu.SemaphoreType.DMA((s_len // blk,)),
    )

    def body(*refs):
        n_io = len(refs) - len(scratch)
        _kernel(*refs[:n_io], **dict(zip(scratch, refs[n_io:])), seg=seg, n_mem=n_mem, dh=dh)

    out = pl.pallas_call(
        body,
        out_shape=jax.ShapeDtypeStruct((s_len, dm), A_x.dtype),
        in_specs=[vmem, vmem] + [hbm] * 9,
        out_specs=hbm,
        scratch_shapes=list(scratch.values()),
        compiler_params=pltpu.CompilerParams(
            vmem_limit_bytes=124 * 2**20,
            flags={"XLA_TPU_EVENLY_DISTRIBUTE_CRITICAL_NODES": True}),
    )(c, A_mem0.reshape(n_mem, dm), A_x.reshape(s_len // seg, seg, dm), A_Wq, A_Wk, A_Wv,
      A_Wo.reshape(n_heads * dh, dm), B_w1, B_w3, B_w2, w_mod)
    return out.reshape(bsz, s_len, dm)
```

```python
import functools

import jax
import jax.numpy as jnp
import jax.experimental.pallas as pl
import jax.experimental.pallas.tpu as pltpu

U32 = jnp.uint32
BF16 = jnp.bfloat16
F32 = jnp.float32
LN_EPS = 1e-5
FFN_SEGS = 4
N_STAGE = 5
N_PRE = 9
PRE_ROWS = 8
DOWN_COLS = 128
N_MOD = 5
LAG_S, LAG_M = 2, 4
X_HEAD = 8


def _bf(w):
    return pltpu.bitcast(w, BF16)


def _words(a):
    return pltpu.bitcast(a.astype(BF16), U32)


def _dot(a, b):
    return jax.lax.dot_general(a, b, (((1,), (0,)), ((), ())), preferred_element_type=F32)


def _dot_nt(a, b):
    return jax.lax.dot_general(a, b, (((1,), (1,)), ((), ())), preferred_element_type=F32)


def _round(a):
    return a.astype(BF16).astype(F32)


def _ln(x):
    m = jnp.mean(x, axis=-1, keepdims=True)
    d = x - m
    v = jnp.mean(d * d, axis=-1, keepdims=True)
    return d * jax.lax.rsqrt(v + LN_EPS)


def _mod_ln(x, scale1, shift):
    return _ln(x) * scale1 + shift


def _strassen_lhs(a11, a12, a21, a22):
    return [a11 + a22, a21 + a22, a11, a22, a11 + a12, a21 - a11, a12 - a22]


def _strassen_out(m):
    return m[0] + m[3] - m[4] + m[6], m[2] + m[4], m[1] + m[3], m[0] - m[1] + m[2] + m[5]


def _strassen_rhs(b11, b12, b21, b22):
    return [b11 + b22, b11, b12 - b22, b21 - b11, b22, b11 + b12, b21 + b22]


PLACE = (0, 1, 3, 2, 4, 5, 6)
RAW = (1, 2, 3, 4)
KEPT = (1, 4)


def _operand(w, i, r=0, n=None):
    size = w.shape[-2] // 7
    return pl.ds(PLACE[i] * size + r, size if n is None else n)


def _halves(w):
    return pltpu.bitcast(jnp.concatenate([w << 16, w & jnp.uint32(0xFFFF0000)], axis=0), F32)


def _join(t):
    u = pltpu.bitcast(t, U32)
    n = u.shape[0] // 2
    return ((u[:n] + jnp.uint32(0x8000)) >> 16) | ((u[n:] + jnp.uint32(0x7FFF)) & jnp.uint32(0xFFFF0000))


def _prepare_one_level(w, c, r, n, k):
    raw = [_halves(w[c, 0, _operand(w, i, r, n), k:k + 128]) for i in RAW]
    for i, t in enumerate(_strassen_rhs(*raw)):
        if i not in KEPT:
            w[c, 0, _operand(w, i, r, n), k:k + 128] = _join(t)


def _prepare_two_levels(w, c, r, n, k):
    outer = [_strassen_rhs(*[_halves(w[c, i, _operand(w, j, r, n), k:k + 128]) for i in RAW]) for j in RAW]
    for i in range(7):
        for j, t in enumerate(_strassen_rhs(*[sub[i] for sub in outer])):
            if i not in KEPT or j not in KEPT:
                w[c, i, _operand(w, j, r, n), k:k + 128] = _join(t)


def _kernel(c_ref, mem0_ref, x_hbm, wq_hbm, wk_hbm, wv_hbm, wo_hbm, w1_hbm, w3_hbm, w2_hbm,
            wmod_hbm, out_hbm,
            wqkv, wo, wup2, wup1, wdn, wrest, wmod, stage, xs, mod, lhs, obuf, x1, h2, hpre, pre,
            sem_stage, sem_misc, sem_mod, sem_ffn, sem_out, *, seg, n_mem, dh):
    n_pairs = wqkv.shape[0] // 6
    dm = lhs.shape[1]
    rows = n_mem + seg
    hseg = seg // 2
    n_seg = xs.shape[0]
    n_blk = n_seg // FFN_SEGS
    blk = FFN_SEGS * seg
    fq = wup2.shape[3]
    fc = 2 * fq + wup1.shape[3]
    kd = 2 * wdn.shape[2] // 7
    hd = dm // 2
    scale = dh ** -0.5

    wmod32 = wmod_hbm.bitcast(U32)
    x32 = x_hbm.bitcast(U32)
    out32 = out_hbm.bitcast(U32)
    qkv32 = [w.bitcast(U32) for w in (wq_hbm, wk_hbm, wv_hbm)]
    hpr = PRE_ROWS // 2
    tail = pl.ds(hseg - hpr, hpr)
    cp_xpre = pltpu.make_async_copy(x32.at[:, tail, :], xs.at[:, tail, :], sem_misc.at[0])
    cp_x0 = pltpu.make_async_copy(x32.at[pl.ds(0, X_HEAD)], xs.at[pl.ds(0, X_HEAD)], sem_misc.at[1])
    cp_x1 = pltpu.make_async_copy(x32.at[pl.ds(X_HEAD, n_seg - X_HEAD)], xs.at[pl.ds(X_HEAD, n_seg - X_HEAD)],
                                  sem_misc.at[2])
    cp_wo = pltpu.make_async_copy(wo_hbm.bitcast(U32), wo, sem_misc.at[3])

    def cp_mod(k):
        return pltpu.make_async_copy(wmod32.at[:, pl.ds(pl.multiple_of(k * dm, dm), dm)], wmod.at[k % N_MOD],
                                     sem_mod.at[k])

    def cp_stage(j):
        slot = j % N_STAGE
        return [pltpu.make_async_copy(qkv32[i].at[:, j, :], stage.at[slot, i, pl.ds(0, dm)],
                                      sem_stage.at[3 * slot + i])
                for i in range(3)]

    def cp_ffn(c):
        w1_32, w3_32, w2_32 = w1_hbm.bitcast(U32), w3_hbm.bitcast(U32), w2_hbm.bitcast(U32)

        def up_cols(off, n):
            return pl.ds(pl.multiple_of(c * fc + off, 128), n)

        def w2_rows(off, n):
            return pl.ds(pl.multiple_of(c * (fc // 2) + off, 64), n)

        pairs = []
        for side, w in enumerate((w1_32, w3_32)):
            for i in range(2):
                for j in range(2):
                    pairs.append((w.at[pl.ds(i * (hd // 2), hd // 2), up_cols(j * fq, fq)],
                                  wup2.at[c, RAW[2 * i + side], _operand(wup2, RAW[j], 0, hd // 2)]))
            pairs.append((w.at[:, up_cols(2 * fq, fc - 2 * fq)], wup1.at[c, 0, _operand(wup1, RAW[side], 0, hd)]))
            pairs.append((w2_32.at[w2_rows(0, kd), pl.ds(side * hd, hd)],
                          wdn.at[c, 0, _operand(wdn, RAW[side], 0, kd)]))
        pairs.append((w2_32.at[w2_rows(kd, fc // 2 - kd), :], wrest.at[c]))
        return [pltpu.make_async_copy(src, dst, sem_ffn.at[c]) for src, dst in pairs]

    def cp_out(b):
        r = pl.ds(b * FFN_SEGS, FFN_SEGS)
        return pltpu.make_async_copy(xs.at[r], out32.at[r], sem_out.at[b])

    cp_xpre.start()
    cp_mod(1).start()
    cp_mod(0).start()
    for j in range(N_STAGE):
        for cp in cp_stage(j):
            cp.start()

    cf = c_ref[...].astype(F32)
    sc = jnp.broadcast_to(_round(cf * jax.nn.sigmoid(cf)), (8, dm))

    def set_mod(k):
        mod[k] = _dot(sc, _bf(wmod[k % N_MOD])) + jnp.where(k % 3 == 1, 1.0, 0.0)

    def get_mod(k, n):
        return jnp.concatenate([mod[k]] * (n // 8), axis=0)

    def seg_x(s):
        return _bf(xs[s]).astype(F32)

    def seg_h(s):
        return _round(_mod_ln(seg_x(s), get_mod(1, seg), get_mod(0, seg)))

    parked = pre.shape[0] - dm // dh

    def pre_norm(i, _):
        t = _ln(_bf(jnp.concatenate([xs[2 * i, tail], xs[2 * i + 1, tail]], axis=0)).astype(F32))
        for k in range(dm // dh):
            pre[parked + k, pl.ds(pl.multiple_of(i * 2 * PRE_ROWS, 2 * PRE_ROWS), 2 * PRE_ROWS), :] = (
                t[:, k * dh:(k + 1) * dh])

    def pre_mod(i, _):
        t = jnp.concatenate([pre[parked + k, pl.ds(pl.multiple_of(i * 64, 64), 64), :]
                             for k in range(dm // dh)], axis=1)
        hpre[pl.ds(pl.multiple_of(i * 32, 32), 32), :] = _words(t * get_mod(1, 64) + get_mod(0, 64))

    cp_xpre.wait()
    jax.lax.fori_loop(0, n_seg // 2, pre_norm, None, unroll=8)
    for k in (1, 0):
        cp_mod(k).wait()
        set_mod(k)
    jax.lax.fori_loop(0, n_seg * PRE_ROWS // 64, pre_mod, None)

    def relayout(j, r, n):
        for i in range(3):
            even, odd = [stage[j % N_STAGE, i, pl.ds(2 * r + k, n, stride=2), :] for k in range(2)]
            wqkv[6 * j + 2 * i, pl.ds(r, n), :] = (even & jnp.uint32(0xFFFF)) | (odd << 16)
            wqkv[6 * j + 2 * i + 1, pl.ds(r, n), :] = (even >> 16) | (odd & jnp.uint32(0xFFFF0000))

    def refill(j):
        @pl.when(j + N_STAGE < n_pairs)
        def _():
            for cp in cp_stage(j + N_STAGE):
                cp.start()

        def queue_rest(*_):
            cp_x0.start()
            cp_wo.start()
            for k in range(2, 6):
                cp_mod(k).start()
            cp_x1.start()

        jax.lax.fori_loop(0, jnp.where(j + N_STAGE == n_pairs, 1, 0), queue_rest, None)

    def pre_proj(i, _):
        j = jnp.minimum(i, n_pairs - 1)

        @pl.when(jnp.logical_and(i > 0, i < n_pairs))
        def _():
            for cp in cp_stage(j):
                cp.wait()

        half = hpre.shape[0] // 2
        a = _bf(hpre[pl.ds(pl.multiple_of(i % 2 * half, half), half), :])
        res = []
        for t in range(6):
            tile = i // 2 * 6 + t
            res.append(_dot(a, _bf(wqkv[tile])))
            pre[tile, pl.ds(pl.multiple_of(i % 2 * 2 * half, 2 * half), 2 * half), :] = res[t]
            if 1 <= t <= 4:
                for g in range(2):
                    stage[j % N_STAGE, 0, pl.ds(pl.multiple_of(dm + i // (2 * N_PRE) * 8, 8), 8), :] = (
                        pltpu.bitcast(res[t - 1][g * half:g * half + 8], U32))
                    relayout(j, (2 * t - 2 + g) * (dm // 16), dm // 16)
        refill(i)

    for cp in cp_stage(0):
        cp.wait()
    jax.lax.fori_loop(0, dm // 128, lambda t, _: relayout(0, pl.multiple_of(t * 64, 64), 64), None)
    jax.lax.fori_loop(0, 2 * N_PRE, pre_proj, None)
    cp_x0.wait()
    lhs[0:n_mem, :] = mem0_ref[...].astype(F32)
    lhs[n_mem:rows, :] = seg_h(0)

    def finish(s, attn):
        xn = seg_x(s) + get_mod(2, seg) * attn
        slot = (s >> 2) & 1
        sub = s & 3
        x1[slot, pl.ds(pl.multiple_of(sub * seg, seg), seg), :] = xn
        h = _mod_ln(xn, get_mod(4, seg), get_mod(3, seg))
        for i, t in enumerate(_strassen_lhs(h[:hseg, :hd], h[:hseg, hd:], h[hseg:, :hd], h[hseg:, hd:])):
            h2[slot, i, pl.ds(pl.multiple_of(sub * hseg, hseg), hseg), :] = t

    def step(s, phase):
        do_attn = phase != "ffn"
        do_ffn = phase != "first"
        if do_ffn:
            fb = (s >> 2) - 1
            fch = s & 3
            fslot = fb & 1
            act_a, act_b = [None] * (2 * (fq // 128) + 1), [None] * (2 * (fq // 128) + 1)
        up_work, down_work = [], []
        if phase == "first":
            for cp in cp_ffn(s):
                cp.start()
        if phase == "prep":
            for cp in cp_ffn(fch):
                cp.wait()
            up_work = [(_prepare_two_levels, wup2, r, 8, k)
                       for k in range(0, fq, 128) for r in range(0, hd // 4, 8)]
            down_work = [(_prepare_one_level, w, r, 32, k) for w in (wup1, wdn)
                         for k in range(0, w.shape[3], 128) for r in range(0, w.shape[2] // 7, 32)]

        def prepare_weights(work, i, n, anchor):
            todo = work[-(-len(work) * i // n):-(-len(work) * (i + 1) // n)]
            for _, w, r, _, k in todo[:1]:
                w[fch, fb, r:r + 8, k:k + 128] = pltpu.bitcast(anchor, U32)
            for prepare, w, r, size, k in todo:
                prepare(w, fch, r, size, k)

        nq = fq // 128
        inner_ops = []

        def gate(t, products):
            ga, ua, gb, ub = _strassen_out(products)
            act_a[t] = ga * jax.nn.sigmoid(ga) * ua
            act_b[t] = gb * jax.nn.sigmoid(gb) * ub

        def ffn_up(t):
            if t == nq:
                gate(2 * nq, [_dot(h2[fslot, i].astype(BF16), _bf(wup1[fch, 0, _operand(wup1, i), :])) for i in range(7)])
                return
            if not inner_ops:
                for i in range(7):
                    h = h2[fslot, i]
                    inner_ops.append([v.astype(BF16) for v in _strassen_lhs(
                        h[:seg, :hd // 2], h[:seg, hd // 2:], h[seg:, :hd // 2], h[seg:, hd // 2:])])
            left, right = [], []
            for i in range(7):
                c11, c12, c21, c22 = _strassen_out(
                    [_dot(inner_ops[i][j], _bf(wup2[fch, i, _operand(wup2, j), t * 128:(t + 1) * 128]))
                     for j in range(7)])
                left.append(jnp.concatenate([c11, c21], axis=0))
                right.append(jnp.concatenate([c12, c22], axis=0))
            gate(t, left)
            gate(nq + t, right)

        def ffn_down():
            if do_ffn:
                aa, ab = jnp.concatenate(act_a, axis=1), jnp.concatenate(act_b, axis=1)
                ops = [t.astype(BF16) for t in _strassen_lhs(
                    aa[:, :kd], aa[:, kd:2 * kd], ab[:, :kd], ab[:, kd:2 * kd])]
                rest = _dot(jnp.concatenate([aa[:, 2 * kd:], ab[:, 2 * kd:]], axis=0).astype(BF16),
                            _bf(wrest[fch]))
                for t in range(0, hd, DOWN_COLS):
                    y = _strassen_out([_dot(ops[i], _bf(wdn[fch, 0, _operand(wdn, i), t:t + DOWN_COLS]))
                                       for i in range(7)])
                    for side in range(2):
                        cols = slice(side * hd + t, side * hd + t + DOWN_COLS)
                        ya = y[side] + rest[:blk // 2, cols]
                        yb = y[2 + side] + rest[blk // 2:, cols]
                        yy = jnp.concatenate([v[k * hseg:(k + 1) * hseg] for k in range(FFN_SEGS)
                                              for v in (ya, yb)], axis=0)
                        acc = x1[fslot, :, cols] + get_mod(5, blk)[:, cols] * yy
                        x1[fslot, :, cols] = acc
                        for k in range(FFN_SEGS):
                            xs[fb * FFN_SEGS + k, :, cols] = _words(acc[k * seg:(k + 1) * seg])

        if not do_attn:
            for t in range(nq + 1):
                ffn_up(t)
            ffn_down()
        else:
            r = jax.lax.broadcasted_iota(jnp.int32, (2 * rows, 2 * rows), 0)
            q = jax.lax.broadcasted_iota(jnp.int32, (2 * rows, 2 * rows), 1)
            same = (r >= rows) == (q >= rows)
            rl = jnp.where(r >= rows, r - rows, r)
            ql = jnp.where(q >= rows, q - rows, q)
            keep = same & ((rl < n_mem) | (rl >= ql))
            fill = jnp.where(same, -1e9, -jnp.inf).astype(F32)
            a = lhs[...]
            a_short = a[:rows - PRE_ROWS].astype(BF16)
            qkv, probs = {}, {}

            def proj(j):
                t = []
                for tile in range(6 * j, 6 * j + 6):
                    if tile < pre.shape[0]:
                        t.append(jnp.concatenate(
                            [_dot(a_short, _bf(wqkv[tile])),
                             pre[tile, pl.ds(pl.multiple_of(s * PRE_ROWS, PRE_ROWS), PRE_ROWS), :]], axis=0))
                    else:
                        t.append(_dot(a, _bf(wqkv[tile])))
                prepare_weights(up_work, j, n_pairs, t[0][0:8])
                qkv[j] = [jnp.concatenate(t[2 * i:2 * i + 2], axis=0).astype(BF16) for i in range(3)]

            def scores(j):
                t = jnp.where(keep, _dot_nt(qkv[j][0], qkv[j][1]) * scale, fill)
                e = jnp.exp(t - jnp.max(t, axis=-1, keepdims=True))
                probs[j] = (e / jnp.sum(e, axis=-1, keepdims=True)).astype(BF16)

            def mix(j):
                o = _round(_dot(probs[j], qkv[j][2]))
                obuf[:, 2 * j * dh:(2 * j + 1) * dh] = o[:rows]
                obuf[:, (2 * j + 1) * dh:(2 * j + 2) * dh] = o[rows:]

            def oproj(lo, hi):
                return _dot(obuf[:, lo * 2 * dh:hi * 2 * dh], _bf(wo[lo * dh:hi * dh, :]))

            def oproj_part(k):
                parts.append(oproj(3 * k, 3 * k + 3))
                prepare_weights(down_work, k, LAG_M, parts[k][0:8, 0:128])

            def first_waits():
                @pl.when(s == 0)
                def _():
                    cp_wo.wait()

                @pl.when(s > 0)
                def _():
                    cp_mod(s + 1).wait()

            fillers = [functools.partial(proj, j) for j in range(n_pairs)]
            parts = []
            if phase == "both":
                fillers += [functools.partial(ffn_up, t) for t in range(nq + 1)]
                done = 0
            else:
                if phase == "first":
                    fillers.insert(n_pairs - 1, first_waits)
                fillers += [functools.partial(oproj_part, k) for k in range(LAG_M)]
                done = 3 * LAG_M
            for i, filler in enumerate(fillers):
                filler()
                if 0 <= i - LAG_S < n_pairs:
                    scores(i - LAG_S)
                if 0 <= i - LAG_M < n_pairs:
                    mix(i - LAG_M)
            if phase == "prep":
                for t in range(nq + 1):
                    ffn_up(t)
            o = sum(parts, oproj(done, n_pairs))
            lhs[0:n_mem, :] = _round(o[:n_mem])
            lhs[n_mem:rows, :] = seg_h(jnp.minimum(s + 1, n_seg - 1))
            if phase != "first":
                finish(s, o[n_mem:])
            else:
                x1[0, pl.ds(pl.multiple_of(s * seg, seg), seg), :] = o[n_mem:]
                set_mod(s + 1)
            ffn_down()

        if do_ffn:
            @pl.when(fch == FFN_SEGS - 1)
            def _():
                cp_out(fb).start()

    def run(lo, hi, phase):
        jax.lax.fori_loop(lo, hi, lambda s, _: step(s, phase), None)

    run(0, FFN_SEGS, "first")
    cp_x1.wait()
    cp_mod(5).wait()
    set_mod(5)
    for s in range(FFN_SEGS):
        finish(s, x1[0, s * seg:(s + 1) * seg, :])
    run(FFN_SEGS, 2 * FFN_SEGS, "prep")
    run(2 * FFN_SEGS, n_seg, "both")
    run(n_seg, n_seg + FFN_SEGS, "ffn")
    for b in range(n_blk):
        cp_out(b).wait()


@functools.partial(jax.jit, static_argnames=("A_seg_len",))
def pallas_adaLN_cond__memory_aug_recurrent_mem_tr__glu_gated_swiglu__prompt_kernel(
    A_x, A_mem0, A_Wq, A_Wk, A_Wv, A_Wo, A_seg_len, B_x, B_w1, B_w3, B_w2, c, w_mod,
):
    del B_x
    bsz, s_len, dm = A_x.shape
    _, n_heads, dh = A_Wq.shape
    n_mem = A_mem0.shape[1]
    seg = int(A_seg_len)
    f = B_w1.shape[1]
    fc = f // FFN_SEGS
    kd = (fc - 1) // 256 * 128
    blk = FFN_SEGS * seg
    assert bsz == 1 and s_len % blk == 0 and n_heads % 4 == 0 and fc % 128 == 0 and FFN_SEGS == 4
    assert n_heads // 4 <= N_PRE <= n_heads // 2

    hbm = pl.BlockSpec(memory_space=pltpu.MemorySpace.HBM)
    vmem = pl.BlockSpec(memory_space=pltpu.MemorySpace.VMEM)
    scratch = dict(
        wqkv=pltpu.VMEM((3 * n_heads, dm // 2, dh), U32),
        wo=pltpu.VMEM((n_heads * dh // 2, dm), U32),
        wup2=pltpu.VMEM((FFN_SEGS, 7, 7 * dm // 8, kd), U32),
        wup1=pltpu.VMEM((FFN_SEGS, 1, 7 * dm // 4, fc - 2 * kd), U32),
        wdn=pltpu.VMEM((FFN_SEGS, 1, 7 * kd // 2, dm // 2), U32),
        wrest=pltpu.VMEM((FFN_SEGS, fc // 2 - kd, dm), U32),
        wmod=pltpu.VMEM((N_MOD, dm // 2, dm), U32),
        stage=pltpu.VMEM((N_STAGE, 3, dm + 8, dh), U32),
        xs=pltpu.VMEM((s_len // seg, seg // 2, dm), U32),
        mod=pltpu.VMEM((6, 8, dm), F32),
        lhs=pltpu.VMEM((n_mem + seg, dm), F32),
        obuf=pltpu.VMEM((n_mem + seg, n_heads * dh), F32),
        x1=pltpu.VMEM((2, blk, dm), F32),
        h2=pltpu.VMEM((2, 7, blk // 2, dm // 2), F32),
        hpre=pltpu.VMEM((s_len // seg * PRE_ROWS // 2, dm), U32),
        pre=pltpu.VMEM((6 * N_PRE, s_len // seg * PRE_ROWS, dh), F32),
        sem_stage=pltpu.SemaphoreType.DMA((3 * N_STAGE,)),
        sem_misc=pltpu.SemaphoreType.DMA((4,)),
        sem_mod=pltpu.SemaphoreType.DMA((6,)),
        sem_ffn=pltpu.SemaphoreType.DMA((FFN_SEGS,)),
        sem_out=pltpu.SemaphoreType.DMA((s_len // blk,)),
    )

    def body(*refs):
        n_io = len(refs) - len(scratch)
        _kernel(*refs[:n_io], **dict(zip(scratch, refs[n_io:])), seg=seg, n_mem=n_mem, dh=dh)

    out = pl.pallas_call(
        body,
        out_shape=jax.ShapeDtypeStruct((s_len // seg, seg, dm), A_x.dtype),
        in_specs=[vmem, vmem] + [hbm] * 9,
        out_specs=hbm,
        scratch_shapes=list(scratch.values()),
        compiler_params=pltpu.CompilerParams(
            vmem_limit_bytes=127 * 2**20,
            flags={"XLA_TPU_EVENLY_DISTRIBUTE_CRITICAL_NODES": True}),
    )(c, A_mem0.reshape(n_mem, dm), A_x.reshape(s_len // seg, seg, dm), A_Wq, A_Wk, A_Wv,
      A_Wo.reshape(n_heads * dh, dm), B_w1, B_w3, B_w2, w_mod)
    return out.reshape(bsz, s_len, dm)
```

```python
import functools

import jax
import jax.numpy as jnp
import numpy as np
import jax.experimental.pallas as pl
import jax.experimental.pallas.tpu as pltpu

U32 = jnp.uint32
BF16 = jnp.bfloat16
F32 = jnp.float32
LN_EPS = 1e-5
FFN_SEGS = 4
N_STAGE = 4
N_PRE = 9
PRE_ROWS = 8
DOWN_COLS = 512
N_MOD = 5
LAG_S, LAG_M = 2, 4
X_HEAD = 8


def _bf(w):
    return pltpu.bitcast(w, BF16)


def _words(a):
    return pltpu.bitcast(a.astype(BF16), U32)


def _dot(a, b):
    return jax.lax.dot_general(a, b, (((1,), (0,)), ((), ())), preferred_element_type=F32)


def _dot_nt(a, b):
    return jax.lax.dot_general(a, b, (((1,), (1,)), ((), ())), preferred_element_type=F32)


def _round(a):
    return a.astype(BF16).astype(F32)


def _ln(x):
    m = jnp.mean(x, axis=-1, keepdims=True)
    d = x - m
    v = jnp.mean(d * d, axis=-1, keepdims=True)
    return d * jax.lax.rsqrt(v + LN_EPS)


def _mod_ln(x, scale1, shift):
    return _ln(x) * scale1 + shift


def _strassen_lhs(a11, a12, a21, a22):
    return [a11 + a22, a21 + a22, a11, a22, a11 + a12, a21 - a11, a12 - a22]


def _strassen_out(m):
    return m[0] + m[3] - m[4] + m[6], m[2] + m[4], m[1] + m[3], m[0] - m[1] + m[2] + m[5]


def _strassen_rhs(b11, b12, b21, b22):
    return [b11 + b22, b11, b12 - b22, b21 - b11, b22, b11 + b12, b21 + b22]


PLACE = (0, 1, 3, 2, 4, 5, 6)
RAW = (1, 2, 3, 4)
KEPT = (1, 4)


def _operand(w, i, r=0, n=None):
    size = w.shape[-2] // 7
    return pl.ds(PLACE[i] * size + r, size if n is None else n)


def _halves(w):
    return pltpu.bitcast(jnp.concatenate([w << 16, w & np.uint32(0xFFFF0000)], axis=0), F32)


def _join(t):
    u = pltpu.bitcast(t, U32)
    n = u.shape[0] // 2
    return ((u[:n] + np.uint32(0x8000)) >> 16) | ((u[n:] + np.uint32(0x7FFF)) & np.uint32(0xFFFF0000))


def _prepare_one_level(w, c, r, n, k):
    raw = [_halves(w[c, 0, _operand(w, i, r, n), k:k + 128]) for i in RAW]
    for i, t in enumerate(_strassen_rhs(*raw)):
        if i not in KEPT:
            w[c, 0, _operand(w, i, r, n), k:k + 128] = _join(t)


def _prepare_two_levels(w, c, r, n, k):
    outer = [_strassen_rhs(*[_halves(w[c, i, _operand(w, j, r, n), k:k + 128]) for i in RAW]) for j in RAW]
    for i in range(7):
        for j, t in enumerate(_strassen_rhs(*[sub[i] for sub in outer])):
            if i not in KEPT or j not in KEPT:
                w[c, i, _operand(w, j, r, n), k:k + 128] = _join(t)


def _kernel(c_ref, mem0_ref, x_hbm, wq_hbm, wk_hbm, wv_hbm, wo_hbm, w1_hbm, w3_hbm, w2_hbm,
            wmod_hbm, out_hbm,
            wqkv, wo, wup2, wup1, wdn, wrest, wmod, stage, xs, mod, lhs, obuf, x1, h2, hpre, pre,
            sem_stage, sem_misc, sem_mod, sem_ffn, sem_out, *, seg, n_mem, dh):
    n_pairs = wqkv.shape[0] // 6
    dm = lhs.shape[1]
    rows = n_mem + seg
    hseg = seg // 2
    n_seg = xs.shape[0]
    n_blk = n_seg // FFN_SEGS
    blk = FFN_SEGS * seg
    fq = wup2.shape[3]
    fc = 2 * fq + wup1.shape[3]
    kd = 2 * wdn.shape[2] // 7
    hd = dm // 2
    scale = dh ** -0.5

    wmod32 = wmod_hbm.bitcast(U32)
    x32 = x_hbm.bitcast(U32)
    out32 = out_hbm.bitcast(U32)
    qkv32 = [w.bitcast(U32) for w in (wq_hbm, wk_hbm, wv_hbm)]
    hpr = PRE_ROWS // 2
    tail = pl.ds(hseg - hpr, hpr)
    cp_xpre = pltpu.make_async_copy(x32.at[:, tail, :], xs.at[:, tail, :], sem_misc.at[0])
    cp_x0 = pltpu.make_async_copy(x32.at[pl.ds(0, X_HEAD)], xs.at[pl.ds(0, X_HEAD)], sem_misc.at[1])
    cp_x1 = pltpu.make_async_copy(x32.at[pl.ds(X_HEAD, n_seg - X_HEAD)], xs.at[pl.ds(X_HEAD, n_seg - X_HEAD)],
                                  sem_misc.at[2])
    cp_wo = pltpu.make_async_copy(wo_hbm.bitcast(U32), wo, sem_misc.at[3])

    def cp_mod(k):
        return pltpu.make_async_copy(wmod32.at[:, pl.ds(pl.multiple_of(k * dm, dm), dm)], wmod.at[k % N_MOD],
                                     sem_mod.at[k])

    def cp_stage(j):
        slot = j & (N_STAGE - 1)
        return [pltpu.make_async_copy(qkv32[i].at[:, j, :], stage.at[slot, i, pl.ds(0, dm)],
                                      sem_stage.at[3 * slot + i])
                for i in range(3)]

    def cp_ffn(c):
        w1_32, w3_32, w2_32 = w1_hbm.bitcast(U32), w3_hbm.bitcast(U32), w2_hbm.bitcast(U32)

        def up_cols(off, n):
            return pl.ds(pl.multiple_of(c * fc + off, 128), n)

        def w2_rows(off, n):
            return pl.ds(pl.multiple_of(c * (fc // 2) + off, 64), n)

        pairs = []
        for side, w in enumerate((w1_32, w3_32)):
            for i in range(2):
                for j in range(2):
                    pairs.append((w.at[pl.ds(i * (hd // 2), hd // 2), up_cols(j * fq, fq)],
                                  wup2.at[c, RAW[2 * i + side], _operand(wup2, RAW[j], 0, hd // 2)]))
            pairs.append((w.at[:, up_cols(2 * fq, fc - 2 * fq)], wup1.at[c, 0, _operand(wup1, RAW[side], 0, hd)]))
            pairs.append((w2_32.at[w2_rows(0, kd), pl.ds(side * hd, hd)],
                          wdn.at[c, 0, _operand(wdn, RAW[side], 0, kd)]))
        pairs.append((w2_32.at[w2_rows(kd, fc // 2 - kd), :], wrest.at[c]))
        return [pltpu.make_async_copy(src, dst, sem_ffn.at[c]) for src, dst in pairs]

    def cp_out(b):
        r = pl.ds(b * FFN_SEGS, FFN_SEGS)
        return pltpu.make_async_copy(xs.at[r], out32.at[r], sem_out.at[b])

    cp_xpre.start()
    cp_mod(1).start()
    cp_mod(0).start()
    for j in range(N_STAGE):
        for cp in cp_stage(j):
            cp.start()

    cf = c_ref[...].astype(F32)
    sc = jnp.broadcast_to(_round(cf * jax.nn.sigmoid(cf)), (8, dm))

    def set_mod(k):
        mod[k] = _dot(sc, _bf(wmod[k % N_MOD])) + jnp.where(k % 3 == 1, 1.0, 0.0)

    def get_mod(k, n):
        return jnp.concatenate([mod[k]] * (n // 8), axis=0)

    def seg_x(s):
        return _bf(xs[s]).astype(F32)

    def seg_h(s):
        return _round(_mod_ln(seg_x(s), get_mod(1, seg), get_mod(0, seg)))

    parked = pre.shape[0] - dm // dh

    def pre_norm(i, _):
        t = _ln(_bf(jnp.concatenate([xs[2 * i, tail], xs[2 * i + 1, tail]], axis=0)).astype(F32))
        for k in range(dm // dh):
            pre[parked + k, pl.ds(pl.multiple_of(i * 2 * PRE_ROWS, 2 * PRE_ROWS), 2 * PRE_ROWS), :] = (
                t[:, k * dh:(k + 1) * dh])

    def pre_mod(i, _):
        t = jnp.concatenate([pre[parked + k, pl.ds(pl.multiple_of(i * 64, 64), 64), :]
                             for k in range(dm // dh)], axis=1)
        hpre[pl.ds(pl.multiple_of(i * 32, 32), 32), :] = _words(t * get_mod(1, 64) + get_mod(0, 64))

    cp_xpre.wait()
    jax.lax.fori_loop(0, n_seg // 2, pre_norm, None, unroll=8)
    for k in (1, 0):
        cp_mod(k).wait()
        set_mod(k)
    jax.lax.fori_loop(0, n_seg * PRE_ROWS // 64, pre_mod, None)

    def relayout(j, r, n):
        for i in range(3):
            even, odd = [stage[j & (N_STAGE - 1), i, pl.ds(2 * r + k, n, stride=2), :] for k in range(2)]
            wqkv[6 * j + 2 * i, pl.ds(r, n), :] = (even & np.uint32(0xFFFF)) | (odd << 16)
            wqkv[6 * j + 2 * i + 1, pl.ds(r, n), :] = (even >> 16) | (odd & np.uint32(0xFFFF0000))

    def refill(j):
        @pl.when(j + N_STAGE < n_pairs)
        def _():
            for cp in cp_stage(j + N_STAGE):
                cp.start()

        def queue_rest(*_):
            cp_x0.start()
            cp_wo.start()
            for k in range(2, 6):
                cp_mod(k).start()
            cp_x1.start()

        jax.lax.fori_loop(0, jnp.where(j + N_STAGE == n_pairs, 1, 0), queue_rest, None)

    def pre_proj(i, _):
        j = jnp.minimum(i, n_pairs - 1)

        @pl.when(jnp.logical_and(i > 0, i < n_pairs))
        def _():
            for cp in cp_stage(j):
                cp.wait()

        half = hpre.shape[0] // 2
        a = _bf(hpre[pl.ds(pl.multiple_of((i & 1) * half, half), half), :])
        res = []
        for t in range(6):
            tile = (i >> 1) * 6 + t
            res.append(_dot(a, _bf(wqkv[tile])))
            pre[tile, pl.ds(pl.multiple_of((i & 1) * 2 * half, 2 * half), 2 * half), :] = res[t]
            if 1 <= t <= 4:
                for g in range(2):
                    stage[j & (N_STAGE - 1), 0, pl.ds(pl.multiple_of(dm + (i >> 8) * 8, 8), 8), :] = (
                        pltpu.bitcast(res[t - 1][g * half:g * half + 8], U32))
                    relayout(j, (2 * t - 2 + g) * (dm // 16), dm // 16)
        refill(i)

    for cp in cp_stage(0):
        cp.wait()
    jax.lax.fori_loop(0, dm // 128, lambda t, _: relayout(0, pl.multiple_of(t * 64, 64), 64), None)
    jax.lax.fori_loop(0, 2 * N_PRE, pre_proj, None)
    cp_x0.wait()
    lhs[0:n_mem, :] = mem0_ref[...].astype(F32)
    lhs[n_mem:rows, :] = seg_h(0)

    def finish(s, attn):
        xn = seg_x(s) + get_mod(2, seg) * attn
        slot = (s >> 2) & 1
        sub = s & 3
        x1[slot, pl.ds(pl.multiple_of(sub * seg, seg), seg), :] = xn
        h = _mod_ln(xn, get_mod(4, seg), get_mod(3, seg))
        for i, t in enumerate(_strassen_lhs(h[:hseg, :hd], h[:hseg, hd:], h[hseg:, :hd], h[hseg:, hd:])):
            h2[slot, i, pl.ds(pl.multiple_of(sub * hseg, hseg), hseg), :] = t

    def step(s, phase):
        do_attn = phase != "ffn"
        do_ffn = phase != "first"
        if do_ffn:
            fb = (s >> 2) - 1
            fch = s & 3
            fslot = fb & 1
            act_a, act_b = [None] * (2 * (fq // 128) + 1), [None] * (2 * (fq // 128) + 1)
        up_work, down_work = [], []
        if phase == "first":
            for cp in cp_ffn(s):
                cp.start()
        if phase == "prep":
            for cp in cp_ffn(fch):
                cp.wait()
            up_work = [(_prepare_two_levels, wup2, r, 8, k)
                       for k in range(0, fq, 128) for r in range(0, hd // 4, 8)]
            down_work = [(_prepare_one_level, w, r, 32, k) for w in (wup1, wdn)
                         for k in range(0, w.shape[3], 128) for r in range(0, w.shape[2] // 7, 32)]

        def prepare_weights(work, i, n, anchor):
            todo = work[-(-len(work) * i // n):-(-len(work) * (i + 1) // n)]
            for _, w, r, _, k in todo[:1]:
                w[fch, fb, r:r + 8, k:k + 128] = pltpu.bitcast(anchor, U32)
            for prepare, w, r, size, k in todo:
                prepare(w, fch, r, size, k)

        nq = fq // 128
        def gate(t, products):
            ga, ua, gb, ub = _strassen_out(products)
            act_a[t] = ga * jax.nn.sigmoid(ga) * ua
            act_b[t] = gb * jax.nn.sigmoid(gb) * ub

        def ffn_up():
            inner_ops = []
            for i in range(7):
                h = h2[fslot, i]
                inner_ops.append([v.astype(BF16) for v in _strassen_lhs(
                    h[:seg, :hd // 2], h[:seg, hd // 2:], h[seg:, :hd // 2], h[seg:, hd // 2:])])
            for t in range(nq):
                left, right = [], []
                for i in range(7):
                    c11, c12, c21, c22 = _strassen_out(
                        [_dot(inner_ops[i][j], _bf(wup2[fch, i, _operand(wup2, j), t * 128:(t + 1) * 128]))
                         for j in range(7)])
                    left.append(jnp.concatenate([c11, c21], axis=0))
                    right.append(jnp.concatenate([c12, c22], axis=0))
                gate(t, left)
                gate(nq + t, right)
                yield
            gate(2 * nq, [_dot(h2[fslot, i].astype(BF16), _bf(wup1[fch, 0, _operand(wup1, i), :]))
                          for i in range(7)])

        up = ffn_up()

        def ffn_down():
            if do_ffn:
                aa, ab = jnp.concatenate(act_a, axis=1), jnp.concatenate(act_b, axis=1)
                ops = [t.astype(BF16) for t in _strassen_lhs(
                    aa[:, :kd], aa[:, kd:2 * kd], ab[:, :kd], ab[:, kd:2 * kd])]
                rest = _dot(jnp.concatenate([aa[:, 2 * kd:], ab[:, 2 * kd:]], axis=0).astype(BF16),
                            _bf(wrest[fch]))
                for t in range(0, hd, DOWN_COLS):
                    y = _strassen_out([_dot(ops[i], _bf(wdn[fch, 0, _operand(wdn, i), t:t + DOWN_COLS]))
                                       for i in range(7)])
                    for side in range(2):
                        cols = slice(side * hd + t, side * hd + t + DOWN_COLS)
                        ya = y[side] + rest[:blk // 2, cols]
                        yb = y[2 + side] + rest[blk // 2:, cols]
                        yy = jnp.concatenate([v[k * hseg:(k + 1) * hseg] for k in range(FFN_SEGS)
                                              for v in (ya, yb)], axis=0)
                        acc = x1[fslot, :, cols] + get_mod(5, blk)[:, cols] * yy
                        x1[fslot, :, cols] = acc
                        for k in range(FFN_SEGS):
                            xs[fb * FFN_SEGS + k, :, cols] = _words(acc[k * seg:(k + 1) * seg])

        if not do_attn:
            list(up)
            ffn_down()
        else:
            r = jax.lax.broadcasted_iota(jnp.int32, (2 * rows, 2 * rows), 0)
            q = jax.lax.broadcasted_iota(jnp.int32, (2 * rows, 2 * rows), 1)
            same = (r >= rows) == (q >= rows)
            rl = jnp.where(r >= rows, r - rows, r)
            ql = jnp.where(q >= rows, q - rows, q)
            keep = same & ((rl < n_mem) | (rl >= ql))
            fill = jnp.where(same, -1e9, -jnp.inf).astype(F32)
            a = lhs[...]
            a_short = a[:rows - PRE_ROWS].astype(BF16)
            qkv, probs = {}, {}

            def proj(j):
                t = []
                for tile in range(6 * j, 6 * j + 6):
                    if tile < pre.shape[0]:
                        t.append(jnp.concatenate(
                            [_dot(a_short, _bf(wqkv[tile])),
                             pre[tile, pl.ds(pl.multiple_of(s * PRE_ROWS, PRE_ROWS), PRE_ROWS), :]], axis=0))
                    else:
                        t.append(_dot(a, _bf(wqkv[tile])))
                prepare_weights(up_work, j, n_pairs, t[0][0:8])
                qkv[j] = [jnp.concatenate(t[2 * i:2 * i + 2], axis=0).astype(BF16) for i in range(3)]

            def scores(j):
                t = jnp.where(keep, _dot_nt(qkv[j][0], qkv[j][1]) * scale, fill)
                e = jnp.exp(t - jnp.max(t, axis=-1, keepdims=True))
                probs[j] = (e / jnp.sum(e, axis=-1, keepdims=True)).astype(BF16)

            def mix(j):
                o = _round(_dot(probs[j], qkv[j][2]))
                obuf[:, 2 * j * dh:(2 * j + 1) * dh] = o[:rows]
                obuf[:, (2 * j + 1) * dh:(2 * j + 2) * dh] = o[rows:]

            def oproj(lo, hi):
                return _dot(obuf[:, lo * 2 * dh:hi * 2 * dh], _bf(wo[lo * dh:hi * dh, :]))

            per_part = (n_pairs - 4) // LAG_M

            def oproj_part(k):
                parts.append(oproj(per_part * k, per_part * (k + 1)))
                prepare_weights(down_work, k, LAG_M, parts[k][0:8, 0:128])

            def first_waits():
                @pl.when(s == 0)
                def _():
                    cp_wo.wait()

                @pl.when(s > 0)
                def _():
                    cp_mod(s + 1).wait()

            fillers = [functools.partial(proj, j) for j in range(n_pairs)]
            parts = []
            if phase == "both":
                fillers += [lambda: next(up, None)] * LAG_M
                done = 0
            else:
                if phase == "first":
                    fillers.insert(n_pairs - 1, first_waits)
                fillers += [functools.partial(oproj_part, k) for k in range(LAG_M)]
                done = per_part * LAG_M
            for i, filler in enumerate(fillers):
                filler()
                if 0 <= i - LAG_S < n_pairs:
                    scores(i - LAG_S)
                if 0 <= i - LAG_M < n_pairs:
                    mix(i - LAG_M)
            if do_ffn:
                list(up)
            o = sum(parts, oproj(done, n_pairs))
            lhs[0:n_mem, :] = _round(o[:n_mem])
            lhs[n_mem:rows, :] = seg_h(jnp.minimum(s + 1, n_seg - 1))
            if phase != "first":
                finish(s, o[n_mem:])
            else:
                x1[0, pl.ds(pl.multiple_of(s * seg, seg), seg), :] = o[n_mem:]
                set_mod(s + 1)
            ffn_down()

        if do_ffn:
            @pl.when(fch == FFN_SEGS - 1)
            def _():
                cp_out(fb).start()

    def run(lo, hi, phase):
        jax.lax.fori_loop(lo, hi, lambda s, _: step(s, phase), None)

    run(0, FFN_SEGS, "first")
    cp_x1.wait()
    cp_mod(5).wait()
    set_mod(5)
    for s in range(FFN_SEGS):
        finish(s, x1[0, s * seg:(s + 1) * seg, :])
    run(FFN_SEGS, 2 * FFN_SEGS, "prep")
    run(2 * FFN_SEGS, n_seg, "both")
    run(n_seg, n_seg + FFN_SEGS, "ffn")
    for b in range(n_blk):
        cp_out(b).wait()


@functools.partial(jax.jit, static_argnames=("A_seg_len",))
def pallas_adaLN_cond__memory_aug_recurrent_mem_tr__glu_gated_swiglu__prompt_kernel(
    A_x, A_mem0, A_Wq, A_Wk, A_Wv, A_Wo, A_seg_len, B_x, B_w1, B_w3, B_w2, c, w_mod,
):
    del B_x
    bsz, s_len, dm = A_x.shape
    _, n_heads, dh = A_Wq.shape
    n_mem = A_mem0.shape[1]
    seg = int(A_seg_len)
    f = B_w1.shape[1]
    fc = f // FFN_SEGS
    kd = (fc - 1) // 256 * 128
    blk = FFN_SEGS * seg
    assert bsz == 1 and s_len % blk == 0 and n_heads % 4 == 0 and fc % 128 == 0 and FFN_SEGS == 4
    assert n_heads // 4 <= N_PRE <= n_heads // 2

    hbm = pl.BlockSpec(memory_space=pltpu.MemorySpace.HBM)
    vmem = pl.BlockSpec(memory_space=pltpu.MemorySpace.VMEM)
    scratch = dict(
        wqkv=pltpu.VMEM((3 * n_heads, dm // 2, dh), U32),
        wo=pltpu.VMEM((n_heads * dh // 2, dm), U32),
        wup2=pltpu.VMEM((FFN_SEGS, 7, 7 * dm // 8, kd), U32),
        wup1=pltpu.VMEM((FFN_SEGS, 1, 7 * dm // 4, fc - 2 * kd), U32),
        wdn=pltpu.VMEM((FFN_SEGS, 1, 7 * kd // 2, dm // 2), U32),
        wrest=pltpu.VMEM((FFN_SEGS, fc // 2 - kd, dm), U32),
        wmod=pltpu.VMEM((N_MOD, dm // 2, dm), U32),
        stage=pltpu.VMEM((N_STAGE, 3, dm + 8, dh), U32),
        xs=pltpu.VMEM((s_len // seg, seg // 2, dm), U32),
        mod=pltpu.VMEM((6, 8, dm), F32),
        lhs=pltpu.VMEM((n_mem + seg, dm), F32),
        obuf=pltpu.VMEM((n_mem + seg, n_heads * dh), F32),
        x1=pltpu.VMEM((2, blk, dm), F32),
        h2=pltpu.VMEM((2, 7, blk // 2, dm // 2), F32),
        hpre=pltpu.VMEM((s_len // seg * PRE_ROWS // 2, dm), U32),
        pre=pltpu.VMEM((6 * N_PRE, s_len // seg * PRE_ROWS, dh), F32),
        sem_stage=pltpu.SemaphoreType.DMA((3 * N_STAGE,)),
        sem_misc=pltpu.SemaphoreType.DMA((4,)),
        sem_mod=pltpu.SemaphoreType.DMA((6,)),
        sem_ffn=pltpu.SemaphoreType.DMA((FFN_SEGS,)),
        sem_out=pltpu.SemaphoreType.DMA((s_len // blk,)),
    )

    def body(*refs):
        n_io = len(refs) - len(scratch)
        _kernel(*refs[:n_io], **dict(zip(scratch, refs[n_io:])), seg=seg, n_mem=n_mem, dh=dh)

    out = pl.pallas_call(
        body,
        out_shape=jax.ShapeDtypeStruct((s_len // seg, seg, dm), A_x.dtype),
        in_specs=[vmem, vmem] + [hbm] * 9,
        out_specs=hbm,
        scratch_shapes=list(scratch.values()),
        compiler_params=pltpu.CompilerParams(
            vmem_limit_bytes=127 * 2**20,
            flags={"XLA_TPU_EVENLY_DISTRIBUTE_CRITICAL_NODES": True}),
    )(c, A_mem0.reshape(n_mem, dm), A_x.reshape(s_len // seg, seg, dm), A_Wq, A_Wk, A_Wv,
      A_Wo.reshape(n_heads * dh, dm), B_w1, B_w3, B_w2, w_mod)
    return out.reshape(bsz, s_len, dm)
```

```python
import functools

import jax
import jax.numpy as jnp
import numpy as np
import jax.experimental.pallas as pl
import jax.experimental.pallas.tpu as pltpu

U32 = jnp.uint32
BF16 = jnp.bfloat16
F32 = jnp.float32
LN_EPS = 1e-5
FFN_SEGS = 4
N_STAGE = 4
N_PRE = 9
PRE_ROWS = 8
DOWN_COLS = 512
N_MOD = 5
LAG_S, LAG_M = 2, 4
X_HEAD = 8


def _bf(w):
    return pltpu.bitcast(w, BF16)


def _words(a):
    return pltpu.bitcast(a.astype(BF16), U32)


def _dot(a, b):
    return jax.lax.dot_general(a, b, (((1,), (0,)), ((), ())), preferred_element_type=F32)


def _dot_nt(a, b):
    return jax.lax.dot_general(a, b, (((1,), (1,)), ((), ())), preferred_element_type=F32)


def _round(a):
    return a.astype(BF16).astype(F32)


def _silu(x):
    h = 0.5 * x
    return h * jnp.tanh(h) + h


def _ln(x):
    m = jnp.mean(x, axis=-1, keepdims=True)
    d = x - m
    v = jnp.mean(d * d, axis=-1, keepdims=True)
    return d * jax.lax.rsqrt(v + LN_EPS)


def _mod_ln(x, scale1, shift):
    return _ln(x) * scale1 + shift


def _strassen_lhs(a11, a12, a21, a22):
    return [a11 + a22, a21 + a22, a11, a22, a11 + a12, a21 - a11, a12 - a22]


def _strassen_out(m):
    return m[0] + m[3] - m[4] + m[6], m[2] + m[4], m[1] + m[3], m[0] - m[1] + m[2] + m[5]


def _strassen_rhs(b11, b12, b21, b22):
    return [b11 + b22, b11, b12 - b22, b21 - b11, b22, b11 + b12, b21 + b22]


PLACE = (0, 1, 3, 2, 4, 5, 6)
RAW = (1, 2, 3, 4)
KEPT = (1, 4)


def _operand(w, i, r=0, n=None):
    size = w.shape[-2] // 7
    return pl.ds(PLACE[i] * size + r, size if n is None else n)


def _halves(w):
    return pltpu.bitcast(jnp.concatenate([w << 16, w & np.uint32(0xFFFF0000)], axis=0), F32)


def _join(t):
    u = pltpu.bitcast(t, U32)
    n = u.shape[0] // 2
    return ((u[:n] + np.uint32(0x8000)) >> 16) | ((u[n:] + np.uint32(0x7FFF)) & np.uint32(0xFFFF0000))


def _prepare_one_level(w, c, r, n, k):
    raw = [_halves(w[c, 0, _operand(w, i, r, n), k:k + 128]) for i in RAW]
    for i, t in enumerate(_strassen_rhs(*raw)):
        if i not in KEPT:
            w[c, 0, _operand(w, i, r, n), k:k + 128] = _join(t)


def _prepare_two_levels(w, c, r, n, k):
    outer = [_strassen_rhs(*[_halves(w[c, i, _operand(w, j, r, n), k:k + 128]) for i in RAW]) for j in RAW]
    for i in range(7):
        for j, t in enumerate(_strassen_rhs(*[sub[i] for sub in outer])):
            if i not in KEPT or j not in KEPT:
                w[c, i, _operand(w, j, r, n), k:k + 128] = _join(t)


def _kernel(c_ref, mem0_ref, x_hbm, wq_hbm, wk_hbm, wv_hbm, wo_hbm, w1_hbm, w3_hbm, w2_hbm,
            wmod_hbm, out_hbm,
            wqkv, wo, wup2, wup1, wdn, wrest, wmod, stage, xs, mod, lhs, obuf, x1, h2, hpre, pre,
            sem_stage, sem_misc, sem_mod, sem_ffn, sem_out, *, seg, n_mem, dh):
    n_pairs = wqkv.shape[0] // 6
    dm = lhs.shape[1]
    rows = n_mem + seg
    hseg = seg // 2
    n_seg = xs.shape[0]
    n_blk = n_seg // FFN_SEGS
    blk = FFN_SEGS * seg
    fq = wup2.shape[3]
    fc = 2 * fq + wup1.shape[3]
    kd = 2 * wdn.shape[2] // 7
    hd = dm // 2
    scale = dh ** -0.5

    wmod32 = wmod_hbm.bitcast(U32)
    x32 = x_hbm.bitcast(U32)
    out32 = out_hbm.bitcast(U32)
    qkv32 = [w.bitcast(U32) for w in (wq_hbm, wk_hbm, wv_hbm)]
    hpr = PRE_ROWS // 2
    tail = pl.ds(hseg - hpr, hpr)
    cp_xpre = pltpu.make_async_copy(x32.at[:, tail, :], xs.at[:, tail, :], sem_misc.at[0])
    cp_x0 = pltpu.make_async_copy(x32.at[pl.ds(0, X_HEAD)], xs.at[pl.ds(0, X_HEAD)], sem_misc.at[1])
    cp_x1 = pltpu.make_async_copy(x32.at[pl.ds(X_HEAD, n_seg - X_HEAD)], xs.at[pl.ds(X_HEAD, n_seg - X_HEAD)],
                                  sem_misc.at[2])
    cp_wo = pltpu.make_async_copy(wo_hbm.bitcast(U32), wo, sem_misc.at[3])

    def cp_mod(k):
        return pltpu.make_async_copy(wmod32.at[:, pl.ds(pl.multiple_of(k * dm, dm), dm)], wmod.at[k % N_MOD],
                                     sem_mod.at[k])

    def cp_stage(j):
        slot = j & (N_STAGE - 1)
        return [pltpu.make_async_copy(qkv32[i].at[:, j, :], stage.at[slot, i, pl.ds(0, dm)],
                                      sem_stage.at[3 * slot + i])
                for i in range(3)]

    def cp_ffn(c):
        w1_32, w3_32, w2_32 = w1_hbm.bitcast(U32), w3_hbm.bitcast(U32), w2_hbm.bitcast(U32)

        def up_cols(off, n):
            return pl.ds(pl.multiple_of(c * fc + off, 128), n)

        def w2_rows(off, n):
            return pl.ds(pl.multiple_of(c * (fc // 2) + off, 64), n)

        pairs = []
        for side, w in enumerate((w1_32, w3_32)):
            for i in range(2):
                for j in range(2):
                    pairs.append((w.at[pl.ds(i * (hd // 2), hd // 2), up_cols(j * fq, fq)],
                                  wup2.at[c, RAW[2 * i + side], _operand(wup2, RAW[j], 0, hd // 2)]))
            pairs.append((w.at[:, up_cols(2 * fq, fc - 2 * fq)], wup1.at[c, 0, _operand(wup1, RAW[side], 0, hd)]))
            pairs.append((w2_32.at[w2_rows(0, kd), pl.ds(side * hd, hd)],
                          wdn.at[c, 0, _operand(wdn, RAW[side], 0, kd)]))
        pairs.append((w2_32.at[w2_rows(kd, fc // 2 - kd), :], wrest.at[c]))
        return [pltpu.make_async_copy(src, dst, sem_ffn.at[c]) for src, dst in pairs]

    def cp_out(b):
        r = pl.ds(b * FFN_SEGS, FFN_SEGS)
        return pltpu.make_async_copy(xs.at[r], out32.at[r], sem_out.at[b])

    cp_xpre.start()
    cp_mod(1).start()
    cp_mod(0).start()
    for j in range(N_STAGE):
        for cp in cp_stage(j):
            cp.start()

    cf = c_ref[...].astype(F32)
    sc = jnp.broadcast_to(_round(cf * jax.nn.sigmoid(cf)), (8, dm))

    def set_mod(k):
        mod[k] = _dot(sc, _bf(wmod[k % N_MOD])) + jnp.where(k % 3 == 1, 1.0, 0.0)

    def get_mod(k, n):
        return jnp.concatenate([mod[k]] * (n // 8), axis=0)

    def seg_x(s):
        return _bf(xs[s]).astype(F32)

    def seg_h(s):
        return _round(_mod_ln(seg_x(s), get_mod(1, seg), get_mod(0, seg)))

    parked = pre.shape[0] - dm // dh

    def pre_norm(i, _):
        t = _ln(_bf(jnp.concatenate([xs[2 * i, tail], xs[2 * i + 1, tail]], axis=0)).astype(F32))
        for k in range(dm // dh):
            pre[parked + k, pl.ds(pl.multiple_of(i * 2 * PRE_ROWS, 2 * PRE_ROWS), 2 * PRE_ROWS), :] = (
                t[:, k * dh:(k + 1) * dh])

    def pre_mod(i, _):
        t = jnp.concatenate([pre[parked + k, pl.ds(pl.multiple_of(i * 64, 64), 64), :]
                             for k in range(dm // dh)], axis=1)
        hpre[pl.ds(pl.multiple_of(i * 32, 32), 32), :] = _words(t * get_mod(1, 64) + get_mod(0, 64))

    cp_xpre.wait()
    jax.lax.fori_loop(0, n_seg // 2, pre_norm, None, unroll=8)
    for k in (1, 0):
        cp_mod(k).wait()
        set_mod(k)
    jax.lax.fori_loop(0, n_seg * PRE_ROWS // 64, pre_mod, None)

    def relayout(j, r, n):
        for i in range(3):
            even, odd = [stage[j & (N_STAGE - 1), i, pl.ds(2 * r + k, n, stride=2), :] for k in range(2)]
            wqkv[6 * j + 2 * i, pl.ds(r, n), :] = (even & np.uint32(0xFFFF)) | (odd << 16)
            wqkv[6 * j + 2 * i + 1, pl.ds(r, n), :] = (even >> 16) | (odd & np.uint32(0xFFFF0000))

    def refill(j):
        @pl.when(j + N_STAGE < n_pairs)
        def _():
            for cp in cp_stage(j + N_STAGE):
                cp.start()

        def queue_rest(*_):
            cp_x0.start()
            cp_wo.start()
            for k in range(2, 6):
                cp_mod(k).start()
            cp_x1.start()

        jax.lax.fori_loop(0, jnp.where(j + N_STAGE == n_pairs, 1, 0), queue_rest, None)

    def pre_proj(i, _):
        j = jnp.minimum(i, n_pairs - 1)

        @pl.when(jnp.logical_and(i > 0, i < n_pairs))
        def _():
            for cp in cp_stage(j):
                cp.wait()

        half = hpre.shape[0] // 2
        a = _bf(hpre[pl.ds(pl.multiple_of((i & 1) * half, half), half), :])
        res = []
        for t in range(6):
            tile = (i >> 1) * 6 + t
            res.append(_dot(a, _bf(wqkv[tile])))
            pre[tile, pl.ds(pl.multiple_of((i & 1) * 2 * half, 2 * half), 2 * half), :] = res[t]
            if 1 <= t <= 4:
                for g in range(2):
                    stage[j & (N_STAGE - 1), 0, pl.ds(pl.multiple_of(dm + (i >> 8) * 8, 8), 8), :] = (
                        pltpu.bitcast(res[t - 1][g * half:g * half + 8], U32))
                    relayout(j, (2 * t - 2 + g) * (dm // 16), dm // 16)
        refill(i)

    for cp in cp_stage(0):
        cp.wait()
    jax.lax.fori_loop(0, dm // 128, lambda t, _: relayout(0, pl.multiple_of(t * 64, 64), 64), None)
    jax.lax.fori_loop(0, 2 * N_PRE, pre_proj, None)
    cp_x0.wait()
    lhs[0:n_mem, :] = mem0_ref[...].astype(F32)
    lhs[n_mem:rows, :] = seg_h(0)

    def finish(s, attn):
        xn = seg_x(s) + get_mod(2, seg) * attn
        slot = (s >> 2) & 1
        sub = s & 3
        x1[slot, pl.ds(pl.multiple_of(sub * seg, seg), seg), :] = xn
        h = _mod_ln(xn, get_mod(4, seg), get_mod(3, seg))
        for i, t in enumerate(_strassen_lhs(h[:hseg, :hd], h[:hseg, hd:], h[hseg:, :hd], h[hseg:, hd:])):
            h2[slot, i, pl.ds(pl.multiple_of(sub * hseg, hseg), hseg), :] = t

    def step(s, phase):
        do_attn = phase != "ffn"
        do_ffn = phase != "first"
        if do_ffn:
            fb = (s >> 2) - 1
            fch = s & 3
            fslot = fb & 1
            act_a, act_b = [None] * (2 * (fq // 128) + 1), [None] * (2 * (fq // 128) + 1)
        up_work, down_work = [], []
        if phase == "first":
            for cp in cp_ffn(s):
                cp.start()
        if phase == "prep":
            for cp in cp_ffn(fch):
                cp.wait()
            up_work = [(_prepare_two_levels, wup2, r, 8, k)
                       for k in range(0, fq, 128) for r in range(0, hd // 4, 8)]
            down_work = [(_prepare_one_level, w, r, 32, k) for w in (wup1, wdn)
                         for k in range(0, w.shape[3], 128) for r in range(0, w.shape[2] // 7, 32)]

        def prepare_weights(work, i, n, anchor):
            todo = work[-(-len(work) * i // n):-(-len(work) * (i + 1) // n)]
            for _, w, r, _, k in todo[:1]:
                w[fch, fb, r:r + 8, k:k + 128] = pltpu.bitcast(anchor, U32)
            for prepare, w, r, size, k in todo:
                prepare(w, fch, r, size, k)

        nq = fq // 128
        def gate(t, products):
            ga, ua, gb, ub = _strassen_out(products)
            act_a[t] = _silu(ga) * ua
            act_b[t] = _silu(gb) * ub

        def ffn_up():
            inner_ops = []
            for i in range(7):
                h = h2[fslot, i]
                inner_ops.append([v.astype(BF16) for v in _strassen_lhs(
                    h[:seg, :hd // 2], h[:seg, hd // 2:], h[seg:, :hd // 2], h[seg:, hd // 2:])])
            for t in range(nq):
                left, right = [], []
                for i in range(7):
                    c11, c12, c21, c22 = _strassen_out(
                        [_dot(inner_ops[i][j], _bf(wup2[fch, i, _operand(wup2, j), t * 128:(t + 1) * 128]))
                         for j in range(7)])
                    left.append(jnp.concatenate([c11, c21], axis=0))
                    right.append(jnp.concatenate([c12, c22], axis=0))
                gate(t, left)
                gate(nq + t, right)
                yield
            gate(2 * nq, [_dot(h2[fslot, i].astype(BF16), _bf(wup1[fch, 0, _operand(wup1, i), :]))
                          for i in range(7)])

        up = ffn_up()

        def ffn_down():
            if do_ffn:
                aa, ab = jnp.concatenate(act_a, axis=1), jnp.concatenate(act_b, axis=1)
                ops = [t.astype(BF16) for t in _strassen_lhs(
                    aa[:, :kd], aa[:, kd:2 * kd], ab[:, :kd], ab[:, kd:2 * kd])]
                rest = _dot(jnp.concatenate([aa[:, 2 * kd:], ab[:, 2 * kd:]], axis=0).astype(BF16),
                            _bf(wrest[fch]))
                for t in range(0, hd, DOWN_COLS):
                    y = _strassen_out([_dot(ops[i], _bf(wdn[fch, 0, _operand(wdn, i), t:t + DOWN_COLS]))
                                       for i in range(7)])
                    for side in range(2):
                        cols = slice(side * hd + t, side * hd + t + DOWN_COLS)
                        ya = y[side] + rest[:blk // 2, cols]
                        yb = y[2 + side] + rest[blk // 2:, cols]
                        yy = jnp.concatenate([v[k * hseg:(k + 1) * hseg] for k in range(FFN_SEGS)
                                              for v in (ya, yb)], axis=0)
                        acc = x1[fslot, :, cols] + get_mod(5, blk)[:, cols] * yy
                        x1[fslot, :, cols] = acc
                        for k in range(FFN_SEGS):
                            xs[fb * FFN_SEGS + k, :, cols] = _words(acc[k * seg:(k + 1) * seg])

        if not do_attn:
            list(up)
            ffn_down()
        else:
            r = jax.lax.broadcasted_iota(jnp.int32, (2 * rows, 2 * rows), 0)
            q = jax.lax.broadcasted_iota(jnp.int32, (2 * rows, 2 * rows), 1)
            same = (r >= rows) == (q >= rows)
            rl = jnp.where(r >= rows, r - rows, r)
            ql = jnp.where(q >= rows, q - rows, q)
            keep = same & ((rl < n_mem) | (rl >= ql))
            fill = jnp.where(same, -1e9, -jnp.inf).astype(F32)
            a = lhs[...]
            a_short = a[:rows - PRE_ROWS].astype(BF16)
            qkv, probs = {}, {}

            def proj(j):
                t = []
                for tile in range(6 * j, 6 * j + 6):
                    if tile < pre.shape[0]:
                        t.append(jnp.concatenate(
                            [_dot(a_short, _bf(wqkv[tile])),
                             pre[tile, pl.ds(pl.multiple_of(s * PRE_ROWS, PRE_ROWS), PRE_ROWS), :]], axis=0))
                    else:
                        t.append(_dot(a, _bf(wqkv[tile])))
                prepare_weights(up_work, j, n_pairs, t[0][0:8])
                qkv[j] = [jnp.concatenate(t[2 * i:2 * i + 2], axis=0).astype(BF16) for i in range(3)]

            def scores(j):
                t = jnp.where(keep, _dot_nt(qkv[j][0], qkv[j][1]) * scale, fill)
                e = jnp.exp(t - jnp.max(t, axis=-1, keepdims=True))
                probs[j] = (e / jnp.sum(e, axis=-1, keepdims=True)).astype(BF16)

            def mix(j):
                o = _round(_dot(probs[j], qkv[j][2]))
                obuf[:, 2 * j * dh:(2 * j + 1) * dh] = o[:rows]
                obuf[:, (2 * j + 1) * dh:(2 * j + 2) * dh] = o[rows:]

            def oproj(lo, hi):
                return _dot(obuf[:, lo * 2 * dh:hi * 2 * dh], _bf(wo[lo * dh:hi * dh, :]))

            per_part = (n_pairs - 4) // LAG_M

            def oproj_part(k):
                parts.append(oproj(per_part * k, per_part * (k + 1)))
                prepare_weights(down_work, k, LAG_M, parts[k][0:8, 0:128])

            def first_waits():
                @pl.when(s == 0)
                def _():
                    cp_wo.wait()

                @pl.when(s > 0)
                def _():
                    cp_mod(s + 1).wait()

            fillers = [functools.partial(proj, j) for j in range(n_pairs)]
            parts = []
            if phase == "both":
                fillers += [lambda: next(up, None)] * LAG_M
                done = 0
            else:
                if phase == "first":
                    fillers.insert(n_pairs - 1, first_waits)
                fillers += [functools.partial(oproj_part, k) for k in range(LAG_M)]
                done = per_part * LAG_M
            for i, filler in enumerate(fillers):
                filler()
                if 0 <= i - LAG_S < n_pairs:
                    scores(i - LAG_S)
                if 0 <= i - LAG_M < n_pairs:
                    mix(i - LAG_M)
            if do_ffn:
                list(up)
            o = sum(parts, oproj(done, n_pairs))
            lhs[0:n_mem, :] = _round(o[:n_mem])
            lhs[n_mem:rows, :] = seg_h(jnp.minimum(s + 1, n_seg - 1))
            if phase != "first":
                finish(s, o[n_mem:])
            else:
                x1[0, pl.ds(pl.multiple_of(s * seg, seg), seg), :] = o[n_mem:]
                set_mod(s + 1)
            ffn_down()

        if do_ffn:
            @pl.when(fch == FFN_SEGS - 1)
            def _():
                cp_out(fb).start()

    def run(lo, hi, phase):
        jax.lax.fori_loop(lo, hi, lambda s, _: step(s, phase), None)

    run(0, FFN_SEGS, "first")
    cp_x1.wait()
    cp_mod(5).wait()
    set_mod(5)
    for s in range(FFN_SEGS):
        finish(s, x1[0, s * seg:(s + 1) * seg, :])
    run(FFN_SEGS, 2 * FFN_SEGS, "prep")
    run(2 * FFN_SEGS, n_seg, "both")
    run(n_seg, n_seg + FFN_SEGS, "ffn")
    for b in range(n_blk):
        cp_out(b).wait()


@functools.partial(jax.jit, static_argnames=("A_seg_len",))
def pallas_adaLN_cond__memory_aug_recurrent_mem_tr__glu_gated_swiglu__prompt_kernel(
    A_x, A_mem0, A_Wq, A_Wk, A_Wv, A_Wo, A_seg_len, B_x, B_w1, B_w3, B_w2, c, w_mod,
):
    del B_x
    bsz, s_len, dm = A_x.shape
    _, n_heads, dh = A_Wq.shape
    n_mem = A_mem0.shape[1]
    seg = int(A_seg_len)
    f = B_w1.shape[1]
    fc = f // FFN_SEGS
    kd = (fc - 1) // 256 * 128
    blk = FFN_SEGS * seg
    assert bsz == 1 and s_len % blk == 0 and n_heads % 4 == 0 and fc % 128 == 0 and FFN_SEGS == 4
    assert n_heads // 4 <= N_PRE <= n_heads // 2

    hbm = pl.BlockSpec(memory_space=pltpu.MemorySpace.HBM)
    vmem = pl.BlockSpec(memory_space=pltpu.MemorySpace.VMEM)
    scratch = dict(
        wqkv=pltpu.VMEM((3 * n_heads, dm // 2, dh), U32),
        wo=pltpu.VMEM((n_heads * dh // 2, dm), U32),
        wup2=pltpu.VMEM((FFN_SEGS, 7, 7 * dm // 8, kd), U32),
        wup1=pltpu.VMEM((FFN_SEGS, 1, 7 * dm // 4, fc - 2 * kd), U32),
        wdn=pltpu.VMEM((FFN_SEGS, 1, 7 * kd // 2, dm // 2), U32),
        wrest=pltpu.VMEM((FFN_SEGS, fc // 2 - kd, dm), U32),
        wmod=pltpu.VMEM((N_MOD, dm // 2, dm), U32),
        stage=pltpu.VMEM((N_STAGE, 3, dm + 8, dh), U32),
        xs=pltpu.VMEM((s_len // seg, seg // 2, dm), U32),
        mod=pltpu.VMEM((6, 8, dm), F32),
        lhs=pltpu.VMEM((n_mem + seg, dm), F32),
        obuf=pltpu.VMEM((n_mem + seg, n_heads * dh), F32),
        x1=pltpu.VMEM((2, blk, dm), F32),
        h2=pltpu.VMEM((2, 7, blk // 2, dm // 2), F32),
        hpre=pltpu.VMEM((s_len // seg * PRE_ROWS // 2, dm), U32),
        pre=pltpu.VMEM((6 * N_PRE, s_len // seg * PRE_ROWS, dh), F32),
        sem_stage=pltpu.SemaphoreType.DMA((3 * N_STAGE,)),
        sem_misc=pltpu.SemaphoreType.DMA((4,)),
        sem_mod=pltpu.SemaphoreType.DMA((6,)),
        sem_ffn=pltpu.SemaphoreType.DMA((FFN_SEGS,)),
        sem_out=pltpu.SemaphoreType.DMA((s_len // blk,)),
    )

    def body(*refs):
        n_io = len(refs) - len(scratch)
        _kernel(*refs[:n_io], **dict(zip(scratch, refs[n_io:])), seg=seg, n_mem=n_mem, dh=dh)

    out = pl.pallas_call(
        body,
        out_shape=jax.ShapeDtypeStruct((s_len // seg, seg, dm), A_x.dtype),
        in_specs=[vmem, vmem] + [hbm] * 9,
        out_specs=hbm,
        scratch_shapes=list(scratch.values()),
        compiler_params=pltpu.CompilerParams(
            vmem_limit_bytes=127 * 2**20,
            flags={"XLA_TPU_EVENLY_DISTRIBUTE_CRITICAL_NODES": True}),
    )(c, A_mem0.reshape(n_mem, dm), A_x.reshape(s_len // seg, seg, dm), A_Wq, A_Wk, A_Wv,
      A_Wo.reshape(n_heads * dh, dm), B_w1, B_w3, B_w2, w_mod)
    return out.reshape(bsz, s_len, dm)
```

```python
import functools

import jax
import jax.numpy as jnp
import numpy as np
import jax.experimental.pallas as pl
import jax.experimental.pallas.tpu as pltpu

U32 = jnp.uint32
BF16 = jnp.bfloat16
F32 = jnp.float32
LN_EPS = 1e-5
FFN_SEGS = 4
N_STAGE = 4
N_PRE = 9
PRE_ROWS = 8
DOWN_COLS = 512
N_MOD = 5
LAG_S, LAG_M = 2, 4
X_HEAD = 8


def _bf(w):
    return pltpu.bitcast(w, BF16)


def _words(a):
    return pltpu.bitcast(a.astype(BF16), U32)


def _dot(a, b):
    return jax.lax.dot_general(a, b, (((1,), (0,)), ((), ())), preferred_element_type=F32)


def _dot_nt(a, b):
    return jax.lax.dot_general(a, b, (((1,), (1,)), ((), ())), preferred_element_type=F32)


def _round(a):
    return a.astype(BF16).astype(F32)


def _silu(x):
    h = 0.5 * x
    return h * jnp.tanh(h) + h


def _ln(x):
    m = jnp.mean(x, axis=-1, keepdims=True)
    d = x - m
    v = jnp.mean(d * d, axis=-1, keepdims=True)
    return d * jax.lax.rsqrt(v + LN_EPS)


def _mod_ln(x, scale1, shift):
    return _ln(x) * scale1 + shift


def _strassen_lhs(a11, a12, a21, a22):
    return [a11 + a22, a21 + a22, a11, a22, a11 + a12, a21 - a11, a12 - a22]


def _strassen_out(m):
    return m[3] - m[4] + m[0] + m[6], m[2] + m[4], m[1] + m[3], m[2] - m[1] + m[0] + m[5]


def _strassen_rhs(b11, b12, b21, b22):
    return [b11 + b22, b11, b12 - b22, b21 - b11, b22, b11 + b12, b21 + b22]


PLACE = (0, 1, 3, 2, 4, 5, 6)
RAW = (1, 2, 3, 4)
KEPT = (1, 4)
PRODUCT_ORDER = (1, 3, 2, 4, 0, 6, 5)


def _operand(w, i, r=0, n=None):
    size = w.shape[-2] // 7
    return pl.ds(PLACE[i] * size + r, size if n is None else n)


def _halves(w):
    return pltpu.bitcast(jnp.concatenate([w << 16, w & np.uint32(0xFFFF0000)], axis=0), F32)


def _join(t):
    u = pltpu.bitcast(t, U32)
    n = u.shape[0] // 2
    return ((u[:n] + np.uint32(0x8000)) >> 16) | ((u[n:] + np.uint32(0x7FFF)) & np.uint32(0xFFFF0000))


def _prepare_one_level(w, c, r, n, k):
    raw = [_halves(w[c, 0, _operand(w, i, r, n), k:k + 128]) for i in RAW]
    for i, t in enumerate(_strassen_rhs(*raw)):
        if i not in KEPT:
            w[c, 0, _operand(w, i, r, n), k:k + 128] = _join(t)


def _prepare_two_levels(w, c, r, n, k):
    outer = [_strassen_rhs(*[_halves(w[c, i, _operand(w, j, r, n), k:k + 128]) for i in RAW]) for j in RAW]
    for i in range(7):
        for j, t in enumerate(_strassen_rhs(*[sub[i] for sub in outer])):
            if i not in KEPT or j not in KEPT:
                w[c, i, _operand(w, j, r, n), k:k + 128] = _join(t)


def _kernel(c_ref, mem0_ref, x_hbm, wq_hbm, wk_hbm, wv_hbm, wo_hbm, w1_hbm, w3_hbm, w2_hbm,
            wmod_hbm, out_hbm,
            wqkv, wo, wup2, wup1, wdn, wrest, wmod, stage, xs, mod, lhs, obuf, x1, h2, hpre, pre,
            sem_stage, sem_misc, sem_mod, sem_ffn, sem_out, *, seg, n_mem, dh):
    n_pairs = wqkv.shape[0] // 6
    dm = lhs.shape[1]
    rows = n_mem + seg
    hseg = seg // 2
    n_seg = xs.shape[0]
    n_blk = n_seg // FFN_SEGS
    blk = FFN_SEGS * seg
    fq = wup2.shape[3]
    fc = 2 * fq + wup1.shape[3]
    kd = 2 * wdn.shape[2] // 7
    hd = dm // 2
    scale = dh ** -0.5

    wmod32 = wmod_hbm.bitcast(U32)
    x32 = x_hbm.bitcast(U32)
    out32 = out_hbm.bitcast(U32)
    qkv32 = [w.bitcast(U32) for w in (wq_hbm, wk_hbm, wv_hbm)]
    hpr = PRE_ROWS // 2
    tail = pl.ds(hseg - hpr, hpr)
    cp_xpre = pltpu.make_async_copy(x32.at[:, tail, :], xs.at[:, tail, :], sem_misc.at[0])
    cp_x0 = pltpu.make_async_copy(x32.at[pl.ds(0, X_HEAD)], xs.at[pl.ds(0, X_HEAD)], sem_misc.at[1])
    cp_x1 = pltpu.make_async_copy(x32.at[pl.ds(X_HEAD, n_seg - X_HEAD)], xs.at[pl.ds(X_HEAD, n_seg - X_HEAD)],
                                  sem_misc.at[2])
    cp_wo = pltpu.make_async_copy(wo_hbm.bitcast(U32), wo, sem_misc.at[3])

    def cp_mod(k):
        return pltpu.make_async_copy(wmod32.at[:, pl.ds(pl.multiple_of(k * dm, dm), dm)], wmod.at[k % N_MOD],
                                     sem_mod.at[k])

    def cp_stage(j):
        slot = j & (N_STAGE - 1)
        return [pltpu.make_async_copy(qkv32[i].at[:, j, :], stage.at[slot, i, pl.ds(0, dm)],
                                      sem_stage.at[3 * slot + i])
                for i in range(3)]

    def cp_ffn(c):
        w1_32, w3_32, w2_32 = w1_hbm.bitcast(U32), w3_hbm.bitcast(U32), w2_hbm.bitcast(U32)

        def up_cols(off, n):
            return pl.ds(pl.multiple_of(c * fc + off, 128), n)

        def w2_rows(off, n):
            return pl.ds(pl.multiple_of(c * (fc // 2) + off, 64), n)

        pairs = []
        for side, w in enumerate((w1_32, w3_32)):
            for i in range(2):
                for j in range(2):
                    pairs.append((w.at[pl.ds(i * (hd // 2), hd // 2), up_cols(j * fq, fq)],
                                  wup2.at[c, RAW[2 * i + side], _operand(wup2, RAW[j], 0, hd // 2)]))
            pairs.append((w.at[:, up_cols(2 * fq, fc - 2 * fq)], wup1.at[c, 0, _operand(wup1, RAW[side], 0, hd)]))
            pairs.append((w2_32.at[w2_rows(0, kd), pl.ds(side * hd, hd)],
                          wdn.at[c, 0, _operand(wdn, RAW[side], 0, kd)]))
        pairs.append((w2_32.at[w2_rows(kd, fc // 2 - kd), :], wrest.at[c]))
        return [pltpu.make_async_copy(src, dst, sem_ffn.at[c]) for src, dst in pairs]

    def cp_out(b):
        r = pl.ds(b * FFN_SEGS, FFN_SEGS)
        return pltpu.make_async_copy(xs.at[r], out32.at[r], sem_out.at[b])

    cp_xpre.start()
    cp_mod(1).start()
    cp_mod(0).start()
    for j in range(N_STAGE):
        for cp in cp_stage(j):
            cp.start()

    cf = c_ref[...].astype(F32)
    sc = jnp.broadcast_to(_round(cf * jax.nn.sigmoid(cf)), (8, dm))

    def set_mod(k):
        mod[k] = _dot(sc, _bf(wmod[k % N_MOD])) + jnp.where(k % 3 == 1, 1.0, 0.0)

    def get_mod(k, n):
        return jnp.concatenate([mod[k]] * (n // 8), axis=0)

    def seg_x(s):
        return _bf(xs[s]).astype(F32)

    def seg_h(s):
        return _round(_mod_ln(seg_x(s), get_mod(1, seg), get_mod(0, seg)))

    parked = pre.shape[0] - dm // dh

    def pre_norm(i, _):
        t = _ln(_bf(jnp.concatenate([xs[2 * i, tail], xs[2 * i + 1, tail]], axis=0)).astype(F32))
        for k in range(dm // dh):
            pre[parked + k, pl.ds(pl.multiple_of(i * 2 * PRE_ROWS, 2 * PRE_ROWS), 2 * PRE_ROWS), :] = (
                t[:, k * dh:(k + 1) * dh])

    def pre_mod(i, _):
        t = jnp.concatenate([pre[parked + k, pl.ds(pl.multiple_of(i * 64, 64), 64), :]
                             for k in range(dm // dh)], axis=1)
        hpre[pl.ds(pl.multiple_of(i * 32, 32), 32), :] = _words(t * get_mod(1, 64) + get_mod(0, 64))

    cp_xpre.wait()
    jax.lax.fori_loop(0, n_seg // 2, pre_norm, None, unroll=8)
    for k in (1, 0):
        cp_mod(k).wait()
        set_mod(k)
    jax.lax.fori_loop(0, n_seg * PRE_ROWS // 64, pre_mod, None)

    def relayout(j, r, n):
        for i in range(3):
            even, odd = [stage[j & (N_STAGE - 1), i, pl.ds(2 * r + k, n, stride=2), :] for k in range(2)]
            wqkv[6 * j + 2 * i, pl.ds(r, n), :] = (even & np.uint32(0xFFFF)) | (odd << 16)
            wqkv[6 * j + 2 * i + 1, pl.ds(r, n), :] = (even >> 16) | (odd & np.uint32(0xFFFF0000))

    def refill(j):
        @pl.when(j + N_STAGE < n_pairs)
        def _():
            for cp in cp_stage(j + N_STAGE):
                cp.start()

        def queue_rest(*_):
            cp_x0.start()
            cp_wo.start()
            for k in range(2, 6):
                cp_mod(k).start()
            cp_x1.start()

        jax.lax.fori_loop(0, jnp.where(j + N_STAGE == n_pairs, 1, 0), queue_rest, None)

    def pre_proj(i, _):
        j = jnp.minimum(i, n_pairs - 1)

        @pl.when(jnp.logical_and(i > 0, i < n_pairs))
        def _():
            for cp in cp_stage(j):
                cp.wait()

        half = hpre.shape[0] // 2
        a = _bf(hpre[pl.ds(pl.multiple_of((i & 1) * half, half), half), :])
        res = []
        for t in range(6):
            tile = (i >> 1) * 6 + t
            res.append(_dot(a, _bf(wqkv[tile])))
            pre[tile, pl.ds(pl.multiple_of((i & 1) * 2 * half, 2 * half), 2 * half), :] = res[t]
            if 1 <= t <= 4:
                for g in range(2):
                    stage[j & (N_STAGE - 1), 0, pl.ds(pl.multiple_of(dm + (i >> 8) * 8, 8), 8), :] = (
                        pltpu.bitcast(res[t - 1][g * half:g * half + 8], U32))
                    relayout(j, (2 * t - 2 + g) * (dm // 16), dm // 16)
        refill(i)

    for cp in cp_stage(0):
        cp.wait()
    jax.lax.fori_loop(0, dm // 128, lambda t, _: relayout(0, pl.multiple_of(t * 64, 64), 64), None)
    jax.lax.fori_loop(0, 2 * N_PRE, pre_proj, None)
    cp_x0.wait()
    lhs[0:n_mem, :] = mem0_ref[...].astype(F32)
    lhs[n_mem:rows, :] = seg_h(0)

    def finish(s, attn):
        xn = seg_x(s) + get_mod(2, seg) * attn
        slot = (s >> 2) & 1
        sub = s & 3
        x1[slot, pl.ds(pl.multiple_of(sub * seg, seg), seg), :] = xn
        h = _mod_ln(xn, get_mod(4, seg), get_mod(3, seg))
        for i, t in enumerate(_strassen_lhs(h[:hseg, :hd], h[:hseg, hd:], h[hseg:, :hd], h[hseg:, hd:])):
            h2[slot, i, pl.ds(pl.multiple_of(sub * hseg, hseg), hseg), :] = t

    def step(s, phase):
        do_attn = phase != "ffn"
        do_ffn = phase != "first"
        if do_ffn:
            fb = (s >> 2) - 1
            fch = s & 3
            fslot = fb & 1
            act_a, act_b = [None] * (2 * (fq // 128) + 1), [None] * (2 * (fq // 128) + 1)
        up_work, down_work = [], []
        if phase == "first":
            for cp in cp_ffn(s):
                cp.start()
        if phase == "prep":
            for cp in cp_ffn(fch):
                cp.wait()
            up_work = [(_prepare_two_levels, wup2, r, 8, k)
                       for k in range(0, fq, 128) for r in range(0, hd // 4, 8)]
            down_work = [(_prepare_one_level, w, r, 32, k) for w in (wup1, wdn)
                         for k in range(0, w.shape[3], 128) for r in range(0, w.shape[2] // 7, 32)]

        def prepare_weights(work, i, n, anchor):
            todo = work[-(-len(work) * i // n):-(-len(work) * (i + 1) // n)]
            for _, w, r, _, k in todo[:1]:
                w[fch, fb, r:r + 8, k:k + 128] = pltpu.bitcast(anchor, U32)
            for prepare, w, r, size, k in todo:
                prepare(w, fch, r, size, k)

        nq = fq // 128
        def gate(t, products):
            ga, ua, gb, ub = _strassen_out(products)
            act_a[t] = _silu(ga) * ua
            act_b[t] = _silu(gb) * ub

        def ffn_up():
            inner_ops = []
            for i in range(7):
                h = h2[fslot, i]
                inner_ops.append([v.astype(BF16) for v in _strassen_lhs(
                    h[:seg, :hd // 2], h[:seg, hd // 2:], h[seg:, :hd // 2], h[seg:, hd // 2:])])
            for t in range(nq):
                left, right = {}, {}
                for i in PRODUCT_ORDER:
                    c11, c12, c21, c22 = _strassen_out(
                        {j: _dot(inner_ops[i][j], _bf(wup2[fch, i, _operand(wup2, j), t * 128:(t + 1) * 128]))
                         for j in PRODUCT_ORDER})
                    left[i] = jnp.concatenate([c11, c21], axis=0)
                    right[i] = jnp.concatenate([c12, c22], axis=0)
                gate(t, left)
                gate(nq + t, right)
                yield
            gate(2 * nq, [_dot(h2[fslot, i].astype(BF16), _bf(wup1[fch, 0, _operand(wup1, i), :]))
                          for i in range(7)])

        up = ffn_up()

        def ffn_down():
            if do_ffn:
                aa, ab = jnp.concatenate(act_a, axis=1), jnp.concatenate(act_b, axis=1)
                ops = [t.astype(BF16) for t in _strassen_lhs(
                    aa[:, :kd], aa[:, kd:2 * kd], ab[:, :kd], ab[:, kd:2 * kd])]
                rest = _dot(jnp.concatenate([aa[:, 2 * kd:], ab[:, 2 * kd:]], axis=0).astype(BF16),
                            _bf(wrest[fch]))
                for t in range(0, hd, DOWN_COLS):
                    y = _strassen_out({i: _dot(ops[i], _bf(wdn[fch, 0, _operand(wdn, i), t:t + DOWN_COLS]))
                                       for i in PRODUCT_ORDER})
                    for side in range(2):
                        cols = slice(side * hd + t, side * hd + t + DOWN_COLS)
                        ya = y[side] + rest[:blk // 2, cols]
                        yb = y[2 + side] + rest[blk // 2:, cols]
                        yy = jnp.concatenate([v[k * hseg:(k + 1) * hseg] for k in range(FFN_SEGS)
                                              for v in (ya, yb)], axis=0)
                        acc = x1[fslot, :, cols] + get_mod(5, blk)[:, cols] * yy
                        x1[fslot, :, cols] = acc
                        for k in range(FFN_SEGS):
                            xs[fb * FFN_SEGS + k, :, cols] = _words(acc[k * seg:(k + 1) * seg])

        if not do_attn:
            list(up)
            ffn_down()
        else:
            r = jax.lax.broadcasted_iota(jnp.int32, (2 * rows, 2 * rows), 0)
            q = jax.lax.broadcasted_iota(jnp.int32, (2 * rows, 2 * rows), 1)
            same = (r >= rows) == (q >= rows)
            rl = jnp.where(r >= rows, r - rows, r)
            ql = jnp.where(q >= rows, q - rows, q)
            keep = same & ((rl < n_mem) | (rl >= ql))
            fill = jnp.where(same, -1e9, -jnp.inf).astype(F32)
            a = lhs[...]
            a_short = a[:rows - PRE_ROWS].astype(BF16)
            qkv, probs = {}, {}

            def proj(j):
                t = []
                for tile in range(6 * j, 6 * j + 6):
                    if tile < pre.shape[0]:
                        t.append(jnp.concatenate(
                            [_dot(a_short, _bf(wqkv[tile])),
                             pre[tile, pl.ds(pl.multiple_of(s * PRE_ROWS, PRE_ROWS), PRE_ROWS), :]], axis=0))
                    else:
                        t.append(_dot(a, _bf(wqkv[tile])))
                prepare_weights(up_work, j, n_pairs, t[0][0:8])
                prepare_weights(down_work, j, n_pairs, t[3][0:8])
                qkv[j] = [jnp.concatenate(t[2 * i:2 * i + 2], axis=0).astype(BF16) for i in range(3)]

            def scores(j):
                t = jnp.where(keep, _dot_nt(qkv[j][0], qkv[j][1]) * scale, fill)
                e = jnp.exp(t - jnp.max(t, axis=-1, keepdims=True))
                probs[j] = (e / jnp.sum(e, axis=-1, keepdims=True)).astype(BF16)

            def mix(j):
                o = _round(_dot(probs[j], qkv[j][2]))
                obuf[:, 2 * j * dh:(2 * j + 1) * dh] = o[:rows]
                obuf[:, (2 * j + 1) * dh:(2 * j + 2) * dh] = o[rows:]

            def oproj(lo, hi):
                return _dot(obuf[:, lo * 2 * dh:hi * 2 * dh], _bf(wo[lo * dh:hi * dh, :]))

            per_part = (n_pairs - 4) // LAG_M

            def oproj_part(k):
                parts.append(oproj(per_part * k, per_part * (k + 1)))

            def first_waits():
                @pl.when(s == 0)
                def _():
                    cp_wo.wait()

                @pl.when(s > 0)
                def _():
                    cp_mod(s + 1).wait()

            fillers = [functools.partial(proj, j) for j in range(n_pairs)]
            parts = []
            if phase == "both":
                fillers += [lambda: next(up, None)] * LAG_M
                done = 0
            else:
                if phase == "first":
                    fillers.insert(n_pairs - 1, first_waits)
                fillers += [functools.partial(oproj_part, k) for k in range(LAG_M)]
                done = per_part * LAG_M
            for i, filler in enumerate(fillers):
                filler()
                if 0 <= i - LAG_S < n_pairs:
                    scores(i - LAG_S)
                if 0 <= i - LAG_M < n_pairs:
                    mix(i - LAG_M)
            if do_ffn:
                list(up)
            o = sum(parts, oproj(done, n_pairs))
            lhs[0:n_mem, :] = _round(o[:n_mem])
            lhs[n_mem:rows, :] = seg_h(jnp.minimum(s + 1, n_seg - 1))
            if phase != "first":
                finish(s, o[n_mem:])
            else:
                x1[0, pl.ds(pl.multiple_of(s * seg, seg), seg), :] = o[n_mem:]
                set_mod(s + 1)
            ffn_down()

        if do_ffn:
            @pl.when(fch == FFN_SEGS - 1)
            def _():
                cp_out(fb).start()

    def run(lo, hi, phase):
        jax.lax.fori_loop(lo, hi, lambda s, _: step(s, phase), None)

    run(0, FFN_SEGS, "first")
    cp_x1.wait()
    cp_mod(5).wait()
    set_mod(5)
    for s in range(FFN_SEGS):
        finish(s, x1[0, s * seg:(s + 1) * seg, :])
    run(FFN_SEGS, 2 * FFN_SEGS, "prep")
    run(2 * FFN_SEGS, n_seg, "both")
    run(n_seg, n_seg + FFN_SEGS, "ffn")
    for b in range(n_blk):
        cp_out(b).wait()


@functools.partial(jax.jit, static_argnames=("A_seg_len",))
def pallas_adaLN_cond__memory_aug_recurrent_mem_tr__glu_gated_swiglu__prompt_kernel(
    A_x, A_mem0, A_Wq, A_Wk, A_Wv, A_Wo, A_seg_len, B_x, B_w1, B_w3, B_w2, c, w_mod,
):
    del B_x
    bsz, s_len, dm = A_x.shape
    _, n_heads, dh = A_Wq.shape
    n_mem = A_mem0.shape[1]
    seg = int(A_seg_len)
    f = B_w1.shape[1]
    fc = f // FFN_SEGS
    kd = (fc - 1) // 256 * 128
    blk = FFN_SEGS * seg
    assert bsz == 1 and s_len % blk == 0 and n_heads % 4 == 0 and fc % 128 == 0 and FFN_SEGS == 4
    assert n_heads // 4 <= N_PRE <= n_heads // 2

    hbm = pl.BlockSpec(memory_space=pltpu.MemorySpace.HBM)
    vmem = pl.BlockSpec(memory_space=pltpu.MemorySpace.VMEM)
    scratch = dict(
        wqkv=pltpu.VMEM((3 * n_heads, dm // 2, dh), U32),
        wo=pltpu.VMEM((n_heads * dh // 2, dm), U32),
        wup2=pltpu.VMEM((FFN_SEGS, 7, 7 * dm // 8, kd), U32),
        wup1=pltpu.VMEM((FFN_SEGS, 1, 7 * dm // 4, fc - 2 * kd), U32),
        wdn=pltpu.VMEM((FFN_SEGS, 1, 7 * kd // 2, dm // 2), U32),
        wrest=pltpu.VMEM((FFN_SEGS, fc // 2 - kd, dm), U32),
        wmod=pltpu.VMEM((N_MOD, dm // 2, dm), U32),
        stage=pltpu.VMEM((N_STAGE, 3, dm + 8, dh), U32),
        xs=pltpu.VMEM((s_len // seg, seg // 2, dm), U32),
        mod=pltpu.VMEM((6, 8, dm), F32),
        lhs=pltpu.VMEM((n_mem + seg, dm), F32),
        obuf=pltpu.VMEM((n_mem + seg, n_heads * dh), F32),
        x1=pltpu.VMEM((2, blk, dm), F32),
        h2=pltpu.VMEM((2, 7, blk // 2, dm // 2), F32),
        hpre=pltpu.VMEM((s_len // seg * PRE_ROWS // 2, dm), U32),
        pre=pltpu.VMEM((6 * N_PRE, s_len // seg * PRE_ROWS, dh), F32),
        sem_stage=pltpu.SemaphoreType.DMA((3 * N_STAGE,)),
        sem_misc=pltpu.SemaphoreType.DMA((4,)),
        sem_mod=pltpu.SemaphoreType.DMA((6,)),
        sem_ffn=pltpu.SemaphoreType.DMA((FFN_SEGS,)),
        sem_out=pltpu.SemaphoreType.DMA((s_len // blk,)),
    )

    def body(*refs):
        n_io = len(refs) - len(scratch)
        _kernel(*refs[:n_io], **dict(zip(scratch, refs[n_io:])), seg=seg, n_mem=n_mem, dh=dh)

    out = pl.pallas_call(
        body,
        out_shape=jax.ShapeDtypeStruct((s_len // seg, seg, dm), A_x.dtype),
        in_specs=[vmem, vmem] + [hbm] * 9,
        out_specs=hbm,
        scratch_shapes=list(scratch.values()),
        compiler_params=pltpu.CompilerParams(
            vmem_limit_bytes=127 * 2**20,
            flags={"XLA_TPU_EVENLY_DISTRIBUTE_CRITICAL_NODES": True}),
    )(c, A_mem0.reshape(n_mem, dm), A_x.reshape(s_len // seg, seg, dm), A_Wq, A_Wk, A_Wv,
      A_Wo.reshape(n_heads * dh, dm), B_w1, B_w3, B_w2, w_mod)
    return out.reshape(bsz, s_len, dm)
```

```python
import functools

import jax
import jax.numpy as jnp
import numpy as np
import jax.experimental.pallas as pl
import jax.experimental.pallas.tpu as pltpu

U32 = jnp.uint32
BF16 = jnp.bfloat16
F32 = jnp.float32
LN_EPS = 1e-5
FFN_SEGS = 4
N_STAGE = 4
N_PRE = 9
PRE_ROWS = 8
N_MOD = 5
LAG_S, LAG_M = 2, 4
X_HEAD = 8


def _bf(w):
    return pltpu.bitcast(w, BF16)


def _words(a):
    return pltpu.bitcast(a.astype(BF16), U32)


def _dot(a, b):
    return jax.lax.dot_general(a, b, (((1,), (0,)), ((), ())), preferred_element_type=F32)


def _dot_nt(a, b):
    return jax.lax.dot_general(a, b, (((1,), (1,)), ((), ())), preferred_element_type=F32)


def _round(a):
    return a.astype(BF16).astype(F32)


def _silu(x):
    h = 0.5 * x
    return h * jnp.tanh(h) + h


def _ln(x):
    m = jnp.mean(x, axis=-1, keepdims=True)
    d = x - m
    v = jnp.mean(d * d, axis=-1, keepdims=True)
    return d * jax.lax.rsqrt(v + LN_EPS)


def _mod_ln(x, scale1, shift):
    return _ln(x) * scale1 + shift


def _strassen_lhs(a11, a12, a21, a22):
    return [a11 + a22, a21 + a22, a11, a22, a11 + a12, a21 - a11, a12 - a22]


def _strassen_out(m):
    return m[3] - m[4] + m[0] + m[6], m[2] + m[4], m[1] + m[3], m[2] - m[1] + m[0] + m[5]


def _strassen_rhs(b11, b12, b21, b22):
    return [b11 + b22, b11, b12 - b22, b21 - b11, b22, b11 + b12, b21 + b22]


PLACE = (0, 1, 3, 2, 4, 5, 6)
RAW = (1, 2, 3, 4)
KEPT = (1, 4)
PRODUCT_ORDER = (1, 3, 2, 4, 0, 6, 5)


def _operand(w, i, r=0, n=None):
    size = w.shape[-2] // 7
    return pl.ds(PLACE[i] * size + r, size if n is None else n)


def _halves(w):
    return pltpu.bitcast(jnp.concatenate([w << 16, w & np.uint32(0xFFFF0000)], axis=0), F32)


def _join(t):
    u = pltpu.bitcast(t, U32)
    n = u.shape[0] // 2
    return ((u[:n] + np.uint32(0x8000)) >> 16) | ((u[n:] + np.uint32(0x7FFF)) & np.uint32(0xFFFF0000))


def _prepare_one_level(w, c, r, n, k):
    raw = [_halves(w[c, 0, _operand(w, i, r, n), k:k + 128]) for i in RAW]
    for i, t in enumerate(_strassen_rhs(*raw)):
        if i not in KEPT:
            w[c, 0, _operand(w, i, r, n), k:k + 128] = _join(t)


def _prepare_two_levels(w, c, r, n, k):
    outer = [_strassen_rhs(*[_halves(w[c, i, _operand(w, j, r, n), k:k + 128]) for i in RAW]) for j in RAW]
    for i in range(7):
        for j, t in enumerate(_strassen_rhs(*[sub[i] for sub in outer])):
            if i not in KEPT or j not in KEPT:
                w[c, i, _operand(w, j, r, n), k:k + 128] = _join(t)


def _kernel(c_ref, mem0_ref, x_hbm, wq_hbm, wk_hbm, wv_hbm, wo_hbm, w1_hbm, w3_hbm, w2_hbm,
            wmod_hbm, out_hbm,
            wqkv, wo, wup2, wup1, wdn, wrest, wmod, stage, xs, mod, lhs, obuf, x1, h2, hpre, pre,
            sem_stage, sem_misc, sem_mod, sem_ffn, sem_out, *, seg, n_mem, dh):
    n_pairs = wqkv.shape[0] // 6
    dm = lhs.shape[1]
    rows = n_mem + seg
    hseg = seg // 2
    n_seg = xs.shape[0]
    n_blk = n_seg // FFN_SEGS
    blk = FFN_SEGS * seg
    fq = wup2.shape[3]
    fc = 2 * fq + wup1.shape[3]
    kd = 2 * wdn.shape[2] // 7
    nq = fq // 128
    hd = dm // 2
    scale = dh ** -0.5

    wmod32 = wmod_hbm.bitcast(U32)
    x32 = x_hbm.bitcast(U32)
    out32 = out_hbm.bitcast(U32)
    qkv32 = [w.bitcast(U32) for w in (wq_hbm, wk_hbm, wv_hbm)]
    hpr = PRE_ROWS // 2
    tail = pl.ds(hseg - hpr, hpr)
    cp_xpre = pltpu.make_async_copy(x32.at[:, tail, :], xs.at[:, tail, :], sem_misc.at[0])
    cp_x0 = pltpu.make_async_copy(x32.at[pl.ds(0, X_HEAD)], xs.at[pl.ds(0, X_HEAD)], sem_misc.at[1])
    cp_x1 = pltpu.make_async_copy(x32.at[pl.ds(X_HEAD, n_seg - X_HEAD)], xs.at[pl.ds(X_HEAD, n_seg - X_HEAD)],
                                  sem_misc.at[2])
    cp_wo = pltpu.make_async_copy(wo_hbm.bitcast(U32), wo, sem_misc.at[3])

    def cp_mod(k):
        return pltpu.make_async_copy(wmod32.at[:, pl.ds(pl.multiple_of(k * dm, dm), dm)], wmod.at[k % N_MOD],
                                     sem_mod.at[k])

    def cp_stage(j):
        slot = j & (N_STAGE - 1)
        return [pltpu.make_async_copy(qkv32[i].at[:, j, :], stage.at[slot, i, pl.ds(0, dm)],
                                      sem_stage.at[3 * slot + i])
                for i in range(3)]

    def cp_ffn(c):
        w1_32, w3_32, w2_32 = w1_hbm.bitcast(U32), w3_hbm.bitcast(U32), w2_hbm.bitcast(U32)

        def up_cols(off, n):
            return pl.ds(pl.multiple_of(c * fc + off, 128), n)

        def w2_rows(off, n):
            return pl.ds(pl.multiple_of(c * (fc // 2) + off, 64), n)

        pairs = []
        for side, w in enumerate((w1_32, w3_32)):
            for i in range(2):
                for j in range(2):
                    pairs.append((w.at[pl.ds(i * (hd // 2), hd // 2), up_cols(j * fq, fq)],
                                  wup2.at[c, RAW[2 * i + side], _operand(wup2, RAW[j], 0, hd // 2)]))
            pairs.append((w.at[:, up_cols(2 * fq, fc - 2 * fq)], wup1.at[c, 0, _operand(wup1, RAW[side], 0, hd)]))
            pairs.append((w2_32.at[w2_rows(0, kd), pl.ds(side * hd, hd)],
                          wdn.at[c, 0, _operand(wdn, RAW[side], 0, kd)]))
        pairs.append((w2_32.at[w2_rows(kd, fc // 2 - kd), :], wrest.at[c]))
        return [pltpu.make_async_copy(src, dst, sem_ffn.at[c]) for src, dst in pairs]

    def cp_out(b):
        r = pl.ds(b * FFN_SEGS, FFN_SEGS)
        return pltpu.make_async_copy(xs.at[r], out32.at[r], sem_out.at[b])

    cp_xpre.start()
    cp_mod(1).start()
    cp_mod(0).start()
    for j in range(N_STAGE):
        for cp in cp_stage(j):
            cp.start()

    cf = c_ref[...].astype(F32)
    sc = jnp.broadcast_to(_round(cf * jax.nn.sigmoid(cf)), (8, dm))

    def set_mod(k):
        mod[k] = _dot(sc, _bf(wmod[k % N_MOD])) + jnp.where(k % 3 == 1, 1.0, 0.0)

    def get_mod(k, n):
        return jnp.concatenate([mod[k]] * (n // 8), axis=0)

    def seg_x(s):
        return _bf(xs[s]).astype(F32)

    def seg_h(s):
        return _round(_mod_ln(seg_x(s), get_mod(1, seg), get_mod(0, seg)))

    parked = pre.shape[0] - dm // dh

    def pre_norm(i, _):
        t = _ln(_bf(jnp.concatenate([xs[2 * i, tail], xs[2 * i + 1, tail]], axis=0)).astype(F32))
        for k in range(dm // dh):
            pre[parked + k, pl.ds(pl.multiple_of(i * 2 * PRE_ROWS, 2 * PRE_ROWS), 2 * PRE_ROWS), :] = (
                t[:, k * dh:(k + 1) * dh])

    def pre_mod(i, _):
        t = jnp.concatenate([pre[parked + k, pl.ds(pl.multiple_of(i * 64, 64), 64), :]
                             for k in range(dm // dh)], axis=1)
        hpre[pl.ds(pl.multiple_of(i * 32, 32), 32), :] = _words(t * get_mod(1, 64) + get_mod(0, 64))

    cp_xpre.wait()
    jax.lax.fori_loop(0, n_seg // 2, pre_norm, None, unroll=8)
    for k in (1, 0):
        cp_mod(k).wait()
        set_mod(k)
    jax.lax.fori_loop(0, n_seg * PRE_ROWS // 64, pre_mod, None)

    def relayout(j, r, n):
        for i in range(3):
            even, odd = [stage[j & (N_STAGE - 1), i, pl.ds(2 * r + k, n, stride=2), :] for k in range(2)]
            wqkv[6 * j + 2 * i, pl.ds(r, n), :] = (even & np.uint32(0xFFFF)) | (odd << 16)
            wqkv[6 * j + 2 * i + 1, pl.ds(r, n), :] = (even >> 16) | (odd & np.uint32(0xFFFF0000))

    def refill(j):
        @pl.when(j + N_STAGE < n_pairs)
        def _():
            for cp in cp_stage(j + N_STAGE):
                cp.start()

        def queue_rest(*_):
            cp_x0.start()
            cp_wo.start()
            for k in range(2, 6):
                cp_mod(k).start()
            cp_x1.start()

        jax.lax.fori_loop(0, jnp.where(j + N_STAGE == n_pairs, 1, 0), queue_rest, None)

    def pre_proj(i, _):
        j = jnp.minimum(i, n_pairs - 1)

        @pl.when(jnp.logical_and(i > 0, i < n_pairs))
        def _():
            for cp in cp_stage(j):
                cp.wait()

        half = hpre.shape[0] // 2
        a = _bf(hpre[pl.ds(pl.multiple_of((i & 1) * half, half), half), :])
        res = []
        for t in range(6):
            tile = (i >> 1) * 6 + t
            res.append(_dot(a, _bf(wqkv[tile])))
            pre[tile, pl.ds(pl.multiple_of((i & 1) * 2 * half, 2 * half), 2 * half), :] = res[t]
            if 1 <= t <= 4:
                for g in range(2):
                    stage[j & (N_STAGE - 1), 0, pl.ds(pl.multiple_of(dm + (i >> 8) * 8, 8), 8), :] = (
                        pltpu.bitcast(res[t - 1][g * half:g * half + 8], U32))
                    relayout(j, (2 * t - 2 + g) * (dm // 16), dm // 16)
        refill(i)

    for cp in cp_stage(0):
        cp.wait()
    jax.lax.fori_loop(0, dm // 128, lambda t, _: relayout(0, pl.multiple_of(t * 64, 64), 64), None)
    jax.lax.fori_loop(0, 2 * N_PRE, pre_proj, None)
    cp_x0.wait()
    lhs[0:n_mem, :] = mem0_ref[...].astype(F32)
    lhs[n_mem:rows, :] = seg_h(0)

    def finish(s, attn):
        xn = seg_x(s) + get_mod(2, seg) * attn
        slot = (s >> 2) & 1
        sub = s & 3
        x1[slot, pl.ds(pl.multiple_of(sub * seg, seg), seg), :] = xn
        h = _mod_ln(xn, get_mod(4, seg), get_mod(3, seg))
        for i, t in enumerate(_strassen_lhs(h[:hseg, :hd], h[:hseg, hd:], h[hseg:, :hd], h[hseg:, hd:])):
            h2[slot, i, pl.ds(pl.multiple_of(sub * hseg, hseg), hseg), :] = t

    def step(s, phase):
        do_attn = phase != "ffn"
        do_ffn = phase != "first"
        if do_ffn:
            fb = (s >> 2) - 1
            fch = s & 3
            fslot = fb & 1
            act_a, act_b = [None] * (2 * nq + 1), [None] * (2 * nq + 1)
        up_work, down_work = [], []
        if phase == "first":
            for cp in cp_ffn(s):
                cp.start()
        if phase == "prep":
            for cp in cp_ffn(fch):
                cp.wait()
            up_work = [(_prepare_two_levels, wup2, r, 8, k)
                       for k in range(0, fq, 128) for r in range(0, hd // 4, 8)]
            down_work = [(_prepare_one_level, w, r, 32, k) for w in (wup1, wdn)
                         for k in range(0, w.shape[3], 128) for r in range(0, w.shape[2] // 7, 32)]

        def prepare_weights(work, i, n, anchor):
            todo = work[-(-len(work) * i // n):-(-len(work) * (i + 1) // n)]
            for _, w, r, _, k in todo[:1]:
                w[fch, fb, r:r + 8, k:k + 128] = pltpu.bitcast(anchor, U32)
            for prepare, w, r, size, k in todo:
                prepare(w, fch, r, size, k)

        def gate(t, products):
            ga, ua, gb, ub = _strassen_out(products)
            act_a[t] = _silu(ga) * ua
            act_b[t] = _silu(gb) * ub

        def ffn_up():
            inner_ops = []
            for i in range(7):
                h = h2[fslot, i]
                inner_ops.append([v.astype(BF16) for v in _strassen_lhs(
                    h[:seg, :hd // 2], h[:seg, hd // 2:], h[seg:, :hd // 2], h[seg:, hd // 2:])])
            for t in range(nq):
                left, right = {}, {}
                for i in PRODUCT_ORDER:
                    c11, c12, c21, c22 = _strassen_out(
                        {j: _dot(inner_ops[i][j], _bf(wup2[fch, i, _operand(wup2, j), t * 128:(t + 1) * 128]))
                         for j in PRODUCT_ORDER})
                    left[i] = jnp.concatenate([c11, c21], axis=0)
                    right[i] = jnp.concatenate([c12, c22], axis=0)
                gate(t, left)
                gate(nq + t, right)
                yield
            gate(2 * nq, [_dot(h2[fslot, i].astype(BF16), _bf(wup1[fch, 0, _operand(wup1, i), :]))
                          for i in range(7)])

        up = ffn_up()

        def ffn_down():
            aa, ab = jnp.concatenate(act_a, axis=1), jnp.concatenate(act_b, axis=1)
            ops = [t.astype(BF16) for t in _strassen_lhs(
                aa[:, :kd], aa[:, kd:2 * kd], ab[:, :kd], ab[:, kd:2 * kd])]
            rest = _dot(jnp.concatenate([aa[:, 2 * kd:], ab[:, 2 * kd:]], axis=0).astype(BF16),
                        _bf(wrest[fch]))
            y = _strassen_out({i: _dot(ops[i], _bf(wdn[fch, 0, _operand(wdn, i), :])) for i in PRODUCT_ORDER})
            for side in range(2):
                cols = slice(side * hd, (side + 1) * hd)
                ya = y[side] + rest[:blk // 2, cols]
                yb = y[2 + side] + rest[blk // 2:, cols]
                yy = jnp.concatenate([v[k * hseg:(k + 1) * hseg] for k in range(FFN_SEGS)
                                      for v in (ya, yb)], axis=0)
                acc = x1[fslot, :, cols] + get_mod(5, blk)[:, cols] * yy
                x1[fslot, :, cols] = acc
                for k in range(FFN_SEGS):
                    xs[fb * FFN_SEGS + k, :, cols] = _words(acc[k * seg:(k + 1) * seg])

        if not do_attn:
            list(up)
            ffn_down()
        else:
            r = jax.lax.broadcasted_iota(jnp.int32, (2 * rows, 2 * rows), 0)
            q = jax.lax.broadcasted_iota(jnp.int32, (2 * rows, 2 * rows), 1)
            same = (r >= rows) == (q >= rows)
            rl = jnp.where(r >= rows, r - rows, r)
            ql = jnp.where(q >= rows, q - rows, q)
            keep = same & ((rl < n_mem) | (rl >= ql))
            fill = jnp.where(same, -1e9, -jnp.inf).astype(F32)
            a = lhs[...]
            a_short = a[:rows - PRE_ROWS].astype(BF16)
            qkv, probs = {}, {}

            def proj(j):
                t = []
                for tile in range(6 * j, 6 * j + 6):
                    if tile < pre.shape[0]:
                        t.append(jnp.concatenate(
                            [_dot(a_short, _bf(wqkv[tile])),
                             pre[tile, pl.ds(pl.multiple_of(s * PRE_ROWS, PRE_ROWS), PRE_ROWS), :]], axis=0))
                    else:
                        t.append(_dot(a, _bf(wqkv[tile])))
                prepare_weights(up_work, j, n_pairs, t[0][0:8])
                prepare_weights(down_work, j, n_pairs, t[3][0:8])
                qkv[j] = [jnp.concatenate(t[2 * i:2 * i + 2], axis=0).astype(BF16) for i in range(3)]

            def scores(j):
                t = jnp.where(keep, _dot_nt(qkv[j][0], qkv[j][1]) * scale, fill)
                e = jnp.exp(t - jnp.max(t, axis=-1, keepdims=True))
                probs[j] = (e / jnp.sum(e, axis=-1, keepdims=True)).astype(BF16)

            def mix(j):
                o = _round(_dot(probs[j], qkv[j][2]))
                obuf[:, 2 * j * dh:(2 * j + 1) * dh] = o[:rows]
                obuf[:, (2 * j + 1) * dh:(2 * j + 2) * dh] = o[rows:]

            def oproj(lo, hi):
                return _dot(obuf[:, lo * 2 * dh:hi * 2 * dh], _bf(wo[lo * dh:hi * dh, :]))

            per_part = (n_pairs - 4) // LAG_M

            def oproj_part(k):
                parts.append(oproj(per_part * k, per_part * (k + 1)))

            def first_waits():
                @pl.when(s == 0)
                def _():
                    cp_wo.wait()

                @pl.when(s > 0)
                def _():
                    cp_mod(s + 1).wait()

            fillers = [functools.partial(proj, j) for j in range(n_pairs)]
            parts = []
            if phase == "both":
                fillers += [lambda: next(up, None)] * LAG_M
                done = 0
            else:
                if phase == "first":
                    fillers.insert(n_pairs - 1, first_waits)
                fillers += [functools.partial(oproj_part, k) for k in range(LAG_M)]
                done = per_part * LAG_M
            for i, filler in enumerate(fillers):
                filler()
                if 0 <= i - LAG_S < n_pairs:
                    scores(i - LAG_S)
                if 0 <= i - LAG_M < n_pairs:
                    mix(i - LAG_M)
            if do_ffn:
                list(up)
            o = sum(parts, oproj(done, n_pairs))
            lhs[0:n_mem, :] = _round(o[:n_mem])
            lhs[n_mem:rows, :] = seg_h(jnp.minimum(s + 1, n_seg - 1))
            if do_ffn:
                finish(s, o[n_mem:])
                ffn_down()
            else:
                x1[0, pl.ds(pl.multiple_of(s * seg, seg), seg), :] = o[n_mem:]
                set_mod(s + 1)

        if do_ffn:
            @pl.when(fch == FFN_SEGS - 1)
            def _():
                cp_out(fb).start()

    def run(lo, hi, phase):
        jax.lax.fori_loop(lo, hi, lambda s, _: step(s, phase), None)

    run(0, FFN_SEGS, "first")
    cp_x1.wait()
    cp_mod(5).wait()
    set_mod(5)
    for s in range(FFN_SEGS):
        finish(s, x1[0, s * seg:(s + 1) * seg, :])
    run(FFN_SEGS, 2 * FFN_SEGS, "prep")
    run(2 * FFN_SEGS, n_seg, "both")
    run(n_seg, n_seg + FFN_SEGS, "ffn")
    for b in range(n_blk):
        cp_out(b).wait()


@functools.partial(jax.jit, static_argnames=("A_seg_len",))
def pallas_adaLN_cond__memory_aug_recurrent_mem_tr__glu_gated_swiglu__prompt_kernel(
    A_x, A_mem0, A_Wq, A_Wk, A_Wv, A_Wo, A_seg_len, B_x, B_w1, B_w3, B_w2, c, w_mod,
):
    del B_x
    bsz, s_len, dm = A_x.shape
    _, n_heads, dh = A_Wq.shape
    n_mem = A_mem0.shape[1]
    seg = int(A_seg_len)
    f = B_w1.shape[1]
    fc = f // FFN_SEGS
    kd = (fc - 1) // 256 * 128
    blk = FFN_SEGS * seg
    assert bsz == 1 and s_len % blk == 0 and n_heads % 4 == 0 and fc % 128 == 0 and FFN_SEGS == 4
    assert n_heads // 4 <= N_PRE <= n_heads // 2 and (seg, n_mem, dh) == (32, 8, 128)
    assert all(t.dtype == BF16 for t in (A_x, A_Wq, A_Wk, A_Wv, A_Wo, B_w1, B_w3, B_w2, w_mod))

    hbm = pl.BlockSpec(memory_space=pltpu.MemorySpace.HBM)
    vmem = pl.BlockSpec(memory_space=pltpu.MemorySpace.VMEM)
    scratch = dict(
        wqkv=pltpu.VMEM((3 * n_heads, dm // 2, dh), U32),
        wo=pltpu.VMEM((n_heads * dh // 2, dm), U32),
        wup2=pltpu.VMEM((FFN_SEGS, 7, 7 * dm // 8, kd), U32),
        wup1=pltpu.VMEM((FFN_SEGS, 1, 7 * dm // 4, fc - 2 * kd), U32),
        wdn=pltpu.VMEM((FFN_SEGS, 1, 7 * kd // 2, dm // 2), U32),
        wrest=pltpu.VMEM((FFN_SEGS, fc // 2 - kd, dm), U32),
        wmod=pltpu.VMEM((N_MOD, dm // 2, dm), U32),
        stage=pltpu.VMEM((N_STAGE, 3, dm + 8, dh), U32),
        xs=pltpu.VMEM((s_len // seg, seg // 2, dm), U32),
        mod=pltpu.VMEM((6, 8, dm), F32),
        lhs=pltpu.VMEM((n_mem + seg, dm), F32),
        obuf=pltpu.VMEM((n_mem + seg, n_heads * dh), F32),
        x1=pltpu.VMEM((2, blk, dm), F32),
        h2=pltpu.VMEM((2, 7, blk // 2, dm // 2), F32),
        hpre=pltpu.VMEM((s_len // seg * PRE_ROWS // 2, dm), U32),
        pre=pltpu.VMEM((6 * N_PRE, s_len // seg * PRE_ROWS, dh), F32),
        sem_stage=pltpu.SemaphoreType.DMA((3 * N_STAGE,)),
        sem_misc=pltpu.SemaphoreType.DMA((4,)),
        sem_mod=pltpu.SemaphoreType.DMA((6,)),
        sem_ffn=pltpu.SemaphoreType.DMA((FFN_SEGS,)),
        sem_out=pltpu.SemaphoreType.DMA((s_len // blk,)),
    )

    def body(*refs):
        n_io = len(refs) - len(scratch)
        _kernel(*refs[:n_io], **dict(zip(scratch, refs[n_io:])), seg=seg, n_mem=n_mem, dh=dh)

    out = pl.pallas_call(
        body,
        out_shape=jax.ShapeDtypeStruct((s_len // seg, seg, dm), A_x.dtype),
        in_specs=[vmem, vmem] + [hbm] * 9,
        out_specs=hbm,
        scratch_shapes=list(scratch.values()),
        compiler_params=pltpu.CompilerParams(
            vmem_limit_bytes=127 * 2**20,
            flags={"XLA_TPU_EVENLY_DISTRIBUTE_CRITICAL_NODES": True}),
    )(c, A_mem0.reshape(n_mem, dm), A_x.reshape(s_len // seg, seg, dm), A_Wq, A_Wk, A_Wv,
      A_Wo.reshape(n_heads * dh, dm), B_w1, B_w3, B_w2, w_mod)
    return out.reshape(bsz, s_len, dm)
```
